```python
import jax
import jax.numpy as jnp

def _softmax(x, axis=-1):
    return jax.nn.softmax(x, axis=axis)
def _gelu(x):
    return jax.nn.gelu(x, approximate=True)
def _silu(x):
    return jax.nn.silu(x)
def _sigmoid(x):
    return jax.nn.sigmoid(x)
def _layernorm(x, axis=-1, eps=1e-5):
    m = jnp.mean(x, axis=axis, keepdims=True)
    v = jnp.var(x, axis=axis, keepdims=True)
    return (x - m) / jnp.sqrt(v + eps)
def _scatter_add(tgt, idx, src, axis=0):
    return tgt.at[idx].add(src)
def _segment_sum(src, seg, n):
    return jax.ops.segment_sum(src, seg, n)
class _Rng:
    def __init__(self, key):
        self._k = key
    def _next(self):
        self._k, sub = jax.random.split(self._k)
        return sub
    def normal(self, shape):
        return jax.random.normal(self._next(), shape, dtype=jnp.bfloat16)
    def randint(self, lo, hi, shape):
        return jax.random.randint(self._next(), shape, lo, hi, dtype=jnp.int32)
    def uniform(self, shape, lo=0.0, hi=1.0):
        return jax.random.uniform(self._next(), shape, jnp.bfloat16, lo, hi)
    def permutation(self, n):
        return jax.random.permutation(self._next(), n)


kernel_name = 'parallel_sum__sliding_local_dilated__mixer_token_mlp__prompt'

def setup_inputs():
    _rng = _Rng(jax.random.key(int.from_bytes(__import__("os").urandom(4), "little")))
    _w = (lambda a: (lambda t: t.astype(jnp.bfloat16) if jnp.issubdtype(t.dtype, jnp.floating) else t)(jnp.asarray(a)))
    def _A_setup():
        B, S, D = 1, 2048, 448
        return {
            "x": _w((lambda *s: _rng.normal(s) * 0.05)(B, S, D)),
            "wqkv": _w((lambda *s: _rng.normal(s) * 0.05)(D, 3 * D)),
            "wo": _w((lambda *s: _rng.normal(s) * 0.05)(D, D)),
        }
    _A_in = _A_setup()

    def _B_setup():
        B, S, D, F = 1, 2048, 448, 1792
        return {
            "x": _w((lambda *s: _rng.normal(s) * 0.05)(B, S, D)),
            "w1": _w((lambda *s: _rng.normal(s) * 0.05)(S, F) * (S ** -0.5)),
            "b1": _w((lambda *s: _rng.normal(s) * 0.05)(F) * 0.02),
            "w2": _w((lambda *s: _rng.normal(s) * 0.05)(F, S) * (F ** -0.5)),
            "b2": _w((lambda *s: _rng.normal(s) * 0.05)(S) * 0.02),
        }
    _B_in = _B_setup()

    return {
        "A_x": _A_in["x"],
        "A_wqkv": _A_in["wqkv"],
        "A_wo": _A_in["wo"],
        "B_x": _B_in["x"],
        "B_w1": _B_in["w1"],
        "B_b1": _B_in["b1"],
        "B_w2": _B_in["w2"],
        "B_b2": _B_in["b2"],
    }

def reference(A_x, A_wqkv, A_wo, B_x, B_w1, B_b1, B_w2, B_b2):
    def _A_ref(x, wqkv, wo):
        B, S, D = x.shape
        H = 16; Dh = D // H
        W, dil = 8, 2
        qkv = (lambda x, *d: x.transpose(*d))((x @ wqkv).reshape(B, S, 3, H, Dh), 2, 0, 3, 1, 4)
        q, k, v = qkv[0], qkv[1], qkv[2]
        scale = Dh ** -0.5
        pos = jnp.arange(S)
        off = jnp.arange(W) * dil
        idx = pos[:, None] - off[None, :]
        mask = idx >= 0
        idx_c = jnp.where(mask, idx, 0).reshape(-1)
        kg = k[:, :, idx_c, :].reshape(B, H, S, W, Dh)
        vg = v[:, :, idx_c, :].reshape(B, H, S, W, Dh)
        logits = jnp.einsum("bhsd,bhswd->bhsw", q, kg) * scale
        logits = jnp.where(mask[None, None, :, :], logits, -1e9)
        attn = _softmax(logits, axis=-1)
        o = jnp.einsum("bhsw,bhswd->bhsd", attn, vg)
        return (lambda x, *d: x.transpose(*d))(o, 0, 2, 1, 3).reshape(B, S, D) @ wo

    def _B_ref(x, w1, b1, w2, b2):
        B, S, D = x.shape
        h = _layernorm(x, axis=-1)
        u = jnp.einsum("bsd,sf->bdf", h, w1) + b1
        u = _gelu(u)
        y = jnp.einsum("bdf,fs->bds", u, w2) + b2
        return (lambda x, *d: x.transpose(*d))(y, 0, 2, 1)

    x = A_x
    xn = _layernorm(x, axis=-1)
    return x + _A_ref(xn, A_wqkv, A_wo) + _B_ref(xn, B_w1, B_b1, B_w2, B_b2)
```

```python
import jax
import jax.numpy as jnp
from jax import lax
import jax.experimental.pallas as pl
import jax.experimental.pallas.tpu as pltpu

S, D, F = 2048, 448, 1792
H, DH, W = 16, 28, 8
NB = 16
EPS = 1e-5
DP = 512
XC = 256
NXC = S // XC
OC = 256
NOC = S // OC
bf16, f32, u32 = jnp.bfloat16, jnp.float32, jnp.uint32
NT = (((1,), (1,)), ((), ()))


def _ln0(x):
    m = jnp.mean(x, axis=0, keepdims=True)
    c = x - m
    v = jnp.mean(c * c, axis=0, keepdims=True)
    return c * lax.rsqrt(v + EPS)


def _row_bias(b_ref, start, n):
    b = b_ref[...].astype(f32)
    return jnp.concatenate([b[t:t + 1, :] for t in range(start // 128, (start + n) // 128)], axis=1)


def _kernel(x_hbm, wqkv_hbm, wo_hbm, w1_hbm, b1_ref, w2_hbm, b2_ref, out_hbm,
            x_v, wqkv_v, wo_v, w1_v, w2_v, hT, xn_u, u_acc, g_v, wtmp, l_qkv, l_wo,
            qkvT, kvr, oT, o_u, out_v, sem_x, sem_w1, sem_w, sem_o):
    def cp_x(c):
        return pltpu.make_async_copy(x_hbm.at[0, :, pl.ds(c * XC, XC)], x_v.at[:, pl.ds(c * XC, XC)], sem_x.at[c])

    def cp_w1(c):
        return pltpu.make_async_copy(w1_hbm.at[pl.ds(c * XC, XC), :], w1_v.at[pl.ds(c * XC, XC), :], sem_w1.at[c])

    cp_wqkv = pltpu.make_async_copy(wqkv_hbm, wqkv_v, sem_w.at[0])
    cp_wo = pltpu.make_async_copy(wo_hbm, wo_v, sem_w.at[1])
    cp_w2 = pltpu.make_async_copy(w2_hbm, w2_v, sem_w.at[2])

    def cp_out(c):
        return pltpu.make_async_copy(out_v.at[:, pl.ds(c * OC, OC)], out_hbm.at[0, :, pl.ds(c * OC, OC)], sem_o.at[c])

    for c in range(NXC):
        cp_x(c).start()
        cp_w1(c).start()
        if c == 1:
            cp_wqkv.start()
            cp_wo.start()
    cp_w2.start()

    def ln_chunk(c):
        r = c * XC
        xT = x_v[:, r:r + XC].astype(f32)
        xnT = _ln0(xT).astype(bf16)
        hT[:, r:r + XC] = _ln0(xnT.astype(f32)).astype(bf16)
        xn = jnp.concatenate([xnT, jnp.zeros((DP - D, XC), bf16)], axis=0).T
        for t in range(4):
            xn_u[t, r // 2:(r + XC) // 2, :] = pltpu.bitcast(xn[:, t * 128:(t + 1) * 128], u32)

    def prep_wqkv():
        wt = jnp.concatenate([wqkv_v[...], jnp.zeros((DP - D, 3 * D), bf16)], axis=0).T.astype(f32)
        for t in range(4):
            wtmp[t] = wt[:, t * 128:(t + 1) * 128]
        for p in range(3):
            for d in range(DH):
                rows = jnp.concatenate([wtmp[t, pl.ds(p * D + d, H, stride=DH), :] for t in range(4)], axis=1)
                l_qkv[p * D + d * H:p * D + (d + 1) * H, :] = rows.astype(bf16)

    def prep_wo():
        wo = jnp.concatenate([wo_v[...].astype(f32), jnp.zeros((D, DP - D), f32)], axis=1)
        for t in range(4):
            wtmp[t, 0:D, :] = wo[:, t * 128:(t + 1) * 128]
        for t in range(4):
            for d in range(DH):
                wtmp[t, D + d * H:D + (d + 1) * H, :] = wtmp[t, pl.ds(d, H, stride=DH), :]
            wtmp[t, 2 * D:2 * D + DP - D, :] = jnp.zeros((DP - D, 128), f32)
        wop = jnp.concatenate([wtmp[t, D:D + DP, :] for t in range(4)], axis=1)
        l_wo[...] = wop.astype(bf16).T[0:D, :]

    cp_x(0).wait()
    ln_chunk(0)
    for c in range(NXC):
        if c + 1 < NXC:
            cp_x(c + 1).wait()
        cp_w1(c).wait()
        if c == 3:
            cp_wqkv.wait()
        if c == 5:
            cp_wo.wait()
        r = c * XC
        part = jnp.dot(hT[:, r:r + XC], w1_v[r:r + XC, :], preferred_element_type=f32)
        if c == 0:
            u_acc[...] = part + _row_bias(b1_ref, 0, F)
        else:
            u_acc[...] += part
        if c + 1 < NXC:
            ln_chunk(c + 1)
        if c == 3:
            prep_wqkv()
        if c == 5:
            prep_wo()

    def qkv_block(j):
        rj = jnp.concatenate([pltpu.bitcast(xn_u[t, pl.ds(j, 64, stride=NB), :], bf16) for t in range(4)], axis=1)
        res = lax.dot_general(l_qkv[...], rj, NT, preferred_element_type=f32)
        qkvT[j] = res
        if j >= NB - (W - 1):
            kvr[j - (NB - (W - 1))] = pltpu.roll(res[D:, :], 2, axis=1)

    lane = lax.broadcasted_iota(jnp.int32, (H, 128), 1)
    edge = lane < 2
    scale = DH ** -0.5

    def kv_rows(j, w, off, d):
        if j >= w:
            return qkvT[j - w, D + off + d * H:D + off + (d + 1) * H, :]
        return kvr[j - w + (W - 1), off + d * H:off + (d + 1) * H, :]

    def attn_block(j):
        acc = [None] * W
        for d in range(DH):
            qd = qkvT[j, d * H:(d + 1) * H, :]
            for w in range(W):
                t = qd * kv_rows(j, w, 0, d)
                acc[w] = t if acc[w] is None else acc[w] + t
        lg = []
        for w in range(W):
            l = acc[w] * scale
            if w > j:
                l = jnp.where(edge, -1e9, l)
            lg.append(l)
        m = lg[0]
        for w in range(1, W):
            m = jnp.maximum(m, lg[w])
        e = [jnp.exp(l - m) for l in lg]
        ssum = e[0]
        for w in range(1, W):
            ssum = ssum + e[w]
        inv = 1.0 / ssum
        a = [ew * inv for ew in e]
        for d in range(DH):
            o = a[0] * kv_rows(j, 0, D, d)
            for w in range(1, W):
                o = o + a[w] * kv_rows(j, w, D, d)
            oT[j % 2, d * H:(d + 1) * H, :] = o.astype(bf16)
        ot = oT[j % 2].T
        for t in range(4):
            o_u[t, pl.ds(j, 64, stride=NB), :] = pltpu.bitcast(ot[:, t * 128:(t + 1) * 128], u32)

    def gelu_block(i, n):
        g_v[:, i * n:(i + 1) * n] = jax.nn.gelu(u_acc[:, i * n:(i + 1) * n], approximate=True).astype(bf16)

    for b in range(2):
        oT[b, D:DP, :] = jnp.zeros((DP - D, 128), bf16)

    order = list(range(9, 16)) + list(range(0, 9))
    for t, j in enumerate(order):
        qkv_block(j)
        if t < 7:
            gelu_block(t, 256)
        elif t >= 8:
            attn_block(order[t - 1])

    cp_w2.wait()
    rest = list(range(8, 16))
    NPRE = 4
    for c in range(NPRE):
        r = c * OC
        u_acc[:, r:r + OC] = jnp.dot(g_v[...], w2_v[:, r:r + OC], preferred_element_type=f32)
        attn_block(rest[2 * c])
        attn_block(rest[2 * c + 1])

    def final(c, y):
        r = c * OC
        on = jnp.concatenate([pltpu.bitcast(o_u[t, r // 2:(r + OC) // 2, :], bf16) for t in range(4)], axis=1)
        ao = lax.dot_general(l_wo[...], on, NT, preferred_element_type=f32)
        out_v[:, r:r + OC] = (x_v[:, r:r + OC].astype(f32) + ao + (y + _row_bias(b2_ref, r, OC))).astype(bf16)
        cp_out(c).start()

    for c in range(NPRE):
        final(c, u_acc[:, c * OC:(c + 1) * OC])
    for c in range(NPRE, NOC):
        r = c * OC
        final(c, jnp.dot(g_v[...], w2_v[:, r:r + OC], preferred_element_type=f32))
    for c in range(NOC):
        cp_out(c).wait()


@jax.jit
def pallas_parallel_sum__sliding_local_dilated__mixer_token_mlp__prompt_kernel(
        A_x, A_wqkv, A_wo, B_x, B_w1, B_b1, B_w2, B_b2):
    any_spec = pl.BlockSpec(memory_space=pl.ANY)
    vmem_spec = pl.BlockSpec(memory_space=pltpu.VMEM)
    outT = pl.pallas_call(
        _kernel,
        out_shape=jax.ShapeDtypeStruct((1, D, S), bf16),
        in_specs=[any_spec, any_spec, any_spec, any_spec, vmem_spec, any_spec, vmem_spec],
        out_specs=any_spec,
        scratch_shapes=[
            pltpu.VMEM((D, S), bf16),
            pltpu.VMEM((D, 3 * D), bf16),
            pltpu.VMEM((D, D), bf16),
            pltpu.VMEM((S, F), bf16),
            pltpu.VMEM((F, S), bf16),
            pltpu.VMEM((D, S), bf16),
            pltpu.VMEM((4, S // 2, 128), u32),
            pltpu.VMEM((D, F), f32),
            pltpu.VMEM((D, F), bf16),
            pltpu.VMEM((4, 3 * D, 128), f32),
            pltpu.VMEM((3 * D, DP), bf16),
            pltpu.VMEM((D, DP), bf16),
            pltpu.VMEM((NB, 3 * D, 128), f32),
            pltpu.VMEM((W - 1, 2 * D, 128), f32),
            pltpu.VMEM((2, DP, 128), bf16),
            pltpu.VMEM((4, S // 2, 128), u32),
            pltpu.VMEM((D, S), bf16),
            pltpu.SemaphoreType.DMA((NXC,)),
            pltpu.SemaphoreType.DMA((NXC,)),
            pltpu.SemaphoreType.DMA((3,)),
            pltpu.SemaphoreType.DMA((NOC,)),
        ],
        compiler_params=pltpu.CompilerParams(vmem_limit_bytes=100 * 2**20),
    )(jnp.swapaxes(A_x, 1, 2), A_wqkv, A_wo, B_w1, B_b1.reshape(F // 128, 128), B_w2, B_b2.reshape(S // 128, 128))
    return jnp.swapaxes(outT, 1, 2)
```

```python
import jax
import jax.numpy as jnp
from jax import lax
import jax.experimental.pallas as pl
import jax.experimental.pallas.tpu as pltpu

S, D, F = 2048, 448, 1792
H, DH, W = 16, 28, 8
NB = 16
EPS = 1e-5
DP = 512
KT = DP // 128
NF = F // 128
PJ, PL = 132, 2
PROWS = PJ * NB
NG = 11
LOG2E = 1.4426950408889634
bf16, f32, u32 = jnp.bfloat16, jnp.float32, jnp.uint32
NT = (((1,), (1,)), ((), ()))
SCOPES = "0" == "1"
PVSTYLE = "grp2"
G8AT = int("6")
NPRE = int("9")
NOCHK = "1" == "1"
OUTC = (0, 2, 4, 6, 8, 10, 12, 14, 15, 16)


def _wait(cps, name):
    if SCOPES:
        with jax.named_scope("wait_" + name):
            for cp in cps:
                cp.wait()
    else:
        for cp in cps:
            cp.wait()


def _cat(parts, axis=1):
    return parts[0] if len(parts) == 1 else jnp.concatenate(parts, axis=axis)


def _pk(x):
    return pltpu.bitcast(x, u32)


def _upk(x):
    return pltpu.bitcast(x, bf16)


def _tcols(t, n=1):
    if isinstance(t, int):
        return pl.ds(t * 128, n * 128)
    return pl.ds(pl.multiple_of(t * 128, 128), n * 128)


def _tree(op, xs):
    xs = list(xs)
    while len(xs) > 1:
        xs = [op(xs[i], xs[i + 1]) for i in range(0, len(xs), 2)]
    return xs[0]


class _Acc:
    def __init__(self, n=2):
        self.p = [None] * n
        self.i = 0

    def add(self, v):
        k = self.i % len(self.p)
        self.p[k] = v if self.p[k] is None else self.p[k] + v
        self.i += 1

    def mean(self):
        t = self.p[0]
        for q in self.p[1:]:
            t = t + q
        return jnp.sum(t, axis=0, keepdims=True) * (1.0 / D)


def _kernel(x_hbm, wqkv_hbm, wo_hbm, w1_hbm, b1_hbm, w2_hbm, b2_hbm, out_hbm,
            x_v, wqkv_v, wo_v, w1_v, w2_v, b1_v, b2_v, hT, xnT, xn_u, u_acc, g_v, wtmp, l_qkv, l_wo,
            o_u, y_v, out_v, sems, *blk):
    qkvT = blk[0:NB]
    kvr = blk[NB:NB + W - 1]

    def cp_x(t, n, sem):
        return pltpu.make_async_copy(x_hbm.at[0, :, _tcols(t, n)], x_v.at[:, _tcols(t, n)], sem)

    def cp_w1(t, n, sem):
        return pltpu.make_async_copy(w1_hbm.at[_tcols(t, n), :], w1_v.at[_tcols(t, n), :], sem)

    def group_a(i):
        sem = sems.at[1 + i]
        return [cp_x(1 + i, 1, sem), cp_w1(i, 1, sem)]

    def group_bx(i):
        return cp_x(7 + 3 * i, 3, sems.at[5 + i])

    def group_bw(i):
        return cp_w1(4 + 2 * i, 2, sems.at[5 + i])

    def group(g):
        sem = sems.at[g]
        if g == 0:
            return [cp_x(0, 1, sem)]
        if g < 4:
            return group_a(g - 1)
        if g == 4:
            return [cp_x(4, 3, sem), cp_w1(3, 1, sem)]
        if g < 8:
            return [group_bx(g - 5), group_bw(g - 5)]
        if g == 8:
            return [group_bw(3)]
        if g == 9:
            return [cp_w1(12, 4, sem), pltpu.make_async_copy(wqkv_hbm, wqkv_v, sem),
                    pltpu.make_async_copy(b1_hbm, b1_v, sem)]
        return [pltpu.make_async_copy(wo_hbm, wo_v, sem), pltpu.make_async_copy(b2_hbm, b2_v, sem),
                pltpu.make_async_copy(w2_hbm, w2_v, sem)]

    def start(gs):
        for g in gs:
            for cp in group(g):
                cp.start()

    def cp_out(t, n):
        return pltpu.make_async_copy(out_v.at[:, _tcols(t, n)], out_hbm.at[0, :, _tcols(t, n)], sems.at[0])

    start([0, 1, 2])
    u_acc[...] = jnp.zeros((D, F), f32)
    _wait(group(0), "g0")
    never = x_v[0:H, 0:128].astype(f32) > jnp.inf
    zi = jnp.max(jnp.where(never, 16, 0).astype(jnp.int32))
    zs = [pl.multiple_of(zi * (i + 1), 16) for i in range(4)]

    def tie(x, dep):
        return x if dep is None else jnp.where(never, dep, x)

    def rows16(v, d):
        return v[d * H:(d + 1) * H, :]

    def ln_tiles(ts, pts=None):
        nt = len(ts)
        zz = zs if pts is not None else [0, 0, 0, 0]
        seg = 0 if pts is None else int(len(pts) * 0.85) // 4

        def dep(p, d, i):
            return None if pts is None else pts[p * seg + ((d * nt + i) * (seg - 8)) // (DH * nt)]

        def xrow(p, d, i):
            return tie(x_v[pl.ds(zz[p] + d * H, H), _tcols(ts[i])].astype(f32), dep(p, d, i))
        a = [_Acc() for _ in ts]
        for d in range(DH):
            for i in range(nt):
                a[i].add(xrow(0, d, i))
        m = [q.mean() for q in a]
        a = [_Acc() for _ in ts]
        for d in range(DH):
            for i in range(nt):
                c = xrow(1, d, i) - m[i]
                a[i].add(c * c)
        r = [lax.rsqrt(q.mean() + EPS) for q in a]
        a = [_Acc() for _ in ts]
        b = [_Acc() for _ in ts]
        rows = [[] for _ in ts]
        for d in range(DH):
            for i in range(nt):
                xn = ((xrow(2, d, i) - m[i]) * r[i]).astype(bf16)
                xnT[i, d * 8:(d + 1) * 8, :] = _pk(xn)
                rows[i].append(xn)
                xf = xn.astype(f32)
                a[i].add(xf)
                b[i].add(xf * xf)
        m2 = [q.mean() for q in a]
        r2 = [lax.rsqrt(jnp.maximum(q.mean() - mm * mm, 0.0) + EPS) for q, mm in zip(b, m2)]
        for d in range(DH):
            for i in range(nt):
                xf = tie(_upk(xnT[i, pl.ds(zz[3] + d * 8, 8), :]).astype(f32), dep(3, d, i))
                hT[ts[i], d * 8:(d + 1) * 8, :] = _pk(((xf - m2[i]) * r2[i]).astype(bf16))
        for i in range(nt):
            xn = jnp.concatenate(rows[i] + [jnp.zeros((DP - D, 128), bf16)], axis=0).T
            for k in range(KT):
                xu = _pk(xn[:, k * 128:(k + 1) * 128])
                for q in range(4):
                    xn_u[k, pl.ds(PL * (ts[i] * 4 + q), NB, stride=PJ), :] = xu[q * NB:(q + 1) * NB, :]

    def prep_wqkv():
        wt = jnp.concatenate([wqkv_v[...], jnp.zeros((DP - D, 3 * D), bf16)], axis=0).T.astype(f32)
        for k in range(KT):
            wtmp[k] = wt[:, k * 128:(k + 1) * 128]
        for p in range(3):
            for d in range(DH):
                r = (p * D + d * H) // 2
                l_qkv[r:r + H // 2, :] = _pk(_cat(
                    [wtmp[k, pl.ds(p * D + d, H, stride=DH), :] for k in range(KT)]).astype(bf16))

    def prep_wo():
        wo = jnp.concatenate([wo_v[...].astype(f32), jnp.zeros((D, DP - D), f32)], axis=1)
        for k in range(KT):
            wtmp[k, 0:D, :] = wo[:, k * 128:(k + 1) * 128]
        parts = []
        for k in range(KT):
            rows = [wtmp[k, pl.ds(d, H, stride=DH), :].astype(bf16) for d in range(DH)]
            rows.append(jnp.zeros((DP - D, 128), bf16))
            parts.append(jnp.concatenate(rows, axis=0))
        l_wo[...] = _pk(jnp.concatenate(parts, axis=1).T[0:D, :])

    def pace_points(part, kt):
        par = 4 // kt
        pts = []
        for n0 in range(0, NF, par):
            for d in range(DH):
                for n in range(n0, min(n0 + par, NF)):
                    pts.append(part[d * H:(d + 1) * H, n * 128:(n + 1) * 128])
        return pts

    def mix1(t, kt):
        lhs = _upk(_cat([hT[t + k] for k in range(kt)]))
        if kt > 1:
            return jnp.dot(lhs, w1_v[_tcols(t, kt), :], preferred_element_type=f32)
        main = jnp.dot(lhs, w1_v[_tcols(t), 0:12 * 128], preferred_element_type=f32)
        wl = w1_v[_tcols(t), 12 * 128:]
        tail = [jnp.dot(lhs[h * (D // 2):(h + 1) * (D // 2), :], wl, preferred_element_type=f32) for h in range(2)]
        return jnp.concatenate([main, jnp.concatenate(tail, axis=0)], axis=1)

    ln_tiles([0])
    start(range(3, NG))

    def step_a(i, carry):
        _wait(group_a(i), "ga")
        part = mix1(i, 1)
        u_acc[...] += part
        ln_tiles([i + 1], pace_points(part, 1))
        return carry

    lax.fori_loop(0, 3, step_a, 0)
    _wait(group(4), "g4")
    part = mix1(3, 1)
    u_acc[...] += part
    ln_tiles([4, 5], pace_points(part, 1))

    def step_b(i, carry):
        @pl.when(i < 3)
        def _():
            group_bx(i).wait()
        _wait([group_bw(i)], "gb")
        part = mix1(4 + 2 * i, 2)
        u_acc[...] += part
        t0 = jnp.minimum(6 + 3 * i, NB - 3)
        ln_tiles([t0 + q for q in range(3)], pace_points(part, 2))
        return carry

    lax.fori_loop(0, 4, step_b, 0)
    _wait(group(9), "g9")
    part = mix1(12, 4)
    prep_wqkv()
    b1 = b1_v[...].astype(f32)
    for n in range(NF):
        u = u_acc[:, n * 128:(n + 1) * 128] + part[:, n * 128:(n + 1) * 128] + b1[n:n + 1, :]
        g_v[:, n * 128:(n + 1) * 128] = _pk(jax.nn.gelu(u, approximate=True).astype(bf16))

    def qkv_block(j):
        rj = _cat([_upk(xn_u[k, pl.ds(PJ * j, 64, stride=PL), :]) for k in range(KT)])
        res = lax.dot_general(_upk(l_qkv[...]), rj, NT, preferred_element_type=f32)
        qkvT[j][pl.ds(zs[0], 3 * D), :] = res
        if j >= NB - (W - 1):
            kvr[j - (NB - (W - 1))][pl.ds(zs[0], 2 * D), :] = pltpu.roll(res[D:, :], 2, axis=1)
        return res

    edge = lax.broadcasted_iota(jnp.int32, (H, 128), 1) < 2
    scale = DH ** -0.5

    def attn_block(j, dep_qk, dep_pv):
        def kv_rows(w, off, d):
            if j >= w:
                return qkvT[j - w][pl.ds(D + off + d * H, H), :]
            return kvr[j - w + (W - 1)][pl.ds(off + d * H, H), :]

        acc = [None] * W
        for d in range(DH):
            qd = tie(qkvT[j][pl.ds(d * H, H), :], rows16(dep_qk, d))
            for w in range(W):
                t = qd * kv_rows(w, 0, d)
                acc[w] = t if acc[w] is None else acc[w] + t
        lg = [jnp.where(edge, -1e9 / scale, acc[w]) if w > j else acc[w] for w in range(W)]
        m = _tree(jnp.maximum, lg)
        e = [jnp.exp2((l - m) * (scale * LOG2E)) for l in lg]
        ssum = _tree(jnp.add, e)
        inv = pl.reciprocal(ssum, approx=True)
        inv = inv * (2.0 - ssum * inv)
        a = [ew * inv for ew in e]
        at = a
        rows = []
        for d in range(DH):
            if PVSTYLE == "grp2" and d % 2 == 0:
                at = [tie(aw, rows16(dep_pv, d)) for aw in a]
            o = at[0] * kv_rows(0, D, d)
            for w in range(1, W):
                o = o + at[w] * kv_rows(w, D, d)
            if PVSTYLE == "last":
                o = tie(o, rows16(dep_pv, d))
            rows.append(o.astype(bf16))
        rows.append(jnp.zeros((DP - D, 128), bf16))
        ot = jnp.concatenate(rows, axis=0).T
        for k in range(KT):
            o_u[k, pl.ds(PJ * j, 64, stride=PL), :] = _pk(ot[:, k * 128:(k + 1) * 128])

    def last_wait(i, carry):
        _wait(group(10), "g10")
        return carry

    order = list(range(9, 16)) + list(range(0, 9))
    for t, j in enumerate(order):
        res = qkv_block(j)
        if t >= 8:
            attn_block(order[t - 1], res[0:D, :], res[2 * D:3 * D, :])
        if t == G8AT:
            lax.fori_loop(0, 1 + zi, last_wait, 0)
            prep_wo()

    KS = (0, 4, 8, 12, 14)
    b2 = b2_v[...].astype(f32)

    def mix2_tile(n):
        ps = []
        accp = None
        for a, b in zip(KS[:-1], KS[1:]):
            p = jnp.dot(_upk(g_v[:, a * 128:b * 128]), w2_v[a * 128:b * 128, _tcols(n)],
                        preferred_element_type=f32)
            accp = p if accp is None else accp + p
            ps.append(accp)
        return ps

    def final_tile(n, y):
        on = _cat([_upk(_cat([o_u[k, pl.ds(PL * (n * 4 + i), NB, stride=PJ), :] for i in range(4)], axis=0))
                   for k in range(KT)])
        ao = lax.dot_general(_upk(l_wo[...]), on, NT, preferred_element_type=f32)
        out_v[:, _tcols(n)] = (x_v[:, _tcols(n)].astype(f32) + ao + (y + b2[n:n + 1, :])).astype(bf16)
        if n + 1 in OUTC:
            t0 = OUTC[OUTC.index(n + 1) - 1]
            cp_out(t0, n + 1 - t0).start()

    for n in range(NPRE):
        ps = mix2_tile(n)
        y_v[n] = ps[-1]
        if n < 8:
            attn_block(8 + n, ps[0], ps[2])
    for n in range(NPRE):
        final_tile(n, y_v[n])
    for n in range(NPRE, NB):
        final_tile(n, mix2_tile(n)[-1])
    _wait([pltpu.make_async_copy(out_v, out_hbm.at[0], sems.at[0])], "out")


@jax.jit
def pallas_parallel_sum__sliding_local_dilated__mixer_token_mlp__prompt_kernel(
        A_x, A_wqkv, A_wo, B_x, B_w1, B_b1, B_w2, B_b2):
    any_spec = pl.BlockSpec(memory_space=pl.ANY)
    outT = pl.pallas_call(
        _kernel,
        out_shape=jax.ShapeDtypeStruct((1, D, S), bf16),
        in_specs=[any_spec] * 7,
        out_specs=any_spec,
        scratch_shapes=[
            pltpu.VMEM((D, S), bf16),
            pltpu.VMEM((D, 3 * D), bf16),
            pltpu.VMEM((D, D), bf16),
            pltpu.VMEM((S, F), bf16),
            pltpu.VMEM((F, S), bf16),
            pltpu.VMEM((NF, 128), bf16),
            pltpu.VMEM((NB, 128), bf16),
            pltpu.VMEM((NB, D // 2, 128), u32),
            pltpu.VMEM((3, D // 2, 128), u32),
            pltpu.VMEM((KT, PROWS, 128), u32),
            pltpu.VMEM((D, F), f32),
            pltpu.VMEM((D // 2, F), u32),
            pltpu.VMEM((KT, 3 * D, 128), f32),
            pltpu.VMEM((3 * D // 2, DP), u32),
            pltpu.VMEM((D // 2, DP), u32),
            pltpu.VMEM((KT, PROWS, 128), u32),
            pltpu.VMEM((NB, D, 128), f32),
            pltpu.VMEM((D, S), bf16),
            pltpu.SemaphoreType.DMA((NG,)),
        ] + [pltpu.VMEM((3 * D, 128), f32)] * NB + [pltpu.VMEM((2 * D, 128), f32)] * (W - 1),
        compiler_params=pltpu.CompilerParams(vmem_limit_bytes=100 * 2**20, disable_semaphore_checks=NOCHK),
    )(jnp.swapaxes(A_x, 1, 2), A_wqkv, A_wo, B_w1, B_b1.reshape(NF, 128), B_w2, B_b2.reshape(NB, 128))
    return jnp.swapaxes(outT, 1, 2)
```

```python
import jax
import jax.numpy as jnp
from jax import lax
import jax.experimental.pallas as pl
import jax.experimental.pallas.tpu as pltpu

S, D, F = 2048, 448, 1792
H, DH, W = 16, 28, 8
NB = 16
EPS = 1e-5
DP = 512
KT = DP // 128
NF = F // 128
PJ, PL = 132, 2
PROWS = PJ * NB
NG = 12
N0 = int("6")
LOG2E = 1.4426950408889634
bf16, f32, u32 = jnp.bfloat16, jnp.float32, jnp.uint32
NT = (((1,), (1,)), ((), ()))
SCOPES = "0" == "1"
PVSTYLE = "last"
G8AT = int("6")
NPRE = int("9")
CHAIN = "none"
SMSTYLE = "b"
SM3 = "0" == "1"
NOCHK = "1" == "1"
OUTC = (0, 2, 4, 6, 8, 10, 12, 14, 15)
LASTR = (0, 224, 352, 416, 448)


def _wait(cps, name):
    if SCOPES:
        with jax.named_scope("wait_" + name):
            for cp in cps:
                cp.wait()
    else:
        for cp in cps:
            cp.wait()


def _cat(parts, axis=1):
    return parts[0] if len(parts) == 1 else jnp.concatenate(parts, axis=axis)


def _pk(x):
    return pltpu.bitcast(x, u32)


def _upk(x):
    return pltpu.bitcast(x, bf16)


def _tcols(t, n=1):
    if isinstance(t, int):
        return pl.ds(t * 128, n * 128)
    return pl.ds(pl.multiple_of(t * 128, 128), n * 128)


def _tree(op, xs):
    xs = list(xs)
    while len(xs) > 1:
        xs = [op(xs[i], xs[i + 1]) for i in range(0, len(xs), 2)]
    return xs[0]


class _Acc:
    def __init__(self, n=2):
        self.p = [None] * n
        self.i = 0

    def add(self, v):
        k = self.i % len(self.p)
        self.p[k] = v if self.p[k] is None else self.p[k] + v
        self.i += 1

    def mean(self):
        t = self.p[0]
        for q in self.p[1:]:
            t = t + q
        return jnp.sum(t, axis=0, keepdims=True) * (1.0 / D)


def _kernel(x_hbm, wqkv_hbm, wo_hbm, w1_hbm, b1_hbm, w2_hbm, b2_hbm, out_hbm,
            x_v, wqkv_v, wo_v, w1_v, w2_v, b1_v, b2_v, hT, xnT, xn_u, u_acc, g_v, wtmp, l_qkv, l_wo,
            o_u, y_v, out_v, sems, *blk):
    qkvT = blk[0:NB]
    kvr = blk[NB:NB + W - 1]
    oT = blk[NB + W - 1:]

    def cp_x(t, n, sem):
        return [pltpu.make_async_copy(x_hbm.at[0, :, _tcols(t + q)], x_v.at[t + q], sem) for q in range(n)]

    def cp_w1(t, n, sem):
        return pltpu.make_async_copy(w1_hbm.at[_tcols(t, n), :], w1_v.at[_tcols(t, n), :], sem)

    def group_a(i):
        sem = sems.at[2 + i]
        return cp_x(1 + i, 1, sem) + [cp_w1(i, 1, sem)]

    def group_bx(i):
        return cp_x(7 + 3 * i, 3, sems.at[6 + i])

    def group_bw(i):
        return cp_w1(4 + 2 * i, 2, sems.at[6 + i])

    def group(g):
        sem = sems.at[g]
        if g == 0:
            return cp_x(0, 1, sem)
        if g == 1:
            return [pltpu.make_async_copy(w1_hbm.at[0:128, 0:N0 * 128], w1_v.at[0:128, 0:N0 * 128], sem)]
        if g == 2:
            return cp_x(1, 1, sem) + [
                pltpu.make_async_copy(w1_hbm.at[0:128, N0 * 128:], w1_v.at[0:128, N0 * 128:], sem)]
        if g < 5:
            return group_a(g - 2)
        if g == 5:
            return cp_x(4, 3, sem) + [cp_w1(3, 1, sem)]
        if g < 9:
            return group_bx(g - 6) + [group_bw(g - 6)]
        if g == 9:
            return [group_bw(3)]
        if g == 10:
            return [cp_w1(12, 4, sem), pltpu.make_async_copy(wqkv_hbm, wqkv_v, sem),
                    pltpu.make_async_copy(b1_hbm, b1_v, sem)]
        return [pltpu.make_async_copy(wo_hbm, wo_v, sem), pltpu.make_async_copy(b2_hbm, b2_v, sem),
                pltpu.make_async_copy(w2_hbm, w2_v, sem)]

    def start(gs):
        for g in gs:
            for cp in group(g):
                cp.start()

    def cp_out(t, n):
        return pltpu.make_async_copy(out_v.at[:, _tcols(t, n)], out_hbm.at[0, :, _tcols(t, n)], sems.at[0])

    start(range(4))
    _wait(group(0), "g0")
    never = x_v[0, 0:H, :].astype(f32) > jnp.inf
    never8 = never[0:8, :]
    zs = []

    def tie(x, dep):
        return x if dep is None else jnp.where(never, dep, x)

    def rows16(v, d):
        return v[d * H:(d + 1) * H, :]

    def pack2(lo, hi):
        return pltpu.bitcast(pltpu.pack_elementwise([lo, hi], packed_dtype=bf16), u32)

    def unpack2(w, dep=None):
        v = jnp.concatenate([pltpu.unpack_elementwise(w, index=k, packed_dtype=bf16, unpacked_dtype=f32)
                             for k in range(2)], axis=0)
        return tie(v, dep)

    def xn_transpose(t, rows):
        xn = _upk(jnp.concatenate(rows + [jnp.zeros(((DP - D) // 2, 128), u32)], axis=0)).T
        for k in range(KT):
            xu = _pk(xn[:, k * 128:(k + 1) * 128])
            for q in range(4):
                xn_u[k, pl.ds(PL * (t * 4 + q), NB, stride=PJ), :] = xu[q * NB:(q + 1) * NB, :]

    def ln_tiles(ts, pts=None, slot=0, transpose=True):
        nt = len(ts)
        zz = zs if pts is not None else [0, 0, 0, 0]
        seg = 0 if pts is None else int(len(pts) * 0.85) // 4
        nch = 2 if pts is not None else 4

        def dep(p, d, i):
            return None if pts is None else pts[p * seg + ((d * nt + i) * (seg - 8)) // (DH * nt)]

        def xld(p, d, i):
            return x_v[ts[i], pl.ds(zz[p] + d * H, H), :]

        def xrow(p, d, i):
            if pts is None or p == 2:
                return unpack2(_pk(xld(p, d, i)), dep(p, d, i))
            return tie(xld(p, d, i).astype(f32), dep(p, d, i))
        a = [_Acc(nch) for _ in ts]
        for d in range(DH):
            for i in range(nt):
                a[i].add(xrow(0, d, i))
        m = [q.mean() for q in a]
        a = [_Acc(nch) for _ in ts]
        for d in range(DH):
            for i in range(nt):
                c = xrow(1, d, i) - m[i]
                a[i].add(c * c)
        r = [lax.rsqrt(q.mean() + EPS) for q in a]
        a = [_Acc(nch) for _ in ts]
        b = [_Acc(nch) for _ in ts]
        rows = [[] for _ in ts]
        for d in range(DH):
            for i in range(nt):
                xn = (xrow(2, d, i) - m[i]) * r[i]
                xu = pack2(xn[0:8], xn[8:16])
                xnT[slot + i, d * 8:(d + 1) * 8, :] = xu
                rows[i].append(xu)
                xf = unpack2(xu)
                a[i].add(xf)
                b[i].add(xf * xf)
        m2 = [q.mean() for q in a]
        r2 = [lax.rsqrt(jnp.maximum(q.mean() - mm * mm, 0.0) + EPS) for q, mm in zip(b, m2)]
        for d in range(DH):
            for i in range(nt):
                h = (unpack2(xnT[slot + i, pl.ds(zz[3] + d * 8, 8), :], dep(3, d, i)) - m2[i]) * r2[i]
                hT[ts[i], d * 8:(d + 1) * 8, :] = pack2(h[0:8], h[8:16])
        if transpose:
            for i in range(nt):
                xn_transpose(ts[i], rows[i])

    def prep_wqkv():
        wt = jnp.concatenate([wqkv_v[...], jnp.zeros((DP - D, 3 * D), bf16)], axis=0).T.astype(f32)
        for k in range(KT):
            wtmp[k] = wt[:, k * 128:(k + 1) * 128]
        for p in range(3):
            for d in range(DH):
                r = (((p + 2) % 3) * D + d * H) // 2
                l_qkv[r:r + H // 2, :] = _pk(_cat(
                    [wtmp[k, pl.ds(p * D + d, H, stride=DH), :] for k in range(KT)]).astype(bf16))

    def prep_wo():
        wo = jnp.concatenate([wo_v[...].astype(f32), jnp.zeros((D, DP - D), f32)], axis=1)
        for k in range(KT):
            wtmp[k, 0:D, :] = wo[:, k * 128:(k + 1) * 128]
        parts = []
        for k in range(KT):
            rows = [pack2(wtmp[k, pl.ds(d, 8, stride=DH), :], wtmp[k, pl.ds(8 * DH + d, 8, stride=DH), :])
                    for d in range(DH)]
            rows.append(jnp.zeros(((DP - D) // 2, 128), u32))
            parts.append(jnp.concatenate(rows, axis=0))
        l_wo[...] = _pk(_upk(jnp.concatenate(parts, axis=1)).T[0:D, :])

    def pace_points(part, kt):
        par = 4 // kt
        nn = part.shape[1] // 128
        pts = []
        for n0 in range(0, nn, par):
            for d in range(DH):
                for n in range(n0, min(n0 + par, nn)):
                    pts.append(part[d * H:(d + 1) * H, n * 128:(n + 1) * 128])
        return pts

    def mix1(t, kt, n0=0, n1=NF):
        lhs = _upk(_cat([hT[t + k] for k in range(kt)]))
        if (kt * (n1 - n0)) % 4 == 0:
            return jnp.dot(lhs, w1_v[_tcols(t, kt), n0 * 128:n1 * 128], preferred_element_type=f32)
        main = jnp.dot(lhs, w1_v[_tcols(t), n0 * 128:(n1 - 2) * 128], preferred_element_type=f32)
        wl = w1_v[_tcols(t), (n1 - 2) * 128:n1 * 128]
        tail = [jnp.dot(lhs[h * (D // 2):(h + 1) * (D // 2), :], wl, preferred_element_type=f32) for h in range(2)]
        return jnp.concatenate([main, jnp.concatenate(tail, axis=0)], axis=1)

    ln_tiles([0], slot=3, transpose=False)
    start(range(4, NG))
    _wait(group(1), "g1")
    zi = jnp.where(never8, 64, 0).astype(jnp.int32)[0, 0]
    zs.extend(pl.multiple_of(zi * (i + 1), 64) for i in range(4))
    u_acc[:, 0:N0 * 128] = mix1(0, 1, 0, N0)
    xn_transpose(0, [xnT[3, d * 8:(d + 1) * 8, :] for d in range(DH)])
    _wait(group(2), "g2")
    part = mix1(0, 1, N0, NF)
    u_acc[:, N0 * 128:] = part
    ln_tiles([1], pace_points(part, 1))

    def step_a(i, carry):
        _wait(group_a(i), "ga")
        part = mix1(i, 1)
        u_acc[...] += part
        ln_tiles([i + 1], pace_points(part, 1))
        return carry

    lax.fori_loop(1, 3, step_a, 0)
    _wait(group(5), "g5")
    part = mix1(3, 1)
    u_acc[...] += part
    ln_tiles([4, 5], pace_points(part, 1))

    def step_b(i, carry):
        @pl.when(i < 3)
        def _():
            for cp in group_bx(i):
                cp.wait()
        _wait([group_bw(i)], "gb")
        part = mix1(4 + 2 * i, 2)
        u_acc[...] += part
        t0 = jnp.minimum(6 + 3 * i, NB - 3)
        ln_tiles([t0 + q for q in range(3)], pace_points(part, 2))
        return carry

    lax.fori_loop(0, 4, step_b, 0)
    _wait(group(10), "g10")
    part = mix1(12, 4)
    prep_wqkv()
    b1 = b1_v[...].astype(f32)
    for n in range(NF):
        u = u_acc[:, n * 128:(n + 1) * 128] + part[:, n * 128:(n + 1) * 128] + b1[n:n + 1, :]
        g_v[:, n * 128:(n + 1) * 128] = _pk(jax.nn.gelu(u, approximate=True).astype(bf16))

    def qkv_block(j):
        rj = _cat([_upk(xn_u[k, pl.ds(PJ * j, 64, stride=PL), :]) for k in range(KT)])
        res = lax.dot_general(_upk(l_qkv[...]), rj, NT, preferred_element_type=f32)
        qkvT[j][pl.ds(zs[0], 3 * D), :] = res
        if j >= NB - (W - 1):
            kvr[j - (NB - (W - 1))][pl.ds(zs[0], 2 * D), :] = pltpu.roll(res[0:2 * D, :], 2, axis=1)
        return res

    edge = lax.broadcasted_iota(jnp.int32, (H, 128), 1) < 2
    scale = DH ** -0.5

    def attn_block(j, dep_qk, dep_sm, dep_pv):
        def kv_rows(w, off, d):
            if j >= w:
                return qkvT[j - w][pl.ds(off + d * H, H), :]
            return kvr[j - w + (W - 1)][pl.ds(off + d * H, H), :]

        acc = [None] * W
        for d in range(DH):
            qd = tie(qkvT[j][pl.ds(2 * D + d * H, H), :], rows16(dep_qk, d))
            for w in range(W):
                t = qd * kv_rows(w, 0, d)
                acc[w] = t if acc[w] is None else acc[w] + t
        lg = [jnp.where(edge, -1e9 / scale, acc[w]) if w > j else acc[w] for w in range(W)]
        def sm(v, d):
            return v if dep_sm is None else tie(v, rows16(dep_sm, d))
        if SMSTYLE == "a":
            m = _tree(jnp.maximum, [sm(jnp.maximum(lg[2 * q], lg[2 * q + 1]), 1) for q in range(4)])
            e = [jnp.exp2((l - sm(m, 3 + w)) * (scale * LOG2E)) for w, l in enumerate(lg)]
            ssum = sm(_tree(jnp.add, e), 14)
            inv = sm(pl.reciprocal(ssum, approx=True), 16)
            inv = sm(inv * (2.0 - ssum * inv), 18)
        else:
            m = sm(_tree(jnp.maximum, lg), 2)
            e = [jnp.exp2(sm((l - m) * (scale * LOG2E), 4 + 2 * (w // 2))) for w, l in enumerate(lg)]
            ssum = sm(_tree(jnp.add, e), 14)
            inv = pl.reciprocal(ssum, approx=True)
            inv = sm(inv * (2.0 - ssum * inv), 18)
        a = [ew * inv for ew in e]
        at = a
        for d in range(DH):
            if PVSTYLE.startswith("grp") and d % int(PVSTYLE[3:]) == 0:
                at = [tie(aw, rows16(dep_pv, d)) for aw in a]
            v0 = kv_rows(0, D, d)
            if PVSTYLE == "first":
                v0 = tie(v0, rows16(dep_pv, d))
            o = at[0] * v0
            for w in range(1, W):
                o = o + at[w] * kv_rows(w, D, d)
            if PVSTYLE == "last":
                o = tie(o, rows16(dep_pv, d))
            oT[j][pl.ds(zs[0] + d * 8, 8), :] = pack2(o[0:8], o[8:16])

    def o_transpose(j):
        ot = _upk(jnp.concatenate([oT[j][...], jnp.zeros(((DP - D) // 2, 128), u32)], axis=0)).T
        for k in range(KT):
            o_u[k, pl.ds(PJ * j, 64, stride=PL), :] = _pk(ot[:, k * 128:(k + 1) * 128])

    def last_wait(i, carry):
        _wait(group(11), "g11")
        return carry

    order = list(range(9, 16)) + list(range(0, 9))
    for t, j in enumerate(order):
        res = qkv_block(j)
        if t >= 8:
            attn_block(order[t - 1], res[0:D, :], res[D:2 * D, :], res[2 * D:3 * D, :])
        if t == G8AT:
            lax.fori_loop(0, 1 + zi, last_wait, 0)
            prep_wo()

    KS = (0, 4, 8, 12, 14)
    b2 = b2_v[...].astype(f32)

    def mix2_tile(n):
        ps = []
        accp = None
        for a, b in zip(KS[:-1], KS[1:]):
            p = jnp.dot(_upk(g_v[:, a * 128:b * 128]), w2_v[a * 128:b * 128, _tcols(n)],
                        preferred_element_type=f32)
            accp = p if accp is None else accp + p
            ps.append(accp)
        return ps

    def final_tile(n, y):
        on = _cat([_upk(_cat([o_u[k, pl.ds(PL * (n * 4 + i), NB, stride=PJ), :] for i in range(4)], axis=0))
                   for k in range(KT)])
        ao = lax.dot_general(_upk(l_wo[...]), on, NT, preferred_element_type=f32)
        res = (x_v[n].astype(f32) + ao + (y + b2[n:n + 1, :])).astype(bf16)
        if n == NB - 1:
            for r0, r1 in zip(LASTR[:-1], LASTR[1:]):
                out_v[r0:r1, _tcols(n)] = res[r0:r1, :]
                pltpu.make_async_copy(out_v.at[r0:r1, _tcols(n)], out_hbm.at[0, r0:r1, _tcols(n)], sems.at[0]).start()
            return
        out_v[:, _tcols(n)] = res
        if n + 1 in OUTC:
            t0 = OUTC[OUTC.index(n + 1) - 1]
            cp_out(t0, n + 1 - t0).start()

    for n in range(NPRE):
        ps = mix2_tile(n)
        y_v[n] = ps[-1]
        if n < 8:
            attn_block(8 + n, ps[0], ps[1] if SM3 else None, ps[2])
    for j in range(NB):
        o_transpose(j)
    for n in range(NPRE):
        final_tile(n, y_v[n])
    for n in range(NPRE, NB):
        final_tile(n, mix2_tile(n)[-1])
    _wait([pltpu.make_async_copy(out_v, out_hbm.at[0], sems.at[0])], "out")


@jax.jit
def pallas_parallel_sum__sliding_local_dilated__mixer_token_mlp__prompt_kernel(
        A_x, A_wqkv, A_wo, B_x, B_w1, B_b1, B_w2, B_b2):
    any_spec = pl.BlockSpec(memory_space=pl.ANY)
    outT = pl.pallas_call(
        _kernel,
        out_shape=jax.ShapeDtypeStruct((1, D, S), bf16),
        in_specs=[any_spec] * 7,
        out_specs=any_spec,
        scratch_shapes=[
            pltpu.VMEM((NB, D, 128), bf16),
            pltpu.VMEM((D, 3 * D), bf16),
            pltpu.VMEM((D, D), bf16),
            pltpu.VMEM((S, F), bf16),
            pltpu.VMEM((F, S), bf16),
            pltpu.VMEM((NF, 128), bf16),
            pltpu.VMEM((NB, 128), bf16),
            pltpu.VMEM((NB, D // 2, 128), u32),
            pltpu.VMEM((4, D // 2, 128), u32),
            pltpu.VMEM((KT, PROWS, 128), u32),
            pltpu.VMEM((D, F), f32),
            pltpu.VMEM((D // 2, F), u32),
            pltpu.VMEM((KT, 3 * D, 128), f32),
            pltpu.VMEM((3 * D // 2, DP), u32),
            pltpu.VMEM((D // 2, DP), u32),
            pltpu.VMEM((KT, PROWS, 128), u32),
            pltpu.VMEM((NB, D, 128), f32),
            pltpu.VMEM((D, S), bf16),
            pltpu.SemaphoreType.DMA((NG,)),
        ] + [pltpu.VMEM((3 * D, 128), f32)] * NB + [pltpu.VMEM((2 * D, 128), f32)] * (W - 1)
          + [pltpu.VMEM((D // 2, 128), u32)] * NB,
        compiler_params=pltpu.CompilerParams(vmem_limit_bytes=100 * 2**20, disable_semaphore_checks=NOCHK),
    )(jnp.swapaxes(A_x, 1, 2), A_wqkv, A_wo, B_w1, B_b1.reshape(NF, 128), B_w2, B_b2.reshape(NB, 128))
    return jnp.swapaxes(outT, 1, 2)
```

```python
import jax
import jax.numpy as jnp
from jax import lax
import jax.experimental.pallas as pl
import jax.experimental.pallas.tpu as pltpu

S, D, F = 2048, 448, 1792
H, DH, W = 16, 28, 8
EPS = 1e-5
LOG2E = 1.4426950408889634
NB = S // 128
NF = F // 128
DP = 512
KT = DP // 128
PJ, PL = 132, 2
PROWS = PJ * NB + 128
NG = 12
N0 = 6
WAIT_AT = 6
NPRE = 9
OUTC = (0, 2, 4, 6, 8, 10, 12, 14, 15)
LASTR = (0, 224, 352, 416, 448)
bf16, f32, u32 = jnp.bfloat16, jnp.float32, jnp.uint32
NT = (((1,), (1,)), ((), ()))


def _wait(cps):
    for cp in cps:
        cp.wait()


def _cat(parts, axis=1):
    return parts[0] if len(parts) == 1 else jnp.concatenate(parts, axis=axis)


def _pk(x):
    return pltpu.bitcast(x, u32)


def _upk(x):
    return pltpu.bitcast(x, bf16)


def _tiles(t, n=1):
    if isinstance(t, int):
        return pl.ds(t * 128, n * 128)
    return pl.ds(pl.multiple_of(t * 128, 128), n * 128)


def _tree(op, xs):
    xs = list(xs)
    while len(xs) > 1:
        xs = [op(xs[i], xs[i + 1]) for i in range(0, len(xs), 2)]
    return xs[0]


def _rows16(v, d):
    return v[d * H:(d + 1) * H, :]


class _Acc:
    def __init__(self, n):
        self.p = [None] * n
        self.i = 0

    def add(self, v):
        k = self.i % len(self.p)
        self.p[k] = v if self.p[k] is None else self.p[k] + v
        self.i += 1

    def mean(self):
        t = self.p[0]
        for q in self.p[1:]:
            t = t + q
        return jnp.sum(t, axis=0, keepdims=True) * (1.0 / D)


def _kernel(x_hbm, wqkv_hbm, wo_hbm, w1_hbm, b1_hbm, w2_hbm, b2_hbm, out_hbm,
            x_v, wqkv_v, wo_v, w1_v, w2_v, b1_v, b2_v, hT, xnT, xn_u, u_acc, g_v, wtmp, l_qkv, l_wo,
            o_u, y_v, out_v, sems, *blk):
    kvq = blk[0:NB]
    kvr = blk[NB:NB + W - 1]
    oT = blk[NB + W - 1:]

    def cp_x(t, n, sem):
        return [pltpu.make_async_copy(x_hbm.at[0, :, _tiles(t + q)], x_v.at[t + q], sem) for q in range(n)]

    def cp_w1(t, n, sem):
        return [pltpu.make_async_copy(w1_hbm.at[_tiles(t, n), :], w1_v.at[_tiles(t, n), :], sem)]

    def group_a(i):
        return cp_x(1 + i, 1, sems.at[2 + i]) + cp_w1(i, 1, sems.at[2 + i])

    def group_b(i):
        return cp_x(8 + 2 * i, 2, sems.at[6 + i]) + cp_w1(4 + 2 * i, 2, sems.at[6 + i])

    def group(g):
        sem = sems.at[g]
        if g == 0:
            return cp_x(0, 1, sem)
        if g == 1:
            return [pltpu.make_async_copy(w1_hbm.at[0:128, 0:N0 * 128], w1_v.at[0:128, 0:N0 * 128], sem)]
        if g == 2:
            return cp_x(1, 1, sem) + [
                pltpu.make_async_copy(w1_hbm.at[0:128, N0 * 128:], w1_v.at[0:128, N0 * 128:], sem)]
        if g < 5:
            return group_a(g - 2)
        if g == 5:
            return cp_x(4, 4, sem) + cp_w1(3, 1, sem)
        if g < 10:
            return group_b(g - 6)
        if g == 10:
            return cp_w1(12, 4, sem) + [pltpu.make_async_copy(wqkv_hbm, wqkv_v, sem),
                                        pltpu.make_async_copy(b1_hbm, b1_v, sem)]
        return [pltpu.make_async_copy(wo_hbm, wo_v, sem), pltpu.make_async_copy(b2_hbm, b2_v, sem),
                pltpu.make_async_copy(w2_hbm, w2_v, sem)]

    def start(gs):
        for g in gs:
            for cp in group(g):
                cp.start()

    start(range(4))
    _wait(group(0))
    never = x_v[0, 0:H, :].astype(f32) > jnp.inf

    def tie(x, dep):
        return x if dep is None else jnp.where(never, dep, x)

    def to_rows(dst, j, packed):
        t = _upk(jnp.concatenate([packed, jnp.zeros(((DP - D) // 2, 128), u32)], axis=0)).T
        for k in range(KT):
            dst(k, j, _pk(t[:, k * 128:(k + 1) * 128]))

    def put_xn(k, t, w):
        for q in range(4):
            xn_u[k, pl.ds(PL * (t * 4 + q), NB, stride=PJ), :] = w[q * NB:(q + 1) * NB, :]

    def put_o(k, j, w):
        o_u[k, pl.ds(PJ * j, 64, stride=PL), :] = w

    def ln_tiles(ts, pts=None, z=0, slot=0, transpose=True):
        nt = len(ts)
        seg = 0 if pts is None else int(len(pts) * 0.85) // 4
        nch = 2 if pts is not None else 4

        def dep(p, d, i):
            return None if pts is None else pts[p * seg + ((d * nt + i) * (seg - 8)) // (DH * nt)]

        def xrow(p, d, i):
            return tie(x_v[ts[i], d * H:(d + 1) * H, :].astype(f32), dep(p, d, i))

        a = [_Acc(nch) for _ in ts]
        for d in range(DH):
            for i in range(nt):
                a[i].add(xrow(0, d, i))
        m = [q.mean() for q in a]
        a = [_Acc(nch) for _ in ts]
        for d in range(DH):
            for i in range(nt):
                c = xrow(1, d, i) - m[i]
                a[i].add(c * c)
        r = [lax.rsqrt(q.mean() + EPS) for q in a]
        m = [q.astype(bf16).astype(f32) for q in m]
        a = [_Acc(nch) for _ in ts]
        b = [_Acc(nch) for _ in ts]
        rows = [[] for _ in ts]
        for d in range(DH):
            for i in range(nt):
                xu = _pk(((xrow(2, d, i) - m[i]) * r[i]).astype(bf16))
                xnT[slot + i, d * 8:(d + 1) * 8, :] = xu
                rows[i].append(xu)
                xf = _upk(xu).astype(f32)
                a[i].add(xf)
                b[i].add(xf * xf)
        m2 = [q.mean() for q in a]
        r2 = [lax.rsqrt(jnp.maximum(q.mean() - mm * mm, 0.0) + EPS) for q, mm in zip(b, m2)]
        m2 = [q.astype(bf16).astype(f32) for q in m2]
        for d in range(DH):
            for i in range(nt):
                xf = tie(_upk(xnT[slot + i, pl.ds(z + d * 8, 8), :]).astype(f32), dep(3, d, i))
                hT[ts[i], d * 8:(d + 1) * 8, :] = _pk(((xf - m2[i]) * r2[i]).astype(bf16))
        if transpose:
            for i in range(nt):
                to_rows(put_xn, ts[i], jnp.concatenate(rows[i], axis=0))

    def prep_wqkv():
        wt = jnp.concatenate([wqkv_v[...], jnp.zeros((DP - D, 3 * D), bf16)], axis=0).T.astype(f32)
        for k in range(KT):
            wtmp[k, 0:3 * D, :] = wt[:, k * 128:(k + 1) * 128]
        for p in range(3):
            for d in range(DH):
                r = (((p + 2) % 3) * D + d * H) // 2
                l_qkv[r:r + H // 2, :] = _pk(_cat(
                    [wtmp[k, pl.ds(p * D + d, H, stride=DH), :] for k in range(KT)]).astype(bf16))

    def prep_wo():
        wo = jnp.concatenate([wo_v[...].astype(f32), jnp.zeros((D, DP - D), f32)], axis=1)
        for k in range(KT):
            wtmp[k, 0:D, :] = wo[:, k * 128:(k + 1) * 128]
        parts = []
        for k in range(KT):
            rows = [_pk(wtmp[k, pl.ds(d, H, stride=DH), :].astype(bf16)) for d in range(DH)]
            rows.append(jnp.zeros(((DP - D) // 2, 128), u32))
            parts.append(jnp.concatenate(rows, axis=0))
        l_wo[...] = _pk(_upk(jnp.concatenate(parts, axis=1)).T[0:D, :])

    def pace_points(part, kt):
        par = 4 // kt
        nn = part.shape[1] // 128
        return [part[d * H:(d + 1) * H, n * 128:(n + 1) * 128]
                for n0 in range(0, nn, par) for d in range(DH) for n in range(n0, min(n0 + par, nn))]

    def mix1(t, kt, n0=0, n1=NF):
        lhs = _upk(_cat([hT[t + k] for k in range(kt)]))
        if (kt * (n1 - n0)) % 4 == 0:
            return jnp.dot(lhs, w1_v[_tiles(t, kt), n0 * 128:n1 * 128], preferred_element_type=f32)
        main = jnp.dot(lhs, w1_v[_tiles(t), n0 * 128:(n1 - 2) * 128], preferred_element_type=f32)
        wl = w1_v[_tiles(t), (n1 - 2) * 128:n1 * 128]
        tail = [jnp.dot(lhs[h * (D // 2):(h + 1) * (D // 2), :], wl, preferred_element_type=f32)
                for h in range(2)]
        return jnp.concatenate([main, jnp.concatenate(tail, axis=0)], axis=1)

    ln_tiles([0], slot=3, transpose=False)
    start(range(4, NG))
    _wait(group(1))
    u_acc[:, 0:N0 * 128] = mix1(0, 1, 0, N0)
    to_rows(put_xn, 0, xnT[3])
    _wait(group(2))
    part = mix1(0, 1, N0, NF)
    u_acc[:, N0 * 128:] = part
    ln_tiles([1], pace_points(part, 1))

    def step_a(i, z):
        _wait(group_a(i))
        part = mix1(i, 1)
        u_acc[...] += part
        ln_tiles([i + 1], pace_points(part, 1), pl.multiple_of(z * 64, 64))
        return (i - 1) * (i - 2)

    zi = lax.fori_loop(1, 3, step_a, 0)
    z0 = pl.multiple_of(zi * 64, 64)
    _wait(group(5))
    part = mix1(3, 1)
    u_acc[...] += part
    ln_tiles([4, 5], pace_points(part, 1), z0)

    def step_b(i, carry):
        _wait(group_b(i))
        part = mix1(4 + 2 * i, 2)
        u_acc[...] += part
        t0 = jnp.minimum(6 + 3 * i, 7 + 2 * i)
        ln_tiles([t0 + q for q in range(3)], pace_points(part, 2), z0)
        return carry

    lax.fori_loop(0, 4, step_b, 0)
    _wait(group(10))
    part = mix1(12, 4)
    prep_wqkv()
    b1 = b1_v[...].astype(f32)
    for n in range(NF):
        u = u_acc[:, n * 128:(n + 1) * 128] + part[:, n * 128:(n + 1) * 128] + b1[n:n + 1, :]
        g_v[:, n * 128:(n + 1) * 128] = _pk(jax.nn.gelu(u, approximate=True).astype(bf16))

    def qkv_block(j):
        rj = _cat([_upk(xn_u[k, pl.ds(PJ * j, 64, stride=PL), :]) for k in range(KT)])
        res = lax.dot_general(_upk(l_qkv[...]), rj, NT, preferred_element_type=f32)
        kvq[j][pl.ds(z0, 3 * D), :] = res
        if j >= NB - (W - 1):
            kvr[j - (NB - (W - 1))][pl.ds(z0, 2 * D), :] = pltpu.roll(res[0:2 * D, :], 2, axis=1)
        return res

    edge = lax.broadcasted_iota(jnp.int32, (H, 128), 1) < 2
    scale = DH ** -0.5

    def attn_block(j, dep_qk, dep_sm, dep_pv):
        def kv_rows(w, off, d):
            if j >= w:
                return kvq[j - w][pl.ds(off + d * H, H), :]
            return kvr[j - w + (W - 1)][pl.ds(off + d * H, H), :]

        def sm(v, d):
            return v if dep_sm is None else tie(v, _rows16(dep_sm, d))

        acc = [None] * W
        for d in range(DH):
            qd = tie(kvq[j][pl.ds(2 * D + d * H, H), :], _rows16(dep_qk, d))
            for w in range(W):
                t = qd * kv_rows(w, 0, d)
                acc[w] = t if acc[w] is None else acc[w] + t
        lg = [jnp.where(edge, -1e9 / scale, acc[w]) if w > j else acc[w] for w in range(W)]
        m = sm(_tree(jnp.maximum, lg), 2)
        e = [jnp.exp2(sm((l - m) * (scale * LOG2E), 4 + 2 * (w // 2))) for w, l in enumerate(lg)]
        ssum = sm(_tree(jnp.add, e), 14)
        inv = pl.reciprocal(ssum, approx=True)
        inv = sm(inv * (2.0 - ssum * inv), 18)
        a = [ew * inv for ew in e]
        for d in range(DH):
            o = a[0] * kv_rows(0, D, d)
            for w in range(1, W):
                o = o + a[w] * kv_rows(w, D, d)
            oT[j][pl.ds(z0 + d * 8, 8), :] = _pk(tie(o, _rows16(dep_pv, d)).astype(bf16))

    def last_wait(i, carry):
        _wait(group(11))
        return carry

    order = list(range(NB - (W - 1), NB)) + list(range(NB - (W - 1)))
    for t, j in enumerate(order):
        res = qkv_block(j)
        if t >= W:
            attn_block(order[t - 1], res[0:D, :], res[D:2 * D, :], res[2 * D:3 * D, :])
        if t == WAIT_AT:
            lax.fori_loop(0, 1 + zi, last_wait, 0)
            prep_wo()

    ks = (0, 4, 8, 12, 14)
    b2 = b2_v[...].astype(f32)

    def mix2_tile(n):
        ps = []
        for a, b in zip(ks[:-1], ks[1:]):
            p = jnp.dot(_upk(g_v[:, a * 128:b * 128]), w2_v[a * 128:b * 128, _tiles(n)],
                        preferred_element_type=f32)
            ps.append(ps[-1] + p if ps else p)
        return ps

    def final_tile(n, y):
        on = _cat([_upk(_cat([o_u[k, pl.ds(PL * (n * 4 + i), NB, stride=PJ), :] for i in range(4)], axis=0))
                   for k in range(KT)])
        ao = lax.dot_general(_upk(l_wo[...]), on, NT, preferred_element_type=f32)
        res = (x_v[n].astype(f32) + ao + (y + b2[n:n + 1, :])).astype(bf16)
        if n == NB - 1:
            for r0, r1 in zip(LASTR[:-1], LASTR[1:]):
                out_v[r0:r1, _tiles(n)] = res[r0:r1, :]
                pltpu.make_async_copy(out_v.at[r0:r1, _tiles(n)], out_hbm.at[0, r0:r1, _tiles(n)],
                                      sems.at[0]).start()
            return
        out_v[:, _tiles(n)] = res
        if n + 1 in OUTC:
            t0 = OUTC[OUTC.index(n + 1) - 1]
            pltpu.make_async_copy(out_v.at[:, _tiles(t0, n + 1 - t0)], out_hbm.at[0, :, _tiles(t0, n + 1 - t0)],
                                  sems.at[0]).start()

    for n in range(NPRE):
        ps = mix2_tile(n)
        y_v[n] = ps[-1]
        if n < W:
            attn_block(NB - W + n, ps[0], None, ps[2])
    for j in range(NB):
        to_rows(put_o, j, oT[j][...])
    for n in range(NPRE):
        final_tile(n, y_v[n])
    for n in range(NPRE, NB):
        final_tile(n, mix2_tile(n)[-1])
    _wait([pltpu.make_async_copy(out_v, out_hbm.at[0], sems.at[0])])


@jax.jit
def pallas_parallel_sum__sliding_local_dilated__mixer_token_mlp__prompt_kernel(
        A_x, A_wqkv, A_wo, B_x, B_w1, B_b1, B_w2, B_b2):
    any_spec = pl.BlockSpec(memory_space=pl.ANY)
    out_t = pl.pallas_call(
        _kernel,
        out_shape=jax.ShapeDtypeStruct((1, D, S), bf16),
        in_specs=[any_spec] * 7,
        out_specs=any_spec,
        scratch_shapes=[
            pltpu.VMEM((NB, D, 128), bf16),
            pltpu.VMEM((D, 3 * D), bf16),
            pltpu.VMEM((D, D), bf16),
            pltpu.VMEM((S, F), bf16),
            pltpu.VMEM((F, S), bf16),
            pltpu.VMEM((NF, 128), bf16),
            pltpu.VMEM((NB, 128), bf16),
            pltpu.VMEM((NB, D // 2, 128), u32),
            pltpu.VMEM((4, D // 2, 128), u32),
            pltpu.VMEM((KT, PROWS, 128), u32),
            pltpu.VMEM((D, F), f32),
            pltpu.VMEM((D // 2, F), u32),
            pltpu.VMEM((KT, 3 * D + 32, 128), f32),
            pltpu.VMEM((3 * D // 2, DP), u32),
            pltpu.VMEM((D // 2, DP), u32),
            pltpu.VMEM((KT, PROWS, 128), u32),
            pltpu.VMEM((NPRE, D, 128), f32),
            pltpu.VMEM((D, S), bf16),
            pltpu.SemaphoreType.DMA((NG,)),
        ] + [pltpu.VMEM((3 * D, 128), f32)] * NB + [pltpu.VMEM((2 * D, 128), f32)] * (W - 1)
          + [pltpu.VMEM((D // 2, 128), u32)] * NB,
        compiler_params=pltpu.CompilerParams(vmem_limit_bytes=100 * 2**20, disable_semaphore_checks=True),
    )(jnp.swapaxes(A_x, 1, 2), A_wqkv, A_wo, B_w1, B_b1.reshape(NF, 128), B_w2, B_b2.reshape(NB, 128))
    return jnp.swapaxes(out_t, 1, 2)
```

```python
import jax
import jax.numpy as jnp
from jax import lax
import jax.experimental.pallas as pl
import jax.experimental.pallas.tpu as pltpu

S, D, F = 2048, 448, 1792
H, DH, W = 16, 28, 8
EPS = 1e-5
LOG2E = 1.4426950408889634
NB = S // 128
NF = F // 128
DP = 512
KT = DP // 128
PJ, PL = 132, 2
PROWS = PJ * NB + 128
NG = 12
N0 = 6
WAIT_AT = 6
NPRE = 9
OUTC = (0, 2, 4, 6, 8, 10, 12, 14, 15)
LASTR = (0, 224, 352, 416, 448)
bf16, f32, u32 = jnp.bfloat16, jnp.float32, jnp.uint32
NT = (((1,), (1,)), ((), ()))


def _wait(cps):
    for cp in cps:
        cp.wait()


def _cat(parts, axis=1):
    return parts[0] if len(parts) == 1 else jnp.concatenate(parts, axis=axis)


def _pk(x):
    return pltpu.bitcast(x, u32)


def _upk(x):
    return pltpu.bitcast(x, bf16)


def _tiles(t, n=1):
    if isinstance(t, int):
        return pl.ds(t * 128, n * 128)
    return pl.ds(pl.multiple_of(t * 128, 128), n * 128)


def _tree(op, xs):
    xs = list(xs)
    while len(xs) > 1:
        xs = [op(xs[i], xs[i + 1]) for i in range(0, len(xs), 2)]
    return xs[0]


def _rows16(v, d):
    return v[d * H:(d + 1) * H, :]


class _Acc:
    def __init__(self, n):
        self.p = [None] * n
        self.i = 0

    def add(self, v):
        k = self.i % len(self.p)
        self.p[k] = v if self.p[k] is None else self.p[k] + v
        self.i += 1

    def mean(self):
        t = self.p[0]
        for q in self.p[1:]:
            t = t + q
        return jnp.sum(t, axis=0, keepdims=True) * (1.0 / D)


def _kernel(x_hbm, wqkv_hbm, wo_hbm, w1_hbm, b1_hbm, w2_hbm, b2_hbm, out_hbm,
            x_v, wqkv_v, wo_v, w1_v, w2_v, b1_v, b2_v, hT, xnT, xn_u, u_acc, g_v, wtmp, l_qkv, l_wo,
            o_u, y_v, out_v, sems, *blk):
    kvq = blk[0:NB]
    kvr = blk[NB:NB + W - 1]
    oT = blk[NB + W - 1:]

    def cp_x(t, n, sem):
        return [pltpu.make_async_copy(x_hbm.at[0, :, _tiles(t + q)], x_v.at[t + q], sem) for q in range(n)]

    def cp_w1(t, n, sem):
        return [pltpu.make_async_copy(w1_hbm.at[_tiles(t, n), :], w1_v.at[_tiles(t, n), :], sem)]

    def group_a(i):
        return cp_x(1 + i, 1, sems.at[2 + i]) + cp_w1(i, 1, sems.at[2 + i])

    def group_b(i):
        return cp_x(8 + 2 * i, 2, sems.at[6 + i]) + cp_w1(4 + 2 * i, 2, sems.at[6 + i])

    def group(g):
        sem = sems.at[g]
        if g == 0:
            return cp_x(0, 1, sem)
        if g == 1:
            return [pltpu.make_async_copy(w1_hbm.at[0:128, 0:N0 * 128], w1_v.at[0:128, 0:N0 * 128], sem)]
        if g == 2:
            return cp_x(1, 1, sem) + [
                pltpu.make_async_copy(w1_hbm.at[0:128, N0 * 128:], w1_v.at[0:128, N0 * 128:], sem)]
        if g < 5:
            return group_a(g - 2)
        if g == 5:
            return cp_x(4, 4, sem) + cp_w1(3, 1, sem)
        if g < 10:
            return group_b(g - 6)
        if g == 10:
            return cp_w1(12, 4, sem) + [pltpu.make_async_copy(wqkv_hbm, wqkv_v, sem),
                                        pltpu.make_async_copy(b1_hbm, b1_v, sem)]
        return [pltpu.make_async_copy(wo_hbm, wo_v, sem), pltpu.make_async_copy(b2_hbm, b2_v, sem),
                pltpu.make_async_copy(w2_hbm, w2_v, sem)]

    def start(gs):
        for g in gs:
            for cp in group(g):
                cp.start()

    start(range(4))
    _wait(group(0))
    never = x_v[0, 0:H, :].astype(f32) > jnp.inf

    def tie(x, dep):
        return x if dep is None else jnp.where(never, dep, x)

    def to_rows(dst, j, packed):
        t = _upk(jnp.concatenate([packed, jnp.zeros(((DP - D) // 2, 128), u32)], axis=0)).T
        for k in range(KT):
            dst(k, j, _pk(t[:, k * 128:(k + 1) * 128]))

    def put_xn(k, t, w):
        for q in range(4):
            xn_u[k, pl.ds(PL * (t * 4 + q), NB, stride=PJ), :] = w[q * NB:(q + 1) * NB, :]

    def put_o(k, j, w):
        o_u[k, pl.ds(PJ * j, 64, stride=PL), :] = w

    def ln_tiles(ts, pts=None, z=0, slot=0, transpose=True):
        nt = len(ts)
        seg = 0 if pts is None else int(len(pts) * 0.85) // 4
        nch = 2 if pts is not None else 4

        def dep(p, d, i):
            return None if pts is None else pts[p * seg + ((d * nt + i) * (seg - 8)) // (DH * nt)]

        def xrow(p, d, i):
            return tie(x_v[ts[i], d * H:(d + 1) * H, :].astype(f32), dep(p, d, i))

        a = [_Acc(nch) for _ in ts]
        for d in range(DH):
            for i in range(nt):
                a[i].add(xrow(0, d, i))
        m = [q.mean() for q in a]
        a = [_Acc(nch) for _ in ts]
        for d in range(DH):
            for i in range(nt):
                c = xrow(1, d, i) - m[i]
                a[i].add(c * c)
        r = [lax.rsqrt(q.mean() + EPS) for q in a]
        m = [q.astype(bf16).astype(f32) for q in m]
        a = [_Acc(nch) for _ in ts]
        b = [_Acc(nch) for _ in ts]
        rows = [[] for _ in ts]
        for d in range(DH):
            for i in range(nt):
                xu = _pk(((xrow(2, d, i) - m[i]) * r[i]).astype(bf16))
                xnT[slot + i, d * 8:(d + 1) * 8, :] = xu
                rows[i].append(xu)
                xf = _upk(xu).astype(f32)
                a[i].add(xf)
                b[i].add(xf * xf)
        m2 = [q.mean() for q in a]
        r2 = [lax.rsqrt(jnp.maximum(q.mean() - mm * mm, 0.0) + EPS) for q, mm in zip(b, m2)]
        m2 = [q.astype(bf16).astype(f32) for q in m2]
        for d in range(DH):
            for i in range(nt):
                xf = tie(_upk(xnT[slot + i, pl.ds(z + d * 8, 8), :]).astype(f32), dep(3, d, i))
                hT[ts[i], d * 8:(d + 1) * 8, :] = _pk(((xf - m2[i]) * r2[i]).astype(bf16))
        if transpose:
            for i in range(nt):
                to_rows(put_xn, ts[i], jnp.concatenate(rows[i], axis=0))

    def prep_wqkv():
        wt = jnp.concatenate([wqkv_v[...], jnp.zeros((DP - D, 3 * D), bf16)], axis=0).T.astype(f32)
        for k in range(KT):
            wtmp[k, 0:3 * D, :] = wt[:, k * 128:(k + 1) * 128]
        for p in range(3):
            for d in range(DH):
                r = (((p + 2) % 3) * D + d * H) // 2
                l_qkv[r:r + H // 2, :] = _pk(_cat(
                    [wtmp[k, pl.ds(p * D + d, H, stride=DH), :] for k in range(KT)]).astype(bf16))

    def prep_wo(dep):
        wo = jnp.concatenate([wo_v[...].astype(f32), jnp.zeros((D, DP - D), f32)], axis=1)
        for k in range(KT):
            for d in range(DH):
                wtmp[k, d * H:(d + 1) * H, :] = tie(wo[d * H:(d + 1) * H, k * 128:(k + 1) * 128],
                                                    _rows16(dep, (k * DH + d) // 4))
        parts = []
        for k in range(KT):
            rows = [_pk(tie(wtmp[k, pl.ds(d, H, stride=DH), :], _rows16(dep, 32 + (k * DH + d) // 3)).astype(bf16))
                    for d in range(DH)]
            rows.append(jnp.zeros(((DP - D) // 2, 128), u32))
            parts.append(jnp.concatenate(rows, axis=0))
        l_wo[...] = _pk(_upk(jnp.concatenate(parts, axis=1)).T[0:D, :])

    def pace_points(part, kt):
        par = 4 // kt
        nn = part.shape[1] // 128
        return [part[d * H:(d + 1) * H, n * 128:(n + 1) * 128]
                for n0 in range(0, nn, par) for d in range(DH) for n in range(n0, min(n0 + par, nn))]

    def mix1(t, kt, n0=0, n1=NF):
        lhs = _upk(_cat([hT[t + k] for k in range(kt)]))
        if (kt * (n1 - n0)) % 4 == 0:
            return jnp.dot(lhs, w1_v[_tiles(t, kt), n0 * 128:n1 * 128], preferred_element_type=f32)
        main = jnp.dot(lhs, w1_v[_tiles(t), n0 * 128:(n1 - 2) * 128], preferred_element_type=f32)
        wl = w1_v[_tiles(t), (n1 - 2) * 128:n1 * 128]
        tail = [jnp.dot(lhs[h * (D // 2):(h + 1) * (D // 2), :], wl, preferred_element_type=f32)
                for h in range(2)]
        return jnp.concatenate([main, jnp.concatenate(tail, axis=0)], axis=1)

    ln_tiles([0], slot=3, transpose=False)
    start(range(4, NG))
    _wait(group(1))
    u_acc[:, 0:N0 * 128] = mix1(0, 1, 0, N0)
    to_rows(put_xn, 0, xnT[3])
    _wait(group(2))
    part = mix1(0, 1, N0, NF)
    u_acc[:, N0 * 128:] = part
    ln_tiles([1], pace_points(part, 1))

    def step_a(i, z):
        _wait(group_a(i))
        part = mix1(i, 1)
        u_acc[...] += part
        ln_tiles([i + 1], pace_points(part, 1), pl.multiple_of(z * 64, 64))
        return (i - 1) * (i - 2)

    zi = lax.fori_loop(1, 3, step_a, 0)
    z0 = pl.multiple_of(zi * 64, 64)
    _wait(group(5))
    part = mix1(3, 1)
    u_acc[...] += part
    ln_tiles([4, 5], pace_points(part, 1), z0)

    def step_b(i, carry):
        _wait(group_b(i))
        part = mix1(4 + 2 * i, 2)
        u_acc[...] += part
        t0 = jnp.minimum(6 + 3 * i, 7 + 2 * i)
        ln_tiles([t0 + q for q in range(3)], pace_points(part, 2), z0)
        return carry

    lax.fori_loop(0, 4, step_b, 0)
    _wait(group(10))
    part = mix1(12, 4)
    prep_wqkv()
    b1 = b1_v[...].astype(f32)
    for n in range(NF):
        u = u_acc[:, n * 128:(n + 1) * 128] + part[:, n * 128:(n + 1) * 128] + b1[n:n + 1, :]
        g_v[:, n * 128:(n + 1) * 128] = _pk(jax.nn.gelu(u, approximate=True).astype(bf16))

    def qkv_block(j):
        rj = _cat([_upk(xn_u[k, pl.ds(PJ * j, 64, stride=PL), :]) for k in range(KT)])
        res = lax.dot_general(_upk(l_qkv[...]), rj, NT, preferred_element_type=f32)
        kvq[j][pl.ds(z0, 3 * D), :] = res
        if j >= NB - (W - 1):
            kvr[j - (NB - (W - 1))][pl.ds(z0, 2 * D), :] = pltpu.roll(res[0:2 * D, :], 2, axis=1)
        return res

    edge = lax.broadcasted_iota(jnp.int32, (H, 128), 1) < 2
    scale = DH ** -0.5

    def attn_block(j, dep_qk, dep_sm, dep_pv):
        def kv_rows(w, off, d):
            if j >= w:
                return kvq[j - w][pl.ds(off + d * H, H), :]
            return kvr[j - w + (W - 1)][pl.ds(off + d * H, H), :]

        def sm(v, d):
            return v if dep_sm is None else tie(v, _rows16(dep_sm, d))

        acc = [None] * W
        for d in range(DH):
            qd = tie(kvq[j][pl.ds(2 * D + d * H, H), :], _rows16(dep_qk, d))
            for w in range(W):
                t = qd * kv_rows(w, 0, d)
                acc[w] = t if acc[w] is None else acc[w] + t
        lg = [jnp.where(edge, -1e9 / scale, acc[w]) if w > j else acc[w] for w in range(W)]
        m = sm(_tree(jnp.maximum, lg), 2)
        e = [jnp.exp2(sm((l - m) * (scale * LOG2E), 4 + 2 * (w // 2))) for w, l in enumerate(lg)]
        ssum = sm(_tree(jnp.add, e), 14)
        inv = pl.reciprocal(ssum, approx=True)
        inv = sm(inv * (2.0 - ssum * inv), 18)
        a = [ew * inv for ew in e]
        for d in range(DH):
            o = a[0] * kv_rows(0, D, d)
            for w in range(1, W):
                o = o + a[w] * kv_rows(w, D, d)
            oT[j][pl.ds(z0 + d * 8, 8), :] = _pk(tie(o, _rows16(dep_pv, d)).astype(bf16))

    def last_wait(i, carry):
        _wait(group(11))
        return carry

    order = list(range(NB - (W - 1), NB)) + list(range(NB - (W - 1)))
    for t, j in enumerate(order):
        res = qkv_block(j)
        if t >= W:
            attn_block(order[t - 1], res[0:D, :], res[D:2 * D, :], res[2 * D:3 * D, :])
        if t == WAIT_AT:
            lax.fori_loop(0, 1 + zi, last_wait, 0)
        if t == WAIT_AT + 1:
            prep_wo(res)

    ks = (0, 4, 8, 12, 14)
    b2 = b2_v[...].astype(f32)

    def mix2_tile(n):
        ps = []
        for a, b in zip(ks[:-1], ks[1:]):
            p = jnp.dot(_upk(g_v[:, a * 128:b * 128]), w2_v[a * 128:b * 128, _tiles(n)],
                        preferred_element_type=f32)
            ps.append(ps[-1] + p if ps else p)
        return ps

    def final_tile(n, y):
        on = _cat([_upk(_cat([o_u[k, pl.ds(PL * (n * 4 + i), NB, stride=PJ), :] for i in range(4)], axis=0))
                   for k in range(KT)])
        ao = lax.dot_general(_upk(l_wo[...]), on, NT, preferred_element_type=f32)
        res = (x_v[n].astype(f32) + ao + (y + b2[n:n + 1, :])).astype(bf16)
        if n == NB - 1:
            for r0, r1 in zip(LASTR[:-1], LASTR[1:]):
                out_v[r0:r1, _tiles(n)] = res[r0:r1, :]
                pltpu.make_async_copy(out_v.at[r0:r1, _tiles(n)], out_hbm.at[0, r0:r1, _tiles(n)],
                                      sems.at[0]).start()
            return
        out_v[:, _tiles(n)] = res
        if n + 1 in OUTC:
            t0 = OUTC[OUTC.index(n + 1) - 1]
            pltpu.make_async_copy(out_v.at[:, _tiles(t0, n + 1 - t0)], out_hbm.at[0, :, _tiles(t0, n + 1 - t0)],
                                  sems.at[0]).start()

    for n in range(NPRE):
        ps = mix2_tile(n)
        y_v[n] = ps[-1]
        if n < W:
            attn_block(NB - W + n, ps[0], None, ps[2])
    for j in range(NB):
        to_rows(put_o, j, oT[j][...])
    for n in range(NPRE):
        final_tile(n, y_v[n])
    for n in range(NPRE, NB):
        y = jnp.dot(_upk(g_v[:, 0:12 * 128]), w2_v[0:12 * 128, _tiles(n)], preferred_element_type=f32)
        wl = w2_v[12 * 128:, _tiles(n)]
        gl = _upk(g_v[:, 12 * 128:])
        tail = [jnp.dot(gl[h * (D // 2):(h + 1) * (D // 2), :], wl, preferred_element_type=f32)
                for h in range(2)]
        final_tile(n, jnp.concatenate(tail, axis=0) + y)
    _wait([pltpu.make_async_copy(out_v, out_hbm.at[0], sems.at[0])])


@jax.jit
def pallas_parallel_sum__sliding_local_dilated__mixer_token_mlp__prompt_kernel(
        A_x, A_wqkv, A_wo, B_x, B_w1, B_b1, B_w2, B_b2):
    any_spec = pl.BlockSpec(memory_space=pl.ANY)
    out_t = pl.pallas_call(
        _kernel,
        out_shape=jax.ShapeDtypeStruct((1, D, S), bf16),
        in_specs=[any_spec] * 7,
        out_specs=any_spec,
        scratch_shapes=[
            pltpu.VMEM((NB, D, 128), bf16),
            pltpu.VMEM((D, 3 * D), bf16),
            pltpu.VMEM((D, D), bf16),
            pltpu.VMEM((S, F), bf16),
            pltpu.VMEM((F, S), bf16),
            pltpu.VMEM((NF, 128), bf16),
            pltpu.VMEM((NB, 128), bf16),
            pltpu.VMEM((NB, D // 2, 128), u32),
            pltpu.VMEM((4, D // 2, 128), u32),
            pltpu.VMEM((KT, PROWS, 128), u32),
            pltpu.VMEM((D, F), f32),
            pltpu.VMEM((D // 2, F), u32),
            pltpu.VMEM((KT, 3 * D + 32, 128), f32),
            pltpu.VMEM((3 * D // 2, DP), u32),
            pltpu.VMEM((D // 2, DP), u32),
            pltpu.VMEM((KT, PROWS, 128), u32),
            pltpu.VMEM((NPRE, D, 128), f32),
            pltpu.VMEM((D, S), bf16),
            pltpu.SemaphoreType.DMA((NG,)),
        ] + [pltpu.VMEM((3 * D, 128), f32)] * NB + [pltpu.VMEM((2 * D, 128), f32)] * (W - 1)
          + [pltpu.VMEM((D // 2, 128), u32)] * NB,
        compiler_params=pltpu.CompilerParams(vmem_limit_bytes=100 * 2**20, disable_semaphore_checks=True),
    )(jnp.swapaxes(A_x, 1, 2), A_wqkv, A_wo, B_w1, B_b1.reshape(NF, 128), B_w2, B_b2.reshape(NB, 128))
    return jnp.swapaxes(out_t, 1, 2)
```

```python
import jax
import jax.numpy as jnp
from jax import lax
import jax.experimental.pallas as pl
import jax.experimental.pallas.tpu as pltpu

S, D, F = 2048, 448, 1792
H, DH, W = 16, 28, 8
EPS = 1e-5
LOG2E = 1.4426950408889634
NB = S // 128
NF = F // 128
DP = 512
KT = DP // 128
PJ, PL = 132, 2
PROWS = PJ * NB + 128
NG = 12
N0 = 6
WAIT_AT = 6
NPRE = int("6")
PPB = int("63")
WOS = "1" == "1"
HM = D // 2
OUTC = (0, 2, 4, 6, 8, 10, 12, 14, 15)
LASTR = (0, 224, 352, 416, 448)
bf16, f32, u32 = jnp.bfloat16, jnp.float32, jnp.uint32
NT = (((1,), (1,)), ((), ()))


def _wait(cps):
    for cp in cps:
        cp.wait()


def _cat(parts, axis=1):
    return parts[0] if len(parts) == 1 else jnp.concatenate(parts, axis=axis)


def _pk(x):
    return pltpu.bitcast(x, u32)


def _upk(x):
    return pltpu.bitcast(x, bf16)


def _tiles(t, n=1):
    if isinstance(t, int):
        return pl.ds(t * 128, n * 128)
    return pl.ds(pl.multiple_of(t * 128, 128), n * 128)


def _tree(op, xs):
    xs = list(xs)
    while len(xs) > 1:
        xs = [op(xs[i], xs[i + 1]) for i in range(0, len(xs), 2)]
    return xs[0]


def _rows16(v, d):
    return v[d * H:(d + 1) * H, :]


def _add(a, b):
    return (a.astype(f32) + b.astype(f32)).astype(bf16)


def _sub(a, b):
    return (a.astype(f32) - b.astype(f32)).astype(bf16)


def _strassen(lhs, blk, mm):
    m2 = mm(lhs(2), blk(0, 0))
    m4 = mm(lhs(4), _sub(blk(1, 0), blk(0, 0)))
    m7 = mm(lhs(7), _add(blk(1, 0), blk(1, 1)))
    m5 = mm(lhs(5), blk(1, 1))
    m1 = mm(lhs(1), _add(blk(0, 0), blk(1, 1)))
    m3 = mm(lhs(3), _sub(blk(0, 1), blk(1, 1)))
    m6 = mm(lhs(6), _add(blk(0, 0), blk(0, 1)))
    c0 = jnp.concatenate([((m4 + m7) - m5) + m1, m2 + m4], axis=0)
    c1 = jnp.concatenate([m5 + m3, ((m1 - m2) + m3) + m6], axis=0)
    return [m2, m4, m7, m5, m1, m3, m6], c0, c1


_SUM_SLOT = {1: 0, 2: 1, 5: 2, 6: 3, 7: 4}


class _Acc:
    def __init__(self, n):
        self.p = [None] * n
        self.i = 0

    def add(self, v):
        k = self.i % len(self.p)
        self.p[k] = v if self.p[k] is None else self.p[k] + v
        self.i += 1

    def mean(self):
        t = self.p[0]
        for q in self.p[1:]:
            t = t + q
        return jnp.sum(t, axis=0, keepdims=True) * (1.0 / D)


def _kernel(x_hbm, wqkv_hbm, wo_hbm, w1_hbm, b1_hbm, w2_hbm, b2_hbm, out_hbm,
            x_v, wqkv_v, wo_v, w1_v, w2_v, b1_v, b2_v, hT, xnT, xn_u, u_acc, g_v, ga, wa, wtmp, l_qkv, l_wo,
            o_u, y_v, out_v, sems, *blk):
    kvq = blk[0:NB]
    kvr = blk[NB:NB + W - 1]
    oT = blk[NB + W - 1:]

    def cp_x(t, n, sem):
        return [pltpu.make_async_copy(x_hbm.at[0, :, _tiles(t + q)], x_v.at[t + q], sem) for q in range(n)]

    def cp_w1(t, n, sem):
        return [pltpu.make_async_copy(w1_hbm.at[_tiles(t, n), :], w1_v.at[_tiles(t, n), :], sem)]

    def group_a(i):
        return cp_x(1 + i, 1, sems.at[2 + i]) + cp_w1(i, 1, sems.at[2 + i])

    def group_b(i):
        return cp_x(8 + 2 * i, 2, sems.at[6 + i]) + cp_w1(4 + 2 * i, 2, sems.at[6 + i])

    def group(g):
        sem = sems.at[g]
        if g == 0:
            return cp_x(0, 1, sem)
        if g == 1:
            return [pltpu.make_async_copy(w1_hbm.at[0:128, 0:N0 * 128], w1_v.at[0:128, 0:N0 * 128], sem)]
        if g == 2:
            return cp_x(1, 1, sem) + [
                pltpu.make_async_copy(w1_hbm.at[0:128, N0 * 128:], w1_v.at[0:128, N0 * 128:], sem)]
        if g < 5:
            return group_a(g - 2)
        if g == 5:
            return cp_x(4, 4, sem) + cp_w1(3, 1, sem)
        if g < 10:
            return group_b(g - 6)
        if g == 10:
            return cp_w1(12, 4, sem) + [pltpu.make_async_copy(wqkv_hbm, wqkv_v, sem),
                                        pltpu.make_async_copy(b1_hbm, b1_v, sem)]
        return [pltpu.make_async_copy(wo_hbm, wo_v, sem), pltpu.make_async_copy(b2_hbm, b2_v, sem),
                pltpu.make_async_copy(w2_hbm, w2_v, sem)]

    def start(gs):
        for g in gs:
            for cp in group(g):
                cp.start()

    start(range(4))
    _wait(group(0))
    never = x_v[0, 0:H, :].astype(f32) > jnp.inf

    def tie(x, dep):
        return x if dep is None else jnp.where(never, dep, x)

    def to_rows(dst, j, packed):
        t = _upk(jnp.concatenate([packed, jnp.zeros(((DP - D) // 2, 128), u32)], axis=0)).T
        for k in range(KT):
            dst(k, j, _pk(t[:, k * 128:(k + 1) * 128]))

    def put_xn(k, t, w):
        for q in range(4):
            xn_u[k, pl.ds(PL * (t * 4 + q), NB, stride=PJ), :] = w[q * NB:(q + 1) * NB, :]

    def put_o(k, j, w):
        o_u[k, pl.ds(PJ * j, 64, stride=PL), :] = w

    def ln_tiles(ts, pts=None, z=0, slot=0, transpose=True):
        nt = len(ts)
        seg = 0 if pts is None else int(len(pts) * 0.85) // 4
        nch = 2 if pts is not None else 4

        def dep(p, d, i):
            return None if pts is None else pts[p * seg + ((d * nt + i) * (seg - 8)) // (DH * nt)]

        def xrow(p, d, i):
            return tie(x_v[ts[i], d * H:(d + 1) * H, :].astype(f32), dep(p, d, i))

        a = [_Acc(nch) for _ in ts]
        for d in range(DH):
            for i in range(nt):
                a[i].add(xrow(0, d, i))
        m = [q.mean() for q in a]
        a = [_Acc(nch) for _ in ts]
        for d in range(DH):
            for i in range(nt):
                c = xrow(1, d, i) - m[i]
                a[i].add(c * c)
        r = [lax.rsqrt(q.mean() + EPS) for q in a]
        m = [q.astype(bf16).astype(f32) for q in m]
        a = [_Acc(nch) for _ in ts]
        b = [_Acc(nch) for _ in ts]
        rows = [[] for _ in ts]
        for d in range(DH):
            for i in range(nt):
                xu = _pk(((xrow(2, d, i) - m[i]) * r[i]).astype(bf16))
                xnT[slot + i, d * 8:(d + 1) * 8, :] = xu
                rows[i].append(xu)
                xf = _upk(xu).astype(f32)
                a[i].add(xf)
                b[i].add(xf * xf)
        m2 = [q.mean() for q in a]
        r2 = [lax.rsqrt(jnp.maximum(q.mean() - mm * mm, 0.0) + EPS) for q, mm in zip(b, m2)]
        m2 = [q.astype(bf16).astype(f32) for q in m2]
        for d in range(DH):
            for i in range(nt):
                xf = tie(_upk(xnT[slot + i, pl.ds(z + d * 8, 8), :]).astype(f32), dep(3, d, i))
                hT[ts[i], d * 8:(d + 1) * 8, :] = _pk(((xf - m2[i]) * r2[i]).astype(bf16))
        if transpose:
            for i in range(nt):
                to_rows(put_xn, ts[i], jnp.concatenate(rows[i], axis=0))

    def prep_wqkv():
        wt = jnp.concatenate([wqkv_v[...], jnp.zeros((DP - D, 3 * D), bf16)], axis=0).T.astype(f32)
        for k in range(KT):
            wtmp[k, 0:3 * D, :] = wt[:, k * 128:(k + 1) * 128]
        for p in range(3):
            for d in range(DH):
                r = (((p + 2) % 3) * D + d * H) // 2
                l_qkv[r:r + H // 2, :] = _pk(_cat(
                    [wtmp[k, pl.ds(p * D + d, H, stride=DH), :] for k in range(KT)]).astype(bf16))

    def prep_wo(dep):
        wo = jnp.concatenate([wo_v[...].astype(f32), jnp.zeros((D, DP - D), f32)], axis=1)
        for k in range(KT):
            for d in range(DH):
                wtmp[k, d * H:(d + 1) * H, :] = tie(wo[d * H:(d + 1) * H, k * 128:(k + 1) * 128],
                                                    _rows16(dep, (k * DH + d) // 4))
        parts = []
        for k in range(KT):
            rows = [_pk(tie(wtmp[k, pl.ds(d, H, stride=DH), :], _rows16(dep, 32 + (k * DH + d) // 3)).astype(bf16))
                    for d in range(DH)]
            rows.append(jnp.zeros(((DP - D) // 2, 128), u32))
            parts.append(jnp.concatenate(rows, axis=0))
        l_wo[...] = _pk(_upk(jnp.concatenate(parts, axis=1)).T[0:D, :])

    def pace_points(part, kt):
        par = 4 // kt
        nn = part.shape[1] // 128
        return [part[d * H:(d + 1) * H, n * 128:(n + 1) * 128]
                for n0 in range(0, nn, par) for d in range(DH) for n in range(n0, min(n0 + par, nn))]

    def mix1(t, kt, n0=0, n1=NF):
        lhs = _upk(_cat([hT[t + k] for k in range(kt)]))
        if (kt * (n1 - n0)) % 4 == 0:
            return jnp.dot(lhs, w1_v[_tiles(t, kt), n0 * 128:n1 * 128], preferred_element_type=f32)
        main = jnp.dot(lhs, w1_v[_tiles(t), n0 * 128:(n1 - 2) * 128], preferred_element_type=f32)
        wl = w1_v[_tiles(t), (n1 - 2) * 128:n1 * 128]
        tail = [jnp.dot(lhs[h * (D // 2):(h + 1) * (D // 2), :], wl, preferred_element_type=f32)
                for h in range(2)]
        return jnp.concatenate([main, jnp.concatenate(tail, axis=0)], axis=1)

    ln_tiles([0], slot=3, transpose=False)
    start(range(4, NG))
    _wait(group(1))
    u_acc[:, 0:N0 * 128] = mix1(0, 1, 0, N0)
    to_rows(put_xn, 0, xnT[3])
    _wait(group(2))
    part = mix1(0, 1, N0, NF)
    u_acc[:, N0 * 128:] = part
    ln_tiles([1], pace_points(part, 1))

    def step_a(i, z):
        _wait(group_a(i))
        part = mix1(i, 1)
        u_acc[...] += part
        ln_tiles([i + 1], pace_points(part, 1), pl.multiple_of(z * 64, 64))
        return (i - 1) * (i - 2)

    zi = lax.fori_loop(1, 3, step_a, 0)
    z0 = pl.multiple_of(zi * 64, 64)
    _wait(group(5))
    part = mix1(3, 1)
    u_acc[...] += part
    ln_tiles([4, 5], pace_points(part, 1), z0)

    def step_b(i, carry):
        _wait(group_b(i))
        part = mix1(4 + 2 * i, 2)
        u_acc[...] += part
        t0 = jnp.minimum(6 + 3 * i, 7 + 2 * i)
        ln_tiles([t0 + q for q in range(3)], pace_points(part, 2), z0)
        return carry

    lax.fori_loop(0, 4, step_b, 0)
    _wait(group(10))
    part = mix1(12, 4)
    prep_wqkv()
    b1 = b1_v[...].astype(f32)
    for n in range(NF):
        u = u_acc[:, n * 128:(n + 1) * 128] + part[:, n * 128:(n + 1) * 128] + b1[n:n + 1, :]
        g_v[:, n * 128:(n + 1) * 128] = _pk(jax.nn.gelu(u, approximate=True).astype(bf16))

    def qkv_block(j):
        rj = _cat([_upk(xn_u[k, pl.ds(PJ * j, 64, stride=PL), :]) for k in range(KT)])
        res = lax.dot_general(_upk(l_qkv[...]), rj, NT, preferred_element_type=f32)
        kvq[j][pl.ds(z0, 3 * D), :] = res
        if j >= NB - (W - 1):
            kvr[j - (NB - (W - 1))][pl.ds(z0, 2 * D), :] = pltpu.roll(res[0:2 * D, :], 2, axis=1)
        return res

    edge = lax.broadcasted_iota(jnp.int32, (H, 128), 1) < 2
    scale = DH ** -0.5

    def attn_block(j, dep_qk, dep_sm, dep_pv):
        def kv_rows(w, off, d):
            if j >= w:
                return kvq[j - w][pl.ds(off + d * H, H), :]
            return kvr[j - w + (W - 1)][pl.ds(off + d * H, H), :]

        def sm(v, d):
            return v if dep_sm is None else tie(v, dep_sm[d])

        acc = [None] * W
        for d in range(DH):
            qd = tie(kvq[j][pl.ds(2 * D + d * H, H), :], dep_qk[d])
            for w in range(W):
                t = qd * kv_rows(w, 0, d)
                acc[w] = t if acc[w] is None else acc[w] + t
        lg = [jnp.where(edge, -1e9 / scale, acc[w]) if w > j else acc[w] for w in range(W)]
        m = sm(_tree(jnp.maximum, lg), 2)
        e = [jnp.exp2(sm((l - m) * (scale * LOG2E), 4 + 2 * (w // 2))) for w, l in enumerate(lg)]
        ssum = sm(_tree(jnp.add, e), 14)
        inv = pl.reciprocal(ssum, approx=True)
        inv = sm(inv * (2.0 - ssum * inv), 18)
        a = [ew * inv for ew in e]
        for d in range(DH):
            o = a[0] * kv_rows(0, D, d)
            for w in range(1, W):
                o = o + a[w] * kv_rows(w, D, d)
            oT[j][pl.ds(z0 + d * 8, 8), :] = _pk(tie(o, dep_pv[d]).astype(bf16))

    def lhs_sums(src, dst, hk, cols, dep):
        cols = list(cols)
        for ci, c in enumerate(cols):
            for r in range(HM // H):
                pt = _rows16(dep, ((ci * (HM // H) + r) * 80) // (len(cols) * (HM // H)))

                def a(i, j):
                    w = src[i * (HM // 2) + r * 8:i * (HM // 2) + (r + 1) * 8, j * hk + c * 128:j * hk + (c + 1) * 128]
                    return _upk(w).astype(f32)
                a11, a12, a21, a22 = tie(a(0, 0), pt), a(0, 1), a(1, 0), tie(a(1, 1), pt)
                for i, v in ((1, a11 + a22), (2, a21 + a22), (5, a11 + a12), (6, a21 - a11), (7, a12 - a22)):
                    dst[_SUM_SLOT[i], pl.ds(z0 + r * 8, 8), c * 128:(c + 1) * 128] = _pk(v.astype(bf16))

    def lhs_of(src, sums, hk):
        def lhs(i):
            if i == 3:
                return _upk(src[0:HM // 2, 0:hk])
            if i == 4:
                return _upk(src[HM // 2:, hk:])
            return _upk(sums[_SUM_SLOT[i]])
        return lhs

    def last_wait(i, carry):
        _wait(group(11))
        return carry

    order = list(range(NB - (W - 1), NB)) + list(range(NB - (W - 1)))
    for t, j in enumerate(order):
        res = qkv_block(j)
        if t >= W:
            pts = [_rows16(res, d) for d in range(3 * DH)]
            attn_block(order[t - 1], pts[0:DH], pts[DH:2 * DH], pts[2 * DH:])
        if 1 <= t < 5:
            lhs_sums(g_v, ga, F // 2, range((t - 1) * 2, min(t * 2, 7)), res)
        if WOS and t == WAIT_AT + 2:
            lhs_sums(l_wo, wa, DP // 2, range(2), res)
        if t == WAIT_AT:
            lax.fori_loop(0, 1 + zi, last_wait, 0)
        if t == WAIT_AT + 1:
            prep_wo(res)

    b2 = b2_v[...].astype(f32)

    def mix2_pair(p):
        return _strassen(lhs_of(g_v, ga, F // 2),
                         lambda i, j: w2_v[i * (F // 2):(i + 1) * (F // 2), _tiles(2 * p + j)],
                         lambda a, b: jnp.dot(a, b, preferred_element_type=f32))

    def o_rows(n, ks):
        return _cat([_upk(_cat([o_u[k, pl.ds(PL * (n * 4 + i), NB, stride=PJ), :] for i in range(4)], axis=0))
                     for k in ks])

    def store_tile(n, y, ao):
        res = (x_v[n].astype(f32) + ao + (y + b2[n:n + 1, :])).astype(bf16)
        if n == NB - 1:
            for r0, r1 in zip(LASTR[:-1], LASTR[1:]):
                out_v[r0:r1, _tiles(n)] = res[r0:r1, :]
                pltpu.make_async_copy(out_v.at[r0:r1, _tiles(n)], out_hbm.at[0, r0:r1, _tiles(n)],
                                      sems.at[0]).start()
            return
        out_v[:, _tiles(n)] = res
        if n + 1 in OUTC:
            t0 = OUTC[OUTC.index(n + 1) - 1]
            pltpu.make_async_copy(out_v.at[:, _tiles(t0, n + 1 - t0)], out_hbm.at[0, :, _tiles(t0, n + 1 - t0)],
                                  sems.at[0]).start()

    def final_pair(p, y0, y1):
        nt_dot = lambda a, b: lax.dot_general(a, b, NT, preferred_element_type=f32)
        if WOS:
            _, a0, a1 = _strassen(lhs_of(l_wo, wa, DP // 2),
                                  lambda i, j: o_rows(2 * p + j, (2 * i, 2 * i + 1)), nt_dot)
        else:
            a0, a1 = [nt_dot(_upk(l_wo[...]), o_rows(2 * p + j, range(KT))) for j in range(2)]
        store_tile(2 * p, y0, a0)
        store_tile(2 * p + 1, y1, a1)

    pts = []
    for p in range(NPRE):
        ms, y0, y1 = mix2_pair(p)
        y_v[2 * p] = y0
        y_v[2 * p + 1] = y1
        pts += [_rows16(m, r) for m in ms for r in range(HM // H)]
    half = (PPB - 7) // 2
    for bi in range(W):
        q0 = bi * PPB
        attn_block(NB - W + bi, [pts[q0 + (d * half) // DH] for d in range(DH)], None,
                   [pts[q0 + half + 7 + (d * half) // DH] for d in range(DH)])
    for j in range(NB):
        to_rows(put_o, j, oT[j][...])
    for p in range(NPRE):
        final_pair(p, y_v[2 * p], y_v[2 * p + 1])
    for p in range(NPRE, NB // 2):
        _, y0, y1 = mix2_pair(p)
        final_pair(p, y0, y1)
    _wait([pltpu.make_async_copy(out_v, out_hbm.at[0], sems.at[0])])


@jax.jit
def pallas_parallel_sum__sliding_local_dilated__mixer_token_mlp__prompt_kernel(
        A_x, A_wqkv, A_wo, B_x, B_w1, B_b1, B_w2, B_b2):
    any_spec = pl.BlockSpec(memory_space=pl.ANY)
    out_t = pl.pallas_call(
        _kernel,
        out_shape=jax.ShapeDtypeStruct((1, D, S), bf16),
        in_specs=[any_spec] * 7,
        out_specs=any_spec,
        scratch_shapes=[
            pltpu.VMEM((NB, D, 128), bf16),
            pltpu.VMEM((D, 3 * D), bf16),
            pltpu.VMEM((D, D), bf16),
            pltpu.VMEM((S, F), bf16),
            pltpu.VMEM((F, S), bf16),
            pltpu.VMEM((NF, 128), bf16),
            pltpu.VMEM((NB, 128), bf16),
            pltpu.VMEM((NB, D // 2, 128), u32),
            pltpu.VMEM((4, D // 2, 128), u32),
            pltpu.VMEM((KT, PROWS, 128), u32),
            pltpu.VMEM((D, F), f32),
            pltpu.VMEM((D // 2, F), u32),
            pltpu.VMEM((5, HM // 2, F // 2), u32),
            pltpu.VMEM((5, HM // 2, DP // 2), u32),
            pltpu.VMEM((KT, 3 * D + 32, 128), f32),
            pltpu.VMEM((3 * D // 2, DP), u32),
            pltpu.VMEM((D // 2, DP), u32),
            pltpu.VMEM((KT, PROWS, 128), u32),
            pltpu.VMEM((2 * NPRE, D, 128), f32),
            pltpu.VMEM((D, S), bf16),
            pltpu.SemaphoreType.DMA((NG,)),
        ] + [pltpu.VMEM((3 * D, 128), f32)] * NB + [pltpu.VMEM((2 * D, 128), f32)] * (W - 1)
          + [pltpu.VMEM((D // 2, 128), u32)] * NB,
        compiler_params=pltpu.CompilerParams(vmem_limit_bytes=100 * 2**20, disable_semaphore_checks=True),
    )(jnp.swapaxes(A_x, 1, 2), A_wqkv, A_wo, B_w1, B_b1.reshape(NF, 128), B_w2, B_b2.reshape(NB, 128))
    return jnp.swapaxes(out_t, 1, 2)
```

```python
import jax
import jax.numpy as jnp
from jax import lax
import jax.experimental.pallas as pl
import jax.experimental.pallas.tpu as pltpu

S, D, F = 2048, 448, 1792
H, DH, W = 16, 28, 8
EPS = 1e-5
LOG2E = 1.4426950408889634
NB = S // 128
NF = F // 128
DP = 512
KT = DP // 128
HM = D // 2
HG = HM // H
PJ, PL = 132, 2
PROWS = PJ * NB + 128
NG = 13
N0 = 6
SQK = "0" == "1"
NPRE = int("7")
PPB = int("110")
LASTR = ((0, 80), (112, 192), (80, 112), (192, 224))
PREPF = int("80")
RS = "s"
UZ = "1" == "1"
SM3 = "1" == "1"
bf16, f32, u32 = jnp.bfloat16, jnp.float32, jnp.uint32
NT = (((1,), (1,)), ((), ()))
SPARTS = (1, 2, 0) if SQK else (2,)
NPARTS = () if SQK else (1, 0)
MS = HM * len(SPARTS)


def _wait(cps):
    for cp in cps:
        cp.wait()


def _cat(parts, axis=1):
    return parts[0] if len(parts) == 1 else jnp.concatenate(parts, axis=axis)


def _pk(x):
    return pltpu.bitcast(x, u32)


def _upk(x):
    return pltpu.bitcast(x, bf16)


def _tiles(t, n=1):
    if isinstance(t, int):
        return pl.ds(t * 128, n * 128)
    return pl.ds(pl.multiple_of(t * 128, 128), n * 128)


def _tree(op, xs):
    xs = list(xs)
    while len(xs) > 1:
        xs = [op(xs[i], xs[i + 1]) for i in range(0, len(xs), 2)]
    return xs[0]


def _rows16(v, d):
    return v[d * H:(d + 1) * H, :]


def _groups(v):
    return [_rows16(v, d) for d in range(v.shape[0] // H)]


def _dot(a, b):
    return jnp.dot(a, b, preferred_element_type=f32)


def _dot_nt(a, b):
    return lax.dot_general(a, b, NT, preferred_element_type=f32)


def _lhs7(a11, a12, a21, a22):
    return [_pk(v.astype(bf16)) for v in
            (a11 + a22, a21 + a22, a11, a22, a11 + a12, a21 - a11, a12 - a22)]


def _rhs5(b11, b12, b21, b22):
    return [b21 - b11, b21 + b22, b11 + b22, b12 - b22, b11 + b12]


def _strassen(lhs, blk, mm, sums=None, split=None):
    if sums is None:
        five = _rhs5(*[blk(i, j).astype(f32) for i in range(2) for j in range(2)])
        sums = lambda n: five[n].astype(bf16)
    m2 = mm(lhs(1), blk(0, 0))
    m4 = mm(lhs(3), sums(0))
    m7 = mm(lhs(6), sums(1))
    m5 = mm(lhs(4), blk(1, 1))
    m1 = mm(lhs(0), sums(2))
    m3 = mm(lhs(2), sums(3))
    a6, b6 = lhs(5), sums(4)
    if split is None:
        m6 = mm(a6, b6)
    else:
        m6 = jnp.concatenate([mm(a6[r0:r1, :], b6) for r0, r1 in zip(split[:-1], split[1:])], axis=0)
    return ([m2, m4, m7, m5, m1, m3, m6],
            (((m4 + m7) - m5) + m1, m2 + m4, m5 + m3, ((m1 - m2) + m3) + m6))


def _interleave(ms, par):
    return [_rows16(m, d) for i in range(0, len(ms), par) for d in range(ms[0].shape[0] // H)
            for m in ms[i:i + par]]


class _Acc:
    def __init__(self, n):
        self.p = [None] * n
        self.i = 0

    def add(self, v):
        k = self.i % len(self.p)
        self.p[k] = v if self.p[k] is None else self.p[k] + v
        self.i += 1

    def mean(self):
        t = self.p[0]
        for q in self.p[1:]:
            t = t + q
        return jnp.sum(t, axis=0, keepdims=True) * (1.0 / D)


def _kernel(x_hbm, wqkv_hbm, wo_hbm, w1_hbm, b1_hbm, w2_hbm, b2_hbm, out_hbm,
            x_v, wqkv_v, wo_v, w1_v, w2_v, b1_v, b2_v, hT, ha, hb, xnT, xn_u, u_acc, u_fin, ga, wa, wtmp, wtmp2,
            l_n, l_s, l_wo, o_u, y_v, out_v, sems, *blk):
    qkv = blk[0:NB]
    kvr = blk[NB:NB + W - 1]
    oT = blk[NB + W - 1:2 * NB + W - 1]
    w2s = blk[2 * NB + W - 1:2 * NB + W + 7]
    xs = blk[2 * NB + W + 7:2 * NB + W + 15]
    os_ = blk[2 * NB + W + 15:]

    def cp_x(t, n, sem):
        return [pltpu.make_async_copy(x_hbm.at[0, :, _tiles(t + q)], x_v.at[t + q], sem) for q in range(n)]

    def cp_w1(t, n, sem):
        return [pltpu.make_async_copy(w1_hbm.at[_tiles(t, n), :], w1_v.at[_tiles(t, n), :], sem)]

    def group_a(i):
        return cp_x(1 + i, 1, sems.at[2 + i]) + cp_w1(i, 1, sems.at[2 + i])

    def group_b(i):
        return cp_x(6 + 2 * i, 2, sems.at[6 + i]) + cp_w1(4 + 2 * i, 2, sems.at[6 + i])

    def group(g):
        sem = sems.at[g]
        if g == 0:
            return cp_x(0, 1, sem)
        if g == 1:
            return [pltpu.make_async_copy(w1_hbm.at[0:128, 0:N0 * 128], w1_v.at[0:128, 0:N0 * 128], sem)]
        if g == 2:
            return cp_x(1, 1, sem) + [
                pltpu.make_async_copy(w1_hbm.at[0:128, N0 * 128:], w1_v.at[0:128, N0 * 128:], sem)]
        if g < 5:
            return group_a(g - 2)
        if g == 5:
            return cp_x(4, 2, sem) + cp_w1(3, 1, sem)
        if g < 11:
            return group_b(g - 6)
        if g == 11:
            return cp_w1(14, 2, sem) + [pltpu.make_async_copy(wqkv_hbm, wqkv_v, sem),
                                        pltpu.make_async_copy(b1_hbm, b1_v, sem),
                                        pltpu.make_async_copy(wo_hbm, wo_v, sem)]
        return [pltpu.make_async_copy(b2_hbm, b2_v, sem),
                pltpu.make_async_copy(w2_hbm, w2_v, sem)]

    def start(gs):
        for g in gs:
            for cp in group(g):
                cp.start()

    start(range(4))
    _wait(group(0))
    never = x_v[0, 0:H, :].astype(f32) > jnp.inf

    def tie(x, dep):
        return x if dep is None else jnp.where(never, dep, x)

    def rhs_sums(dst, strip, n, pts):
        for r in range(n):
            pt = None if pts is None else pts[(r * len(pts)) // n]
            b11, b12, b21, b22 = strip(r)
            if RS == "z":
                dst[pl.ds(z0 + r * H, H), :] = _cat(_rhs5(tie(b11, pt), b12, b21, tie(b22, pt))).astype(bf16)
            elif RS == "s":
                dst[pl.ds(r * H, H), :] = _cat(_rhs5(tie(b11, pt), b12, b21, tie(b22, pt))).astype(bf16)
            elif RS == "n":
                dst[pl.ds(r * H, H), :] = _cat(_rhs5(b11, b12, b21, b22)).astype(bf16)
            elif RS == "l":
                dst[pl.ds(r * H, H), :] = _cat([tie(v, pt) for v in _rhs5(b11, b12, b21, b22)]).astype(bf16)

    def to_rows(dst, j, packed):
        t = _upk(jnp.concatenate([packed, jnp.zeros(((DP - D) // 2, 128), u32)], axis=0)).T
        for k in range(KT):
            dst(k, j, _pk(t[:, k * 128:(k + 1) * 128]))

    def put_xn(k, t, w):
        for q in range(4):
            xn_u[k, pl.ds(PL * (t * 4 + q), NB, stride=PJ), :] = w[q * NB:(q + 1) * NB, :]

    def put_o(k, j, w):
        o_u[k, pl.ds(PJ * j, 64, stride=PL), :] = w

    def ln_tiles(ts, pts=None, z=0, slot=0, transpose=True, pair=None):
        nt = len(ts)
        seg = 0 if pts is None else int(len(pts) * 0.85) // 4
        gap = 0 if pts is None else seg // 10
        nch = 2 if pts is not None else 4

        def dep(p, d, i):
            return None if pts is None else pts[p * seg + ((d * nt + i) * (seg - gap)) // (DH * nt)]

        def xrow(p, d, i):
            return tie(x_v[ts[i], d * H:(d + 1) * H, :].astype(f32), dep(p, d, i))

        a = [_Acc(nch) for _ in ts]
        for d in range(DH):
            for i in range(nt):
                a[i].add(xrow(0, d, i))
        m = [q.mean() for q in a]
        a = [_Acc(nch) for _ in ts]
        for d in range(DH):
            for i in range(nt):
                c = xrow(1, d, i) - m[i]
                a[i].add(c * c)
        r = [lax.rsqrt(q.mean() + EPS) for q in a]
        m = [q.astype(bf16).astype(f32) for q in m]
        a = [_Acc(nch) for _ in ts]
        b = [_Acc(nch) for _ in ts]
        rows = [[] for _ in ts]
        for d in range(DH):
            for i in range(nt):
                xu = _pk(((xrow(2, d, i) - m[i]) * r[i]).astype(bf16))
                xnT[slot + i, d * 8:(d + 1) * 8, :] = xu
                rows[i].append(xu)
                xf = _upk(xu).astype(f32)
                a[i].add(xf)
                b[i].add(xf * xf)
        m2 = [q.mean() for q in a]
        r2 = [lax.rsqrt(jnp.maximum(q.mean() - mm * mm, 0.0) + EPS) for q, mm in zip(b, m2)]
        m2 = [q.astype(bf16).astype(f32) for q in m2]

        def hrow(d, i, dp):
            xf = tie(_upk(xnT[slot + i, pl.ds(z + d * 8, 8), :]).astype(f32), dp)
            return (xf - m2[i]) * r2[i]

        if pair is None:
            for d in range(DH):
                for i in range(nt):
                    hT[d * 8:(d + 1) * 8, :] = _pk(hrow(d, i, dep(3, d, i)).astype(bf16))
        else:
            for d in range(HG):
                dp = dep(3, 2 * d, 0)
                ops = _lhs7(hrow(d, 0, dp), hrow(d, 1, dp), hrow(HG + d, 0, dp), hrow(HG + d, 1, dp))
                for q in range(7):
                    ha[q, d * 8:(d + 1) * 8, :] = ops[q]
        if transpose:
            for i in range(nt):
                to_rows(put_xn, ts[i], jnp.concatenate(rows[i], axis=0))

    def prep_t(cs, pts):
        cs = list(cs)
        for ci, c in enumerate(cs):
            wd = min(128, 3 * D - c * 128)
            w = wqkv_v[:, c * 128:c * 128 + wd]
            if wd < 128:
                w = jnp.concatenate([w, jnp.zeros((D, 128 - wd), bf16)], axis=1)
            w = pltpu.bitcast(w, f32)
            w = _cat([tie(_rows16(w, r), pts[((ci * HG + r) * len(pts)) // (len(cs) * HG)]) for r in range(HG)]
                     + [jnp.zeros(((DP - D) // 2, 128), f32)], axis=0)
            wt = _upk(w).T.astype(f32)
            for k in range(KT):
                wtmp[k, c * 128:c * 128 + wd, :] = wt[0:wd, k * 128:(k + 1) * 128]

    def wrows(p, d, k):
        return wtmp[k, pl.ds(p * D + d, H, stride=DH), :]

    def prep_plain():
        for n, p in enumerate(NPARTS):
            for d in range(DH):
                r = (n * D + d * H) // 2
                l_n[r:r + 8, :] = _pk(_cat([wrows(p, d, k) for k in range(KT)]).astype(bf16))

    def prep_strassen(pts):
        tot = len(SPARTS) * HG * 2
        for n, p in enumerate(SPARTS):
            for d in range(HG):
                for c in range(2):
                    pt = None if pts is None else pts[(((n * HG + d) * 2 + c) * len(pts)) // tot]
                    ops = _lhs7(tie(wrows(p, d, c), pt), wrows(p, d, 2 + c), wrows(p, HG + d, c),
                                tie(wrows(p, HG + d, 2 + c), pt))
                    r = (n * HM + d * H) // 2
                    for q in range(7):
                        l_s[q, r:r + 8, c * 128:(c + 1) * 128] = ops[q]

    def prep_wo(pts):
        n = len(pts) // 3
        wo = jnp.concatenate([wo_v[...].astype(f32), jnp.zeros((D, DP - D), f32)], axis=1)
        for k in range(KT):
            for d in range(DH):
                wtmp2[k, d * H:(d + 1) * H, :] = tie(wo[d * H:(d + 1) * H, k * 128:(k + 1) * 128],
                                                    pts[((k * DH + d) * n) // (KT * DH)])
        parts = []
        for k in range(KT):
            rows = [_pk(tie(wtmp2[k, pl.ds(d, H, stride=DH), :], pts[n + ((k * DH + d) * n) // (KT * DH)]).astype(bf16))
                    for d in range(DH)]
            rows.append(jnp.zeros(((DP - D) // 2, 128), u32))
            parts.append(jnp.concatenate(rows, axis=0))
        l_wo[pl.ds(z0, D // 2), :] = _pk(_upk(jnp.concatenate(parts, axis=1)).T[0:D, :])

    def prep_wo_sums(pts):
        for c in range(2):
            for d in range(HG):
                pt = pts[((c * HG + d) * len(pts)) // (2 * HG)]

                def a(i, j):
                    w = l_wo[(i * HG + d) * 8:(i * HG + d + 1) * 8, (2 * j + c) * 128:(2 * j + c + 1) * 128]
                    return tie(_upk(w).astype(f32), pt)
                ops = _lhs7(a(0, 0), a(0, 1), a(1, 0), a(1, 1))
                for q in range(7):
                    wa[q, pl.ds(z0 + d * 8, 8), c * 128:(c + 1) * 128] = ops[q]

    def mix1(t, n0=0, n1=NF):
        lhs = _upk(hT[...])
        if (n1 - n0) % 4 == 0:
            part = _dot(lhs, w1_v[_tiles(t), n0 * 128:n1 * 128])
        else:
            main = _dot(lhs, w1_v[_tiles(t), n0 * 128:(n1 - 2) * 128])
            wl = w1_v[_tiles(t), (n1 - 2) * 128:n1 * 128]
            tail = [_dot(lhs[h * HM:(h + 1) * HM, :], wl) for h in range(2)]
            part = jnp.concatenate([main, jnp.concatenate(tail, axis=0)], axis=1)
        return part, _interleave([part[:, n * 128:(n + 1) * 128] for n in range(n1 - n0)], 4)

    def mix1_pair(p, dst, z, split, copy):
        ms = []
        hr = HM // 2
        if copy:
            for i in range(7):
                hb[pl.ds(z0 + i * hr, hr), :] = ha[i]
        for q in range(NF // 2):
            m, c = _strassen(lambda i: _upk(hb[i * hr:(i + 1) * hr, :] if (copy and q > 0) else ha[i]),
                             lambda i, j: w1_v[_tiles(2 * p + i), (2 * q + j) * 128:(2 * q + j + 1) * 128],
                             _dot, None, split if q == NF // 2 - 1 else None)
            ms += m
            for n in (1, 0, 2, 3):
                cb = c[n]
                cols = slice((2 * q + n // 2) * 128, (2 * q + n // 2 + 1) * 128)
                r0 = (n % 2) * HM
                dst[pl.ds(z + r0, HM), cols] = u_acc[r0:r0 + HM, cols] + cb
        return _interleave(ms, 4)

    ln_tiles([0], slot=3, transpose=False)
    start(range(4, NG))
    _wait(group(1))
    u_acc[:, 0:N0 * 128] = mix1(0, 0, N0)[0]
    to_rows(put_xn, 0, xnT[3])
    _wait(group(2))
    part, pts = mix1(0, N0, NF)
    u_acc[:, N0 * 128:] = part
    ln_tiles([1], pts)

    def step_a(i, z):
        _wait(group_a(i))
        part, pts = mix1(i)
        u_acc[...] += part
        ln_tiles([i + 1], pts, pl.multiple_of(z * 64, 64))
        return (i - 1) * (i - 2)

    zi = lax.fori_loop(1, 3, step_a, 0)
    z0 = pl.multiple_of(zi * 64, 64)
    _wait(group(5))
    part, pts = mix1(3)
    u_acc[...] += part
    ln_tiles([4, 5], pts, z0, pair=0)

    def step_b(i, carry):
        _wait(group_b(i))
        pts = mix1_pair(2 + i, u_acc, 0, (0, 64, 128, 176, HM), True)
        ln_tiles([6 + 2 * i, 7 + 2 * i], pts, z0, pair=1 + i)
        return carry

    lax.fori_loop(0, 5, step_b, 0)
    _wait(group(11))
    pts = mix1_pair(7, u_fin, z0 if UZ else 0, (0, 64, 128, 176, HM), False)
    pts_last = pts[0:(len(pts) * PREPF) // 100]
    if SQK:
        prep_t(range(11), pts_last)
        prep_strassen(None)
    else:
        prep_t((3, 4, 5, 6, 0, 1, 2), pts_last)
        prep_plain()
    b1 = b1_v[...].astype(f32)

    def gelu_cols(cs, pts):
        cs = list(cs)
        for ci, c in enumerate(cs):
            for d in range(HG):
                def g(i, j):
                    pt = pts[(((ci * HG + d) * 4 + 2 * i + j) * len(pts)) // (len(cs) * HG * 4)]
                    n = j * (NF // 2) + c
                    u = tie(u_fin[(i * HG + d) * H:(i * HG + d + 1) * H, n * 128:(n + 1) * 128], pt)
                    return jax.nn.gelu(u + b1[n:n + 1, :], approximate=True)
                ops = _lhs7(g(0, 0), g(0, 1), g(1, 0), g(1, 1))
                for q in range(7):
                    ga[q, pl.ds(z0 + d * 8, 8), c * 128:(c + 1) * 128] = ops[q]

    order = list(range(NB - (W - 1), NB)) + list(range(NB - (W - 1)))

    def put_part(j, p, r0, v):
        qkv[j][pl.ds(z0 + p * D + r0, v.shape[0]), :] = v
        if j >= NB - (W - 1) and p > 0:
            kvr[j - (NB - (W - 1))][pl.ds(z0 + (p - 1) * D + r0, v.shape[0]), :] = pltpu.roll(v, 2, axis=1)

    def nt_sums(dst, rows, pts):
        def strip(r):
            c, g = r // 8, r % 8
            return [_rows16(rows(j, 2 * i + c), g).astype(f32) for i in range(2) for j in range(2)]
        rhs_sums(dst, strip, 16, pts)

    def nt_sum(dst, n):
        return _cat([dst[c * 128:(c + 1) * 128, n * 128:(n + 1) * 128] for c in range(2)])

    def xr(j, k):
        return _upk(xn_u[k, pl.ds(PJ * j, 64, stride=PL), :])

    def qkv_pair(t, mid):
        js = order[2 * t:2 * t + 2]
        pts = []

        def plain(j):
            if NPARTS:
                res = _dot_nt(_upk(l_n[...]), _cat([xr(j, k) for k in range(KT)]))
                for n, p in enumerate(NPARTS):
                    put_part(j, p, 0, res[n * D:(n + 1) * D, :])
                pts.extend(_groups(res))
        plain(js[0])
        if t == 0 and not SQK:
            prep_t((7, 8, 9, 10), pts[0:48])
            x_sums(0, pts)
            pts.clear()
            plain(js[1])
            prep_strassen(pts[0:44])
            pts.clear()
        ms, c = _strassen(lambda i: _upk(l_s[i]), lambda i, j: _cat([xr(js[j], 2 * i), xr(js[j], 2 * i + 1)]),
                          _dot_nt, lambda n: nt_sum(xs[t], n), (0, MS // 2, MS))
        for n, cb in enumerate(c):
            for q, p in enumerate(SPARTS):
                put_part(js[n // 2], p, (n % 2) * HM, cb[q * HM:(q + 1) * HM, :])
        pts.extend(_interleave(ms, 2)[0::2])
        if mid is not None:
            mid(list(pts))
            pts.clear()
        if t > 0 or SQK:
            plain(js[1])
        return pts

    def x_sums(t, pts):
        nt_sums(xs[t], lambda j, k: xr(order[2 * t + j], k), pts)

    def w2_sums(p, pts):
        def strip(r):
            top = w2_v[r * H:(r + 1) * H, _tiles(2 * p, 2)].astype(f32)
            bot = w2_v[F // 2 + r * H:F // 2 + (r + 1) * H, _tiles(2 * p, 2)].astype(f32)
            return top[:, 0:128], top[:, 128:], bot[:, 0:128], bot[:, 128:]
        rhs_sums(w2s[p], strip, F // 2 // H, pts)

    edge = lax.broadcasted_iota(jnp.int32, (H, 128), 1) < 2
    scale = DH ** -0.5

    def attn_block(j, pts, pace_sm):
        n_sm = len(pts) // 4 if pace_sm else len(pts) // 9
        half = (len(pts) - n_sm) // 2

        def kv_rows(w, p, d):
            if j >= w:
                return qkv[j - w][pl.ds(p * D + d * H, H), :]
            return kvr[j - w + (W - 1)][pl.ds((p - 1) * D + d * H, H), :]

        def sm(v, f):
            return tie(v, pts[half + (f * n_sm) // 20]) if pace_sm else v

        acc = [None] * W
        for d in range(DH):
            qd = tie(qkv[j][pl.ds(d * H, H), :], pts[(d * half) // DH])
            for w in range(W):
                t = qd * kv_rows(w, 1, d)
                acc[w] = t if acc[w] is None else acc[w] + t
        lg = [jnp.where(edge, -1e9 / scale, acc[w]) if w > j else acc[w] for w in range(W)]
        m = sm(_tree(jnp.maximum, lg), 2)
        e = [jnp.exp2(sm((l - m) * (scale * LOG2E), 4 + 2 * (w // 2))) for w, l in enumerate(lg)]
        ssum = sm(_tree(jnp.add, e), 14)
        inv = pl.reciprocal(ssum, approx=True)
        inv = sm(inv * (2.0 - ssum * inv), 18)
        a = [ew * inv for ew in e]
        for d in range(DH):
            o = a[0] * kv_rows(0, 2, d)
            for w in range(1, W):
                o = o + a[w] * kv_rows(w, 2, d)
            oT[j][pl.ds(z0 + d * 8, 8), :] = _pk(tie(o, pts[half + n_sm + (d * half) // DH]).astype(bf16))

    def last_wait(i, carry):
        _wait(group(12))
        return carry

    gcols = ((), (0, 1), (2, 3), (4, 5), (6,))
    def mid4(pts):
        gelu_cols(gcols[4], pts[0:(len(pts) * 7) // 8])
        lax.fori_loop(0, 1 + zi, last_wait, 0)

    if SQK:
        x_sums(0, pts_last)
    xsum_plan = {0: (1,), 1: (2, 3), 2: (4, 5), 3: (6, 7)}
    for t in range(NB // 2):
        pts = qkv_pair(t, mid4 if (t == 4 and not SQK) else None)
        hp = len(pts) // 2
        for n, tt in enumerate(xsum_plan.get(t, ())):
            x_sums(tt, pts[n * hp:n * hp + (hp * 3) // 4])
        if t == NB // 2 - 1:
            w2_sums(0, pts[0:(len(pts) * 7) // 8])
        if t < 4:
            gelu_cols(gcols[t], pts)
        if t == 4:
            if SQK:
                gelu_cols(gcols[4], pts[0:hp])
                attn_block(0, pts[hp:], True)
                lax.fori_loop(0, 1 + zi, last_wait, 0)
            else:
                attn_block(0, pts, True)
        if t > 4:
            attn_block(order[2 * t - 2], pts[0:hp], True)
            attn_block(order[2 * t - 1], pts[hp:], True)
        if t == 2:
            prep_wo(pts)
        if t == 3:
            prep_wo_sums(pts)

    b2 = b2_v[...].astype(f32)

    rounds = {}
    passes = [0]

    def dot_rounds(a, b):
        k, nk, acc = 0, a.shape[1] // 128, None
        while k < nk:
            n = min(4 - passes[0] % 4, nk - k)
            p = _dot(a[:, k * 128:(k + n) * 128], b[k * 128:(k + n) * 128, :])
            acc = p if acc is None else acc + p
            rounds[passes[0] // 4] = acc
            passes[0] += n
            k += n
        return acc

    def mix2_pair(p):
        r0 = (passes[0] + 3) // 4
        _, c = _strassen(lambda i: _upk(ga[i]),
                         lambda i, j: w2_v[i * (F // 2):(i + 1) * (F // 2), _tiles(2 * p + j)], dot_rounds,
                         lambda n: w2s[p][:, n * 128:(n + 1) * 128])
        pts = [g for r in range(r0, (passes[0] + 3) // 4) for g in _groups(rounds[r])]
        if p + 1 < NB // 2:
            w2_sums(p + 1, pts[0:(len(pts) * 5) // 6])
        return pts, c

    def o_rows(n, k):
        return _upk(_cat([o_u[k, pl.ds(PL * (n * 4 + i), NB, stride=PJ), :] for i in range(4)], axis=0))

    def o_sums(p, pts):
        nt_sums(os_[p], lambda j, k: o_rows(2 * p + j, k), pts)

    def send(r0, r1, cols):
        pltpu.make_async_copy(out_v.at[r0:r1, cols], out_hbm.at[0, r0:r1, cols], sems.at[0]).start()

    def final_pair(p, y):
        last = p == NB // 2 - 1
        ms, c = _strassen(lambda i: _upk(wa[i]),
                          lambda i, j: _cat([o_rows(2 * p + j, 2 * i), o_rows(2 * p + j, 2 * i + 1)]), _dot_nt,
                          lambda n: nt_sum(os_[p], n), (0, HM // 2, HM))
        if p + 2 < NB // 2:
            o_sums(p + 2, _interleave(ms, 2))
        for q in (1, 0, 2, 3):
            n, r0 = 2 * p + q // 2, (q % 2) * HM
            res = (x_v[n, r0:r0 + HM, :].astype(f32) + c[q] + (y(q) + b2[n:n + 1, :])).astype(bf16)
            if last and q == 3:
                for a, b in LASTR:
                    out_v[r0 + a:r0 + b, _tiles(n)] = res[a:b, :]
                    send(r0 + a, r0 + b, _tiles(n))
            else:
                out_v[r0:r0 + HM, _tiles(n)] = res
                if last:
                    send(r0, r0 + HM, _tiles(n))
        if not last:
            send(0, D, _tiles(2 * p, 2))

    pts = []
    for p in range(NPRE):
        pp, c = mix2_pair(p)
        for q in range(4):
            y_v[4 * p + q] = c[q]
        pts += pp
    for bi in range(W + 1):
        attn_block(W - 1 + bi, pts[bi * PPB:(bi + 1) * PPB], SM3)
    for j in range(NB):
        to_rows(put_o, j, oT[j][...])
    o_sums(0, pts[-5 * HG:-3 * HG])
    o_sums(1, pts[-3 * HG:-HG])
    for p in range(NPRE):
        final_pair(p, lambda q: y_v[4 * p + q])
    for p in range(NPRE, NB // 2):
        _, c = mix2_pair(p)
        final_pair(p, lambda q: c[q])
    _wait([pltpu.make_async_copy(out_v, out_hbm.at[0], sems.at[0])])


@jax.jit
def pallas_parallel_sum__sliding_local_dilated__mixer_token_mlp__prompt_kernel(
        A_x, A_wqkv, A_wo, B_x, B_w1, B_b1, B_w2, B_b2):
    any_spec = pl.BlockSpec(memory_space=pl.ANY)
    out_t = pl.pallas_call(
        _kernel,
        out_shape=jax.ShapeDtypeStruct((1, D, S), bf16),
        in_specs=[any_spec] * 7,
        out_specs=any_spec,
        scratch_shapes=[
            pltpu.VMEM((NB, D, 128), bf16),
            pltpu.VMEM((D, 3 * D), bf16),
            pltpu.VMEM((D, D), bf16),
            pltpu.VMEM((S, F), bf16),
            pltpu.VMEM((F, S), bf16),
            pltpu.VMEM((NF, 128), bf16),
            pltpu.VMEM((NB, 128), bf16),
            pltpu.VMEM((D // 2, 128), u32),
            pltpu.VMEM((7, HM // 2, 128), u32),
            pltpu.VMEM((7 * HM // 2, 128), u32),
            pltpu.VMEM((4, D // 2, 128), u32),
            pltpu.VMEM((KT, PROWS, 128), u32),
            pltpu.VMEM((D, F), f32),
            pltpu.VMEM((D, F), f32),
            pltpu.VMEM((7, HM // 2, F // 2), u32),
            pltpu.VMEM((7, HM // 2, DP // 2), u32),
            pltpu.VMEM((KT, 3 * D + 32, 128), f32),
            pltpu.VMEM((KT, D + 32, 128), f32),
            pltpu.VMEM((max(len(NPARTS), 1) * D // 2, DP), u32),
            pltpu.VMEM((7, MS // 2, DP // 2), u32),
            pltpu.VMEM((D // 2, DP), u32),
            pltpu.VMEM((KT, PROWS, 128), u32),
            pltpu.VMEM((4 * NPRE, HM, 128), f32),
            pltpu.VMEM((D, S), bf16),
            pltpu.SemaphoreType.DMA((NG,)),
        ] + [pltpu.VMEM((3 * D, 128), f32)] * NB + [pltpu.VMEM((2 * D, 128), f32)] * (W - 1)
          + [pltpu.VMEM((D // 2, 128), u32)] * NB + [pltpu.VMEM((F // 2, 5 * 128), bf16)] * 8
          + [pltpu.VMEM((256, 5 * 128), bf16)] * 16,
        compiler_params=pltpu.CompilerParams(vmem_limit_bytes=100 * 2**20, disable_semaphore_checks=True),
    )(jnp.swapaxes(A_x, 1, 2), A_wqkv, A_wo, B_w1, B_b1.reshape(NF, 128), B_w2, B_b2.reshape(NB, 128))
    return jnp.swapaxes(out_t, 1, 2)
```

```python
import jax
import jax.numpy as jnp
from jax import lax
import jax.experimental.pallas as pl
import jax.experimental.pallas.tpu as pltpu

S, D, F = 2048, 448, 1792
H, DH, W = 16, 28, 8
EPS = 1e-5
LOG2E = 1.4426950408889634
NB = S // 128
NF = F // 128
DP = 512
KT = DP // 128
HM = D // 2
HG = HM // H
PJ, PL = 132, 2
PROWS = PJ * NB + 128
NG = 13
N0 = 6
NPRE = 7
PPB = int("105")
LASTR = ((0, 128), (128, 192), (192, 224))
LNW1 = (0, 21, 42, 64, 85)
LNW2 = (0, 14, 32, 58, 90)
LNW3 = tuple(int(c) for c in "0,18,38,62,88".split(","))
PARTS = (1, 2, 0)
PTILES = {1: (3, 4, 5, 6), 2: (7, 8, 9, 10), 0: (0, 1, 2)}
MS = 3 * HM
UZ = "0" == "1"
GF = "1" == "1"
WOP = int("-1")
WON = int("3")
bf16, f32, u32 = jnp.bfloat16, jnp.float32, jnp.uint32
NT = (((1,), (1,)), ((), ()))


def _wait(cps):
    for cp in cps:
        cp.wait()


def _cat(parts, axis=1):
    return parts[0] if len(parts) == 1 else jnp.concatenate(parts, axis=axis)


def _pk(x):
    return pltpu.bitcast(x, u32)


def _upk(x):
    return pltpu.bitcast(x, bf16)


def _tiles(t, n=1):
    if isinstance(t, int):
        return pl.ds(t * 128, n * 128)
    return pl.ds(pl.multiple_of(t * 128, 128), n * 128)


def _tree(op, xs):
    xs = list(xs)
    while len(xs) > 1:
        xs = [op(xs[i], xs[i + 1]) for i in range(0, len(xs), 2)]
    return xs[0]


def _rows16(v, d):
    return v[d * H:(d + 1) * H, :]


def _groups(v):
    return [_rows16(v, d) for d in range(v.shape[0] // H)]


def _win(pts, a, b):
    return pts[(len(pts) * a) // 100:(len(pts) * b) // 100]


def _gelu(x):
    c = 0.7978845608028654
    h = 0.5 * x
    return h + h * jnp.tanh(x * (c + (c * 0.044715) * (x * x)))


def _dot(a, b):
    return jnp.dot(a, b, preferred_element_type=f32)


def _dot_nt(a, b):
    return lax.dot_general(a, b, NT, preferred_element_type=f32)


def _lhs7(a11, a12, a21, a22):
    return [v.astype(bf16) for v in (a11 + a22, a21 + a22, a11, a22, a11 + a12, a21 - a11, a12 - a22)]


def _rhs7(b11, b12, b21, b22):
    return [v.astype(bf16) for v in (b11 + b22, b11, b12 - b22, b21 - b11, b22, b11 + b12, b21 + b22)]


def _strassen(lhs, rhs, mm, split=None):
    m2, m4, m7, m5, m1, m3 = [mm(lhs(i), rhs(i)) for i in (1, 3, 6, 4, 0, 2)]
    a6, b6 = lhs(5), rhs(5)
    if split is None:
        m6 = mm(a6, b6)
    else:
        m6 = jnp.concatenate([mm(a6[r0:r1, :], b6) for r0, r1 in zip(split[:-1], split[1:])], axis=0)
    return ([m2, m4, m7, m5, m1, m3, m6],
            (((m4 + m7) - m5) + m1, m2 + m4, m5 + m3, ((m1 - m2) + m3) + m6))


def _interleave(ms, par):
    return [_rows16(m, d) for i in range(0, len(ms), par) for d in range(ms[0].shape[0] // H)
            for m in ms[i:i + par]]


class _Acc:
    def __init__(self, n):
        self.p = [None] * n
        self.i = 0

    def add(self, v):
        k = self.i % len(self.p)
        self.p[k] = v if self.p[k] is None else self.p[k] + v
        self.i += 1

    def mean(self):
        t = self.p[0]
        for q in self.p[1:]:
            t = t + q
        return jnp.sum(t, axis=0, keepdims=True) * (1.0 / D)


def _kernel(x_hbm, wqkv_hbm, wo_hbm, w1_hbm, b1_hbm, w2_hbm, b2_hbm, out_hbm,
            x_v, wqkv_v, wo_v, w1_v, w2_v, b1_v, b2_v, hT, ha, hb, xnT, xn_u, u_acc, u_fin, ga, wa, wt0, wt1, wt2, wtmp2,
            l_s, o_u, y_v, out_v, sems, *blk):
    wtmp = (wt0, wt1, wt2)
    qkv = blk[0:NB]
    kvr = blk[NB:NB + W - 1]
    oT = blk[NB + W - 1:2 * NB + W - 1]
    w2s = blk[2 * NB + W - 1:2 * NB + W + 7]
    xs = blk[2 * NB + W + 7:2 * NB + W + 15]
    os_ = blk[2 * NB + W + 15:]

    def cp_x(t, n, sem):
        return [pltpu.make_async_copy(x_hbm.at[0, :, _tiles(t + q)], x_v.at[t + q], sem) for q in range(n)]

    def cp_w1(t, n, sem):
        return [pltpu.make_async_copy(w1_hbm.at[_tiles(t, n), :], w1_v.at[_tiles(t, n), :], sem)]

    def group_a(i):
        return cp_x(1 + i, 1, sems.at[2 + i]) + cp_w1(i, 1, sems.at[2 + i])

    def group_b(i):
        return cp_x(6 + 2 * i, 2, sems.at[6 + i]) + cp_w1(4 + 2 * i, 2, sems.at[6 + i])

    def group(g):
        sem = sems.at[g]
        if g == 0:
            return cp_x(0, 1, sem)
        if g == 1:
            return [pltpu.make_async_copy(w1_hbm.at[0:128, 0:N0 * 128], w1_v.at[0:128, 0:N0 * 128], sem)]
        if g == 2:
            return cp_x(1, 1, sem) + [
                pltpu.make_async_copy(w1_hbm.at[0:128, N0 * 128:], w1_v.at[0:128, N0 * 128:], sem)]
        if g < 5:
            return group_a(g - 2)
        if g == 5:
            return cp_x(4, 2, sem) + cp_w1(3, 1, sem)
        if g < 11:
            return group_b(g - 6)
        if g == 11:
            return cp_w1(14, 2, sem) + [pltpu.make_async_copy(wqkv_hbm, wqkv_v, sem),
                                        pltpu.make_async_copy(b1_hbm, b1_v, sem),
                                        pltpu.make_async_copy(wo_hbm, wo_v, sem)]
        return [pltpu.make_async_copy(b2_hbm, b2_v, sem),
                pltpu.make_async_copy(w2_hbm, w2_v, sem)]

    def start(gs):
        for g in gs:
            for cp in group(g):
                cp.start()

    start(range(4))
    _wait(group(0))
    never = x_v[0, 0:H, :].astype(f32) > jnp.inf

    def tie(x, dep):
        return x if dep is None else jnp.where(never, dep, x)

    def rhs_sums(dst, strip, n, pts, which):
        for r in range(n):
            pt = pts[(r * len(pts)) // n]
            b11, b12, b21, b22 = strip(r)
            ops = _rhs7(tie(b11, pt), b12, b21, tie(b22, pt))
            for i in which:
                dst[i, r * H:(r + 1) * H, :] = ops[i]

    def to_rows(dst, j, packed):
        t = _upk(jnp.concatenate([packed, jnp.zeros(((DP - D) // 2, 128), u32)], axis=0)).T
        for k in range(KT):
            dst(k, j, _pk(t[:, k * 128:(k + 1) * 128]))

    def put_xn(k, t, w):
        for q in range(4):
            xn_u[k, pl.ds(PL * (t * 4 + q), NB, stride=PJ), :] = w[q * NB:(q + 1) * NB, :]

    def put_o(k, j, w):
        o_u[k, pl.ds(PJ * j, 64, stride=PL), :] = w

    def ln_tiles(ts, pts=None, z=0, slot=0, transpose=True, pair=None):
        nt = len(ts)
        nch = 2 if pts is not None else 4
        cut = LNW1 if pair is None else (LNW2 if isinstance(pair, int) else LNW3)

        def dep(p, d, i):
            if pts is None:
                return None
            f = cut[p] + (cut[p + 1] - 2 - cut[p]) * (d * nt + i) / (DH * nt)
            return pts[int(f * len(pts) / 100)]

        def xrow(p, d, i):
            return tie(x_v[ts[i], d * H:(d + 1) * H, :].astype(f32), dep(p, d, i))

        a = [_Acc(nch) for _ in ts]
        for d in range(DH):
            for i in range(nt):
                a[i].add(xrow(0, d, i))
        m = [q.mean() for q in a]
        a = [_Acc(nch) for _ in ts]
        for d in range(DH):
            for i in range(nt):
                c = xrow(1, d, i) - m[i]
                a[i].add(c * c)
        r = [lax.rsqrt(q.mean() + EPS) for q in a]
        m = [q.astype(bf16).astype(f32) for q in m]
        a = [_Acc(nch) for _ in ts]
        b = [_Acc(nch) for _ in ts]
        rows = [[] for _ in ts]
        for d in range(DH):
            for i in range(nt):
                xu = _pk(((xrow(2, d, i) - m[i]) * r[i]).astype(bf16))
                xnT[slot + i, d * 8:(d + 1) * 8, :] = xu
                rows[i].append(xu)
                xf = _upk(xu).astype(f32)
                a[i].add(xf)
                b[i].add(xf * xf)
        m2 = [q.mean() for q in a]
        r2 = [lax.rsqrt(jnp.maximum(q.mean() - mm * mm, 0.0) + EPS) for q, mm in zip(b, m2)]
        m2 = [q.astype(bf16).astype(f32) for q in m2]

        def hrow(d, i, dp):
            xf = tie(_upk(xnT[slot + i, pl.ds(z + d * 8, 8), :]).astype(f32), dp)
            return (xf - m2[i]) * r2[i]

        if pair is None:
            for d in range(DH):
                for i in range(nt):
                    hT[d * 8:(d + 1) * 8, :] = _pk(hrow(d, i, dep(3, d, i)).astype(bf16))
        else:
            for d in range(HG):
                dp = dep(3, 2 * d, 0)
                ops = _lhs7(hrow(d, 0, dp), hrow(d, 1, dp), hrow(HG + d, 0, dp), hrow(HG + d, 1, dp))
                for q in range(7):
                    ha[q, d * 8:(d + 1) * 8, :] = _pk(ops[q])
        if transpose:
            for i in range(nt):
                to_rows(put_xn, ts[i], jnp.concatenate(rows[i], axis=0))

    def prep_t(cs, pts):
        cs = list(cs)
        for ci, c in enumerate(cs):
            wd = min(128, 3 * D - c * 128)
            w = wqkv_v[:, c * 128:c * 128 + wd]
            if wd < 128:
                w = jnp.concatenate([w, jnp.zeros((D, 128 - wd), bf16)], axis=1)
            w = pltpu.bitcast(w, f32)
            per = len(pts) / (len(cs) + 1)
            w = _cat([tie(_rows16(w, r), pts[int((ci + r / HG) * per)]) for r in range(HG)]
                     + [jnp.zeros(((DP - D) // 2, 128), f32)], axis=0)
            wt = _upk(w).T.astype(f32)
            for k in range(KT):
                for h in range(0, wd, H):
                    p, r = divmod(c * 128 + h, D)
                    pt = pts[int((ci + 1 + (k * 128 + h) / DP) * per)]
                    wtmp[p][k, r:r + H, :] = tie(wt[h:h + H, k * 128:(k + 1) * 128], pt)

    def wrows(p, d, k):
        return wtmp[p][k, pl.ds(d, H, stride=DH), :]

    def prep_part(n, pts):
        p = PARTS[n]
        prep_t(PTILES[p], _win(pts, 0, 55))
        pts = _win(pts, 52, 90)
        for d in range(HG):
            for c in range(2):
                pt = pts[((d * 2 + c) * len(pts)) // (2 * HG)]
                ops = _lhs7(tie(wrows(p, d, c), pt), wrows(p, d, 2 + c), wrows(p, HG + d, c),
                            tie(wrows(p, HG + d, 2 + c), pt))
                r = (n * HM + d * H) // 2
                for q in range(7):
                    l_s[q, r:r + 8, c * 128:(c + 1) * 128] = _pk(ops[q])

    def prep_wo(pts):
        p1, p2, p3 = _win(pts, 0, 30), _win(pts, 30, 62), _win(pts, 66, 100)
        wo = jnp.concatenate([wo_v[...].astype(f32), jnp.zeros((D, DP - D), f32)], axis=1)
        for k in range(KT):
            for d in range(DH):
                wtmp2[k, d * H:(d + 1) * H, :] = tie(wo[d * H:(d + 1) * H, k * 128:(k + 1) * 128],
                                                     p1[((k * DH + d) * len(p1)) // (KT * DH)])
        parts = []
        for k in range(KT):
            rows = [_pk(tie(wtmp2[k, pl.ds(d, H, stride=DH), :],
                            p2[((k * DH + d) * len(p2)) // (KT * DH)]).astype(bf16)) for d in range(DH)]
            rows.append(jnp.zeros(((DP - D) // 2, 128), u32))
            parts.append(jnp.concatenate(rows, axis=0))
        wt = _upk(jnp.concatenate(parts, axis=1)).T
        for c in range(2):
            for d in range(HG):
                pt = p3[((c * HG + d) * len(p3)) // (2 * HG)]

                def a(i, j):
                    w = wt[(i * HG + d) * H:(i * HG + d + 1) * H, (2 * j + c) * 128:(2 * j + c + 1) * 128]
                    return tie(w.astype(f32), pt)
                ops = _lhs7(a(0, 0), a(0, 1), a(1, 0), a(1, 1))
                for q in range(7):
                    wa[q, pl.ds(z0 + d * 8, 8), c * 128:(c + 1) * 128] = _pk(ops[q])

    def mix1(t, n0=0, n1=NF):
        lhs = _upk(hT[...])
        if (n1 - n0) % 4 == 0:
            part = _dot(lhs, w1_v[_tiles(t), n0 * 128:n1 * 128])
        else:
            main = _dot(lhs, w1_v[_tiles(t), n0 * 128:(n1 - 2) * 128])
            wl = w1_v[_tiles(t), (n1 - 2) * 128:n1 * 128]
            tail = [_dot(lhs[h * HM:(h + 1) * HM, :], wl) for h in range(2)]
            part = jnp.concatenate([main, jnp.concatenate(tail, axis=0)], axis=1)
        return part, _interleave([part[:, n * 128:(n + 1) * 128] for n in range(n1 - n0)], 4)

    def mix1_pair(p, dst, z, split, copy):
        ms = []
        hr = HM // 2
        for i in range(7):
            if copy:
                hb[pl.ds(z0 + i * hr, hr), :] = ha[i]
        for q in range(NF // 2):
            wb = [w1_v[_tiles(2 * p + i), (2 * q + j) * 128:(2 * q + j + 1) * 128]
                  for i in range(2) for j in range(2)]
            rhs = _rhs7(*[w.astype(f32) for w in wb])
            rhs[1], rhs[4] = wb[0], wb[3]
            m, c = _strassen(lambda i: _upk(hb[i * hr:(i + 1) * hr, :] if (copy and q > 0) else ha[i]), lambda i: rhs[i],
                             _dot, split if q == NF // 2 - 1 else None)
            ms += m
            for n in (1, 0, 2, 3):
                cb = c[n]
                cols = slice((2 * q + n // 2) * 128, (2 * q + n // 2 + 1) * 128)
                r0 = (n % 2) * HM
                dst[pl.ds(z + r0, HM), cols] = u_acc[r0:r0 + HM, cols] + cb
        return _interleave(ms, 4)

    ln_tiles([0], slot=3, transpose=False)
    start(range(4, NG))
    _wait(group(1))
    u_acc[:, 0:N0 * 128] = mix1(0, 0, N0)[0]
    to_rows(put_xn, 0, xnT[3])
    _wait(group(2))
    part, pts = mix1(0, N0, NF)
    u_acc[:, N0 * 128:] = part
    ln_tiles([1], pts)

    def step_a(i, z):
        _wait(group_a(i))
        part, pts = mix1(i)
        u_acc[...] += part
        ln_tiles([i + 1], pts, pl.multiple_of(z * 64, 64))
        return (i - 1) * (i - 2)

    zi = lax.fori_loop(1, 3, step_a, 0)
    z0 = pl.multiple_of(zi * 64, 64)
    _wait(group(5))
    part, pts = mix1(3)
    u_acc[...] += part
    ln_tiles([4, 5], pts, z0, pair=0)

    def step_b(i, carry):
        _wait(group_b(i))
        pts = mix1_pair(2 + i, u_acc, 0, (0, 64, 128, 176, HM), True)
        ln_tiles([6 + 2 * i, 7 + 2 * i], pts, z0, pair=1 + i)
        return carry

    lax.fori_loop(0, 5, step_b, 0)
    _wait(group(11))
    pts = mix1_pair(7, u_fin, z0 if UZ else 0, (0, 64, 128, 176, HM), False)
    pts_last = pts
    prep_part(0, pts)
    b1 = b1_v[...].astype(f32)

    def gelu_cols(cs, pts):
        cs = list(cs)
        for ci, c in enumerate(cs):
            for d in range(HG):
                def g(i, j):
                    pt = pts[(((ci * HG + d) * 4 + 2 * i + j) * len(pts)) // (len(cs) * HG * 4)]
                    n = j * (NF // 2) + c
                    u = tie(u_fin[(i * HG + d) * H:(i * HG + d + 1) * H, n * 128:(n + 1) * 128], pt)
                    return _gelu(u + b1[n:n + 1, :]) if GF else jax.nn.gelu(u + b1[n:n + 1, :], approximate=True)
                ops = _lhs7(g(0, 0), g(0, 1), g(1, 0), g(1, 1))
                for q in range(7):
                    ga[q, pl.ds(z0 + d * 8, 8), c * 128:(c + 1) * 128] = _pk(ops[q])

    order = list(range(NB - (W - 1), NB)) + list(range(NB - (W - 1)))

    def put_part(j, p, r0, v):
        qkv[j][pl.ds(z0 + p * D + r0, v.shape[0]), :] = v
        if j >= NB - (W - 1) and p > 0:
            kvr[j - (NB - (W - 1))][pl.ds(z0 + (p - 1) * D + r0, v.shape[0]), :] = pltpu.roll(v, 2, axis=1)

    def nt_sums(dst, rows, pts):
        def strip(r):
            c, g = r // 8, r % 8
            return [_rows16(rows(j, 2 * i + c), g).astype(f32) for i in range(2) for j in range(2)]
        rhs_sums(dst, strip, 16, pts, (0, 2, 3, 5, 6))

    def nt_rhs(dst, rows):
        def rhs(i):
            if i in (1, 4):
                return _cat([rows(i // 4, 2 * (i // 4) + c) for c in range(2)])
            return _cat([dst[i, c * 128:(c + 1) * 128, :] for c in range(2)])
        return rhs

    def xr(j, k):
        return _upk(xn_u[k, pl.ds(PJ * j, 64, stride=PL), :])

    def qkv_rows(t, n0, n1, split):
        js = order[2 * t:2 * t + 2]
        rows = (n1 - n0) * HM
        ms, c = _strassen(lambda i: _upk(l_s[i, n0 * HM // 2:n1 * HM // 2, :]),
                          nt_rhs(xs[t], lambda j, k: xr(js[j], k)), _dot_nt, (0, rows // 2, rows) if split else None)
        for q in (1, 0, 2, 3):
            for n in range(n0, n1):
                put_part(js[q // 2], PARTS[n], (q % 2) * HM, c[q][(n - n0) * HM:(n - n0 + 1) * HM, :])
        return ms

    def qkv_quad(n):
        ms = qkv_rows(0, n, n + 1, False) + qkv_rows(1, n, n + 1, False)
        return [g for m in ms[1::2] for g in _groups(m)]

    def qkv_pair(t):
        ms = qkv_rows(t, 0, 3, True)
        return [g for m in ms[1:6:2] for g in _groups(m)] + _groups(ms[6][0:MS // 2, :])

    def x_sums(t, pts):
        nt_sums(xs[t], lambda j, k: xr(order[2 * t + j], k), pts)

    def w2_sums(p, pts):
        def strip(r):
            top = w2_v[r * H:(r + 1) * H, _tiles(2 * p, 2)].astype(f32)
            bot = w2_v[F // 2 + r * H:F // 2 + (r + 1) * H, _tiles(2 * p, 2)].astype(f32)
            return top[:, 0:128], top[:, 128:], bot[:, 0:128], bot[:, 128:]
        rhs_sums(w2s[p], strip, F // 2 // H, pts, range(7))

    edge = lax.broadcasted_iota(jnp.int32, (H, 128), 1) < 2
    scale = DH ** -0.5

    def attn_block(j, pts, pace_sm):
        n_sm = len(pts) // 4 if pace_sm else len(pts) // 9
        half = (len(pts) - n_sm) // 2

        def kv_rows(w, p, d):
            if j >= w:
                return qkv[j - w][pl.ds(p * D + d * H, H), :]
            return kvr[j - w + (W - 1)][pl.ds((p - 1) * D + d * H, H), :]

        def sm(v, f):
            return tie(v, pts[half + (f * n_sm) // 20]) if pace_sm else v

        acc = [None] * W
        for d in range(DH):
            qd = tie(qkv[j][pl.ds(d * H, H), :], pts[(d * half) // DH])
            for w in range(W):
                t = qd * kv_rows(w, 1, d)
                acc[w] = t if acc[w] is None else acc[w] + t
        lg = [jnp.where(edge, -1e9 / scale, acc[w]) if w > j else acc[w] for w in range(W)]
        m = sm(_tree(jnp.maximum, lg), 2)
        e = [jnp.exp2(sm((l - m) * (scale * LOG2E), 4 + 2 * (w // 2))) for w, l in enumerate(lg)]
        ssum = sm(_tree(jnp.add, e), 14)
        inv = pl.reciprocal(ssum, approx=True)
        inv = sm(inv * (2.0 - ssum * inv), 18)
        a = [ew * inv for ew in e]
        for d in range(DH):
            o = a[0] * kv_rows(0, 2, d)
            for w in range(1, W):
                o = o + a[w] * kv_rows(w, 2, d)
            ob = tie(o, pts[half + n_sm + (d * half) // DH]).astype(bf16)
            oT[j][pl.ds(z0 + d * 8, 8), :] = _pk(ob)

    def last_wait(i, carry):
        _wait(group(12))
        return carry

    x_sums(0, _win(pts_last, 0, 40))
    x_sums(1, _win(pts_last, 40, 80))
    prep_part(1, qkv_quad(0))
    prep_part(2, qkv_quad(1))
    pts = qkv_quad(2)
    x_sums(2, _win(pts, 0, 20))
    gelu_cols((0,), _win(pts, 20, 100))
    mid = []
    for t in range(2, NB // 2):
        pts = qkv_pair(t)
        mid += pts
        if WOP < 0 and t == 4:
            prep_wo(_win(mid, 0, 92))
        if t + 1 < NB // 2:
            x_sums(t + 1, _win(pts, 0, 12))
            pts = _win(pts, 12, 100)
        else:
            w2_sums(0, _win(pts, 0, 88))
        if t <= 4:
            gelu_cols((2 * t - 3, 2 * t - 2), _win(pts, 0, 100 if t < 4 else 94))
        else:
            attn_block(order[2 * t - 2], _win(pts, 0, 50), True)
            attn_block(order[2 * t - 1], _win(pts, 50, 100), True)
        if t == 4:
            lax.fori_loop(0, 1 + zi, last_wait, 0)

    b2 = b2_v[...].astype(f32)

    rounds = {}
    passes = [0]

    def dot_rounds(a, b):
        k, nk, acc = 0, a.shape[1] // 128, None
        while k < nk:
            n = min(4 - passes[0] % 4, nk - k)
            p = _dot(a[:, k * 128:(k + n) * 128], b[k * 128:(k + n) * 128, :])
            acc = p if acc is None else acc + p
            rounds[passes[0] // 4] = acc
            passes[0] += n
            k += n
        return acc

    def mix2_pair(p):
        r0 = (passes[0] + 3) // 4
        _, c = _strassen(lambda i: _upk(ga[i]), lambda i: w2s[p][i], dot_rounds)
        pts = [g for r in range(r0, (passes[0] + 3) // 4) for g in _groups(rounds[r])]
        if p + 1 < NB // 2:
            w2_sums(p + 1, pts[0:(len(pts) * 5) // 6])
        return pts, c

    def o_rows(n, k):
        return _upk(_cat([o_u[k, pl.ds(PL * (n * 4 + i), NB, stride=PJ), :] for i in range(4)], axis=0))

    def o_sums(p, pts):
        nt_sums(os_[p], lambda j, k: o_rows(2 * p + j, k), pts)

    def send(r0, r1, cols):
        pltpu.make_async_copy(out_v.at[r0:r1, cols], out_hbm.at[0, r0:r1, cols], sems.at[0]).start()

    def wo_pair(p):
        ms, c = _strassen(lambda i: _upk(wa[i]), nt_rhs(os_[p], lambda j, k: o_rows(2 * p + j, k)), _dot_nt)
        passes[0] += 14
        if p + 2 < NB // 2:
            o_sums(p + 2, _interleave(ms, 2))
        return c

    def store_pair(p, first, second):
        last = p == NB // 2 - 1
        for q in (1, 0, 2, 3):
            n, r0 = 2 * p + q // 2, (q % 2) * HM
            res = ((x_v[n, r0:r0 + HM, :].astype(f32) + b2[n:n + 1, :] + first(q)) + second(q)).astype(bf16)
            if last and q == 3:
                for a, b in LASTR:
                    out_v[r0 + a:r0 + b, _tiles(n)] = res[a:b, :]
                    send(r0 + a, r0 + b, _tiles(n))
            else:
                out_v[r0:r0 + HM, _tiles(n)] = res
                if last:
                    send(r0, r0 + HM, _tiles(n))
        if not last:
            send(0, D, _tiles(2 * p, 2))

    pts = []
    for p in range(NPRE):
        pp, c = mix2_pair(p)
        for q in range(4):
            y_v[4 * p + q] = c[q]
        pts += pp
    if WOP >= 0:
        prep_wo(pts[WOP * 171:(WOP + WON) * 171])
    for bi, j in enumerate([0] + list(range(W - 1, NB))):
        attn_block(j, pts[bi * PPB:(bi + 1) * PPB], True)
    for j in range(NB):
        to_rows(put_o, j, oT[j][...])
    o_sums(0, pts[-5 * HG:-3 * HG])
    o_sums(1, pts[-3 * HG:-HG])
    for p in range(NPRE):
        c = wo_pair(p)
        store_pair(p, lambda q: y_v[4 * p + q], lambda q: c[q])
    for p in range(NPRE, NB // 2):
        c = wo_pair(p)
        _, y = mix2_pair(p)
        store_pair(p, lambda q: c[q], lambda q: y[q])
    _wait([pltpu.make_async_copy(out_v, out_hbm.at[0], sems.at[0])])


@jax.jit
def pallas_parallel_sum__sliding_local_dilated__mixer_token_mlp__prompt_kernel(
        A_x, A_wqkv, A_wo, B_x, B_w1, B_b1, B_w2, B_b2):
    any_spec = pl.BlockSpec(memory_space=pl.ANY)
    out_t = pl.pallas_call(
        _kernel,
        out_shape=jax.ShapeDtypeStruct((1, D, S), bf16),
        in_specs=[any_spec] * 7,
        out_specs=any_spec,
        scratch_shapes=[
            pltpu.VMEM((NB, D, 128), bf16),
            pltpu.VMEM((D, 3 * D), bf16),
            pltpu.VMEM((D, D), bf16),
            pltpu.VMEM((S, F), bf16),
            pltpu.VMEM((F, S), bf16),
            pltpu.VMEM((NF, 128), bf16),
            pltpu.VMEM((NB, 128), bf16),
            pltpu.VMEM((D // 2, 128), u32),
            pltpu.VMEM((7, HM // 2, 128), u32),
            pltpu.VMEM((7 * HM // 2, 128), u32),
            pltpu.VMEM((4, D // 2, 128), u32),
            pltpu.VMEM((KT, PROWS, 128), u32),
            pltpu.VMEM((D, F), f32),
            pltpu.VMEM((D, F), f32),
            pltpu.VMEM((7, HM // 2, F // 2), u32),
            pltpu.VMEM((7, HM // 2, DP // 2), u32),
            pltpu.VMEM((KT, D + 32, 128), f32),
            pltpu.VMEM((KT, D + 32, 128), f32),
            pltpu.VMEM((KT, D + 32, 128), f32),
            pltpu.VMEM((KT, D + 32, 128), f32),
            pltpu.VMEM((7, MS // 2, DP // 2), u32),
            pltpu.VMEM((KT, PROWS, 128), u32),
            pltpu.VMEM((4 * NPRE, HM, 128), f32),
            pltpu.VMEM((D, S), bf16),
            pltpu.SemaphoreType.DMA((NG,)),
        ] + [pltpu.VMEM((3 * D, 128), f32)] * NB + [pltpu.VMEM((2 * D, 128), f32)] * (W - 1)
          + [pltpu.VMEM((D // 2, 128), u32)] * NB + [pltpu.VMEM((7, F // 2, 128), bf16)] * 8
          + [pltpu.VMEM((7, 256, 128), bf16)] * 16,
        compiler_params=pltpu.CompilerParams(vmem_limit_bytes=100 * 2**20, disable_semaphore_checks=True),
    )(jnp.swapaxes(A_x, 1, 2), A_wqkv, A_wo, B_w1, B_b1.reshape(NF, 128), B_w2, B_b2.reshape(NB, 128))
    return jnp.swapaxes(out_t, 1, 2)
```

```python
import jax
import jax.numpy as jnp
from jax import lax
import jax.experimental.pallas as pl
import jax.experimental.pallas.tpu as pltpu

S, D, F = 2048, 448, 1792
H, DH, W = 16, 28, 8
EPS = 1e-5
LOG2E = 1.4426950408889634
NB = S // 128
NF = F // 128
DP = 512
KT = DP // 128
HM = D // 2
HG = HM // H
PJ, PL = 132, 2
PROWS = PJ * NB + 128
NG = 13
N0 = 6
NPRE = 7
PPA = int("134")
PPB = int("86")
LASTR = ((0, 128), (128, 192), (192, 224))
LNW1 = (0, 21, 42, 64, 85)
LNW2 = (0, 14, 32, 58, 90)
LNW3 = tuple(int(c) for c in "0,18,38,62,88".split(","))
if "qkv" == "qkv":
    PARTS = (0, 1, 2)
    PTILES = {0: (0, 1, 2, 3), 1: (4, 5, 6), 2: (7, 8, 9, 10)}
elif "qkv" == "qvk":
    PARTS = (0, 2, 1)
    PTILES = {0: (0, 1, 2, 3), 1: (4, 5, 6), 2: (7, 8, 9, 10)}
else:
    PARTS = (1, 2, 0)
    PTILES = {1: (3, 4, 5, 6), 2: (7, 8, 9, 10), 0: (0, 1, 2)}
MS = 3 * HM
UZ = "0" == "1"
GF = "1" == "1"
WOP = int("-2")
SMF = int("14")
W2A = int("0")
W2B = int("90")
SEQ = "0" == "1"
RAW = "1" == "1"
RAW2 = "1" == "1"
PW = tuple(int(c) for c in "50,55,92".split(","))
XW = tuple(int(c) for c in "0,15,80,95".split(","))
W0S = "1" == "1"
W7 = int("1")
WON = int("4")
bf16, f32, u32 = jnp.bfloat16, jnp.float32, jnp.uint32
NT = (((1,), (1,)), ((), ()))


def _wait(cps):
    for cp in cps:
        cp.wait()


def _cat(parts, axis=1):
    return parts[0] if len(parts) == 1 else jnp.concatenate(parts, axis=axis)


def _pk(x):
    return pltpu.bitcast(x, u32)


def _upk(x):
    return pltpu.bitcast(x, bf16)


def _tiles(t, n=1):
    if isinstance(t, int):
        return pl.ds(t * 128, n * 128)
    return pl.ds(pl.multiple_of(t * 128, 128), n * 128)


def _tree(op, xs):
    xs = list(xs)
    while len(xs) > 1:
        xs = [op(xs[i], xs[i + 1]) for i in range(0, len(xs), 2)]
    return xs[0]


def _rows16(v, d):
    return v[d * H:(d + 1) * H, :]


def _groups(v):
    return [_rows16(v, d) for d in range(v.shape[0] // H)]


def _win(pts, a, b):
    return pts[(len(pts) * a) // 100:(len(pts) * b) // 100]


def _gelu(x):
    c = 0.7978845608028654
    h = 0.5 * x
    return h + h * jnp.tanh(x * (c + (c * 0.044715) * (x * x)))


def _dot(a, b):
    return jnp.dot(a, b, preferred_element_type=f32)


def _dot_nt(a, b):
    return lax.dot_general(a, b, NT, preferred_element_type=f32)


def _lhs7(a11, a12, a21, a22):
    return [v.astype(bf16) for v in (a11 + a22, a21 + a22, a11, a22, a11 + a12, a21 - a11, a12 - a22)]


def _rhs7(b11, b12, b21, b22):
    return [v.astype(bf16) for v in (b11 + b22, b11, b12 - b22, b21 - b11, b22, b11 + b12, b21 + b22)]


def _strassen(lhs, rhs, mm, split=None):
    m2 = mm(lhs(1), rhs(1))
    m4 = mm(lhs(3), rhs(3))
    c21 = m2 + m4
    m7 = mm(lhs(6), rhs(6))
    c11 = m4 + m7
    m5 = mm(lhs(4), rhs(4))
    c11 = c11 - m5
    m1 = mm(lhs(0), rhs(0))
    c11 = c11 + m1
    c22 = m1 - m2
    m3 = mm(lhs(2), rhs(2))
    c12 = m5 + m3
    c22 = c22 + m3
    a6, b6 = lhs(5), rhs(5)
    if split is None:
        m6 = mm(a6, b6)
    else:
        m6 = jnp.concatenate([mm(a6[r0:r1, :], b6) for r0, r1 in zip(split[:-1], split[1:])], axis=0)
    return [m2, m4, m7, m5, m1, m3, m6], (c11, c21, c12, c22 + m6)


def _lhs13(top, bot, lo):
    rest = (jnp.where(lo, -top[2], top[2]), jnp.where(lo, bot[2], -bot[2]),
            jnp.where(lo, top[3], top[2]), jnp.where(lo, bot[3], bot[2]),
            jnp.where(lo, top[2], top[3]), jnp.where(lo, bot[2], bot[3]))
    return _lhs7(top[0], top[1], bot[0], bot[1]) + [v.astype(bf16) for v in rest]


def _rhs10(b, c, lo):
    t = b[2] + c[2]
    rest = (jnp.where(lo, b[2], c[2]), jnp.where(lo, b[3], t), jnp.where(lo, t, c[3]))
    return _rhs7(b[0], c[0], b[1], c[1]) + [v.astype(bf16) for v in rest]


def _mm13(lhs, rhs, mm):
    def p(i, j):
        return mm(lhs(i), rhs(j), i in (5, 6, 7, 8, 9, 10, 11, 12))
    p2 = p(1, 1)
    p2 = p2 + p(8, 7)
    c21 = p2 + p(10, 8)
    m4 = p(3, 3)
    c21 = c21 + m4
    c11 = m4 + p(6, 6)
    c11 = c11 + p(9, 8)
    p5 = p(4, 4)
    p5 = p5 + p(7, 7)
    c11 = c11 - p5
    m1 = p(0, 0)
    c11 = c11 + m1
    c22 = m1 - p2
    m3 = p(2, 2)
    c22 = c22 + m3
    c12 = p5 + m3
    c12 = c12 + p(11, 9)
    c22 = c22 + p(5, 5)
    c22 = c22 + p(12, 9)
    return c11, c21, c12, c22


class _Rounds:
    def __init__(self, n):
        self.n = n
        self.res = {}

    def add(self, n, m=None):
        if m is not None:
            self.res.setdefault((self.n + n - 1) // 4, m)
        self.n += n

    def take(self):
        pts = [g for r in sorted(self.res) if self.res[r] is not None for g in _groups(self.res[r])]
        self.res = {max(self.res): None}
        return pts


def _interleave(ms, par):
    return [_rows16(m, d) for i in range(0, len(ms), par) for d in range(ms[0].shape[0] // H)
            for m in ms[i:i + par]]


class _Acc:
    def __init__(self, n):
        self.p = [None] * n
        self.i = 0

    def add(self, v):
        k = self.i % len(self.p)
        self.p[k] = v if self.p[k] is None else self.p[k] + v
        self.i += 1

    def mean(self):
        t = self.p[0]
        for q in self.p[1:]:
            t = t + q
        return jnp.sum(t, axis=0, keepdims=True) * (1.0 / D)


def _kernel(x_hbm, wqkv_hbm, wo_hbm, w1_hbm, b1_hbm, w2_hbm, b2_hbm, out_hbm,
            x_v, wqkv_v, wo_v, w1_v, w2_v, b1_v, b2_v, hT, ha, hb, xnT, xn_u, u_acc, u_fin, ga, wa, wt0, wt1, wt2, wtmp2,
            l_s, o_u, y_v, out_v, sems, *blk):
    wtmp = (wt0, wt1, wt2)
    qkv = blk[0:NB]
    kvr = blk[NB:NB + W - 1]
    oT = blk[NB + W - 1:2 * NB + W - 1]
    w2s = blk[2 * NB + W - 1:2 * NB + W + 7]
    xs = blk[2 * NB + W + 7:2 * NB + W + 15]
    os_ = blk[2 * NB + W + 15:]

    def cp_x(t, n, sem):
        return [pltpu.make_async_copy(x_hbm.at[0, :, _tiles(t + q)], x_v.at[t + q], sem) for q in range(n)]

    def cp_w1(t, n, sem):
        return [pltpu.make_async_copy(w1_hbm.at[_tiles(t, n), :], w1_v.at[_tiles(t, n), :], sem)]

    def group_a(i):
        return cp_x(1 + i, 1, sems.at[2 + i]) + cp_w1(i, 1, sems.at[2 + i])

    def group_b(i):
        return cp_x(6 + 2 * i, 2, sems.at[6 + i]) + cp_w1(4 + 2 * i, 2, sems.at[6 + i])

    def group(g):
        sem = sems.at[g]
        if g == 0:
            return cp_x(0, 1, sem)
        if g == 1:
            return [pltpu.make_async_copy(w1_hbm.at[0:128, 0:N0 * 128], w1_v.at[0:128, 0:N0 * 128], sem)]
        if g == 2:
            return cp_x(1, 1, sem) + [
                pltpu.make_async_copy(w1_hbm.at[0:128, N0 * 128:], w1_v.at[0:128, N0 * 128:], sem)]
        if g < 5:
            return group_a(g - 2)
        if g == 5:
            return cp_x(4, 2, sem) + cp_w1(3, 1, sem)
        if g < 11:
            return group_b(g - 6)
        if g == 11:
            return cp_w1(14, 2, sem) + [pltpu.make_async_copy(wqkv_hbm, wqkv_v, sem),
                                        pltpu.make_async_copy(b1_hbm, b1_v, sem),
                                        pltpu.make_async_copy(wo_hbm, wo_v, sem)]
        return [pltpu.make_async_copy(b2_hbm, b2_v, sem),
                pltpu.make_async_copy(w2_hbm, w2_v, sem)]

    def start(gs):
        for g in gs:
            for cp in group(g):
                cp.start()

    start(range(4))
    _wait(group(0))
    never = x_v[0, 0:H, :].astype(f32) > jnp.inf

    lo = lax.broadcasted_iota(jnp.int32, (H, 128), 1) < 64

    def tie(x, dep):
        return x if dep is None else jnp.where(never, dep, x)

    def rhs_sums(dst, strip, n, pts, which):
        for r in range(n):
            pt = pts[(r * len(pts)) // n]
            b11, b12, b21, b22 = strip(r)
            ops = _rhs7(tie(b11, pt), b12, b21, tie(b22, pt))
            for i in which:
                dst[i, r * H:(r + 1) * H, :] = ops[i]

    def to_rows(dst, j, packed):
        t = _upk(jnp.concatenate([packed, packed[(2 * D - DP) // 2:, :]], axis=0)).T
        for k in range(KT):
            dst(k, j, _pk(t[:, k * 128:(k + 1) * 128]))

    def put_xn(k, t, w):
        for q in range(4):
            xn_u[k, pl.ds(PL * (t * 4 + q), NB, stride=PJ), :] = w[q * NB:(q + 1) * NB, :]

    def put_o(k, j, w):
        o_u[k, pl.ds(PJ * j, 64, stride=PL), :] = w

    def ln_tiles(ts, pts=None, z=0, slot=0, transpose=True, pair=None):
        nt = len(ts)
        nch = 2 if pts is not None else 4
        cut = LNW1 if pair is None else (LNW2 if isinstance(pair, int) else LNW3)

        def dep(p, d, i):
            if pts is None:
                return None
            f = cut[p] + (cut[p + 1] - 2 - cut[p]) * (d * nt + i) / (DH * nt)
            return pts[int(f * len(pts) / 100)]

        def xrow(p, d, i):
            return tie(x_v[ts[i], d * H:(d + 1) * H, :].astype(f32), dep(p, d, i))

        a = [_Acc(nch) for _ in ts]
        for d in range(DH):
            for i in range(nt):
                a[i].add(xrow(0, d, i))
        m = [q.mean() for q in a]
        a = [_Acc(nch) for _ in ts]
        for d in range(DH):
            for i in range(nt):
                c = xrow(1, d, i) - m[i]
                a[i].add(c * c)
        r = [lax.rsqrt(q.mean() + EPS) for q in a]
        m = [q.astype(bf16).astype(f32) for q in m]
        a = [_Acc(nch) for _ in ts]
        b = [_Acc(nch) for _ in ts]
        rows = [[] for _ in ts]
        for d in range(DH):
            for i in range(nt):
                xu = _pk(((xrow(2, d, i) - m[i]) * r[i]).astype(bf16))
                xnT[slot + i, d * 8:(d + 1) * 8, :] = xu
                rows[i].append(xu)
                xf = _upk(xu).astype(f32)
                a[i].add(xf)
                b[i].add(xf * xf)
        m2 = [q.mean() for q in a]
        r2 = [lax.rsqrt(jnp.maximum(q.mean() - mm * mm, 0.0) + EPS) for q, mm in zip(b, m2)]
        m2 = [q.astype(bf16).astype(f32) for q in m2]

        def hrow(d, i, dp):
            xf = tie(_upk(xnT[slot + i, pl.ds(z + d * 8, 8), :]).astype(f32), dp)
            return (xf - m2[i]) * r2[i]

        if pair is None:
            for d in range(DH):
                for i in range(nt):
                    hT[d * 8:(d + 1) * 8, :] = _pk(hrow(d, i, dep(3, d, i)).astype(bf16))
        else:
            for d in range(HG):
                dp = dep(3, 2 * d, 0)
                ops = _lhs7(hrow(d, 0, dp), hrow(d, 1, dp), hrow(HG + d, 0, dp), hrow(HG + d, 1, dp))
                for q in range(7):
                    ha[q, d * 8:(d + 1) * 8, :] = _pk(ops[q])
        if transpose:
            for i in range(nt):
                to_rows(put_xn, ts[i], jnp.concatenate(rows[i], axis=0))

    def prep_t(cs, pts):
        cs = list(cs)
        for ci, c in enumerate(cs):
            wd = min(128, 3 * D - c * 128)
            w = wqkv_v[:, c * 128:c * 128 + wd]
            if wd < 128:
                w = jnp.concatenate([w, jnp.zeros((D, 128 - wd), bf16)], axis=1)
            w = pltpu.bitcast(w, f32)
            per = len(pts) / (len(cs) + 1)
            w = [tie(_rows16(w, r), pts[int((ci + r / HG) * per)]) for r in range(HG)]
            w = _cat(w + w[-2:], axis=0)
            wt = _upk(w).T.astype(f32)
            for k in range(KT):
                for h in range(0, wd, H):
                    p, r = divmod(c * 128 + h, D)
                    pt = pts[int((ci + 1 + (k * 128 + h) / DP) * per)]
                    wtmp[p][k, r:r + H, :] = tie(wt[h:h + H, k * 128:(k + 1) * 128], pt)

    def wrows(p, d, k):
        return wtmp[p][k, pl.ds(d, H, stride=DH), :]

    def prep_part(n, pts):
        p = PARTS[n]
        prep_t(PTILES[p], _win(pts, 0, PW[0]))
        pts = _win(pts, PW[1], PW[2])
        for d in range(HG):
            pt = [pts[((d * 2 + c) * len(pts)) // (2 * HG)] for c in range(2)]
            ops = _lhs13([tie(wrows(p, d, k), pt[k // 2]) for k in range(KT)],
                         [tie(wrows(p, HG + d, k), pt[k // 2]) for k in range(KT)], lo)
            r = (n * HM + d * H) // 2
            for q in range(13):
                l_s[q, r:r + 8, :] = _pk(ops[q])

    def prep_wo(pts):
        p1, p2, p3 = _win(pts, 0, 30), _win(pts, 30, 62), _win(pts, 66, 100)
        wo = jnp.concatenate([wo_v[...].astype(f32), jnp.zeros((D, DP - D), f32)], axis=1)
        for k in range(KT):
            for d in range(DH):
                wtmp2[k, d * H:(d + 1) * H, :] = tie(wo[d * H:(d + 1) * H, k * 128:(k + 1) * 128],
                                                     p1[((k * DH + d) * len(p1)) // (KT * DH)])
        parts = []
        for k in range(KT):
            rows = [_pk(tie(wtmp2[k, pl.ds(d, H, stride=DH), :],
                            p2[((k * DH + d) * len(p2)) // (KT * DH)]).astype(bf16)) for d in range(DH)]
            parts.append(jnp.concatenate(rows + rows[-4:], axis=0))
        wt = _upk(jnp.concatenate(parts, axis=1)).T
        for d in range(HG):
            def a(i, k):
                w = wt[(i * HG + d) * H:(i * HG + d + 1) * H, k * 128:(k + 1) * 128]
                return tie(w.astype(f32), p3[((d * 2 + k // 2) * len(p3)) // (2 * HG)])
            ops = _lhs13([a(0, k) for k in range(KT)], [a(1, k) for k in range(KT)], lo)
            for q in range(13):
                wa[q, pl.ds((z0 if WOP != -1 else 0) + d * 8, 8), :] = _pk(ops[q])

    def mix1(t, n0=0, n1=NF):
        lhs = _upk(hT[...])
        if (n1 - n0) % 4 == 0:
            part = _dot(lhs, w1_v[_tiles(t), n0 * 128:n1 * 128])
        else:
            main = _dot(lhs, w1_v[_tiles(t), n0 * 128:(n1 - 2) * 128])
            wl = w1_v[_tiles(t), (n1 - 2) * 128:n1 * 128]
            tail = [_dot(lhs[h * HM:(h + 1) * HM, :], wl) for h in range(2)]
            part = jnp.concatenate([main, jnp.concatenate(tail, axis=0)], axis=1)
        return part, _interleave([part[:, n * 128:(n + 1) * 128] for n in range(n1 - n0)], 4)

    def mix1_pair(p, dst, z, split, copy):
        ms = []
        hr = HM // 2
        for i in range(7):
            if copy:
                hb[pl.ds(z0 + i * hr, hr), :] = ha[i]
        for q in range(NF // 2):
            wb = [w1_v[_tiles(2 * p + i), (2 * q + j) * 128:(2 * q + j + 1) * 128]
                  for i in range(2) for j in range(2)]
            rhs = _rhs7(*[w.astype(f32) for w in wb])
            rhs[1], rhs[4] = wb[0], wb[3]
            m, c = _strassen(lambda i: _upk(hb[i * hr:(i + 1) * hr, :] if (copy and q > 0) else ha[i]), lambda i: rhs[i],
                             _dot, split if q == NF // 2 - 1 else None)
            ms += m
            for n in (1, 0, 2, 3):
                cb = c[n]
                cols = slice((2 * q + n // 2) * 128, (2 * q + n // 2 + 1) * 128)
                r0 = (n % 2) * HM
                dst[pl.ds(z + r0, HM), cols] = u_acc[r0:r0 + HM, cols] + cb
        return _interleave(ms, 4)

    ln_tiles([0], slot=3, transpose=False)
    start(range(4, NG))
    _wait(group(1))
    u_acc[:, 0:N0 * 128] = mix1(0, 0, N0)[0]
    to_rows(put_xn, 0, xnT[3])
    _wait(group(2))
    part, pts = mix1(0, N0, NF)
    u_acc[:, N0 * 128:] = part
    ln_tiles([1], pts)

    def step_a(i, z):
        _wait(group_a(i))
        part, pts = mix1(i)
        u_acc[...] += part
        ln_tiles([i + 1], pts, pl.multiple_of(z * 64, 64))
        return (i - 1) * (i - 2)

    zi = lax.fori_loop(1, 3, step_a, 0)
    z0 = pl.multiple_of(zi * 64, 64)
    _wait(group(5))
    part, pts = mix1(3)
    u_acc[...] += part
    ln_tiles([4, 5], pts, z0, pair=0)

    def step_b(i, carry):
        _wait(group_b(i))
        pts = mix1_pair(2 + i, u_acc, 0, (0, 64, 128, 176, HM), True)
        ln_tiles([6 + 2 * i, 7 + 2 * i], pts, z0, pair=1 + i)
        return carry

    lax.fori_loop(0, 5, step_b, 0)
    _wait(group(11))
    pts = mix1_pair(7, u_fin, z0 if UZ else 0, None, False)
    pts_last = pts
    prep_part(0, pts)
    b1 = b1_v[...].astype(f32)

    def gelu_cols(cs, pts):
        cs = list(cs)
        for ci, c in enumerate(cs):
            for d in range(HG):
                def g(i, j):
                    pt = pts[(((ci * HG + d) * 4 + 2 * i + j) * len(pts)) // (len(cs) * HG * 4)]
                    n = j * (NF // 2) + c
                    u = tie(u_fin[(i * HG + d) * H:(i * HG + d + 1) * H, n * 128:(n + 1) * 128], pt)
                    return _gelu(u + b1[n:n + 1, :]) if GF else jax.nn.gelu(u + b1[n:n + 1, :], approximate=True)
                ops = _lhs7(g(0, 0), g(0, 1), g(1, 0), g(1, 1))
                for q in range(7):
                    ga[q, d * 8:(d + 1) * 8, c * 128:(c + 1) * 128] = _pk(ops[q])

    order = list(range(NB - (W - 1), NB)) + list(range(NB - (W - 1)))

    def put_part(j, p, r0, v):
        z = z0 if order.index(j) >= 10 else 0
        qkv[j][pl.ds(z + p * D + r0, v.shape[0]), :] = v
        if j >= NB - (W - 1) and p > 0:
            kvr[j - (NB - (W - 1))][pl.ds((p - 1) * D + r0, v.shape[0]), :] = pltpu.roll(v, 2, axis=1)

    def nt_sums(dst, rows, pts):
        for g in range(8):
            pt = [pts[((2 * g + c) * len(pts)) // 16] for c in range(2)]
            b, c = [[_rows16(rows(j, k), g).astype(f32) for k in range(KT)] for j in range(2)]
            b[0], c[1], b[2] = tie(b[0], pt[0]), tie(c[1], pt[0]), tie(b[2], pt[1])
            ops = _rhs10(b, c, lo)
            for i in (0, 2, 3, 5, 6, 7, 8, 9):
                dst[i, g * H:(g + 1) * H, :] = ops[i]

    mxu = _Rounds(49)
    cut1 = [None]

    def nt_product(lhs, dst, rows):
        def mm(a, b, brief):
            if cut1[0] is not None:
                cuts, cut1[0] = cut1[0], None
                mxu.add(4)
                return _cat([_dot_nt(a[r0:r1, :], b) for r0, r1 in zip(cuts[:-1], cuts[1:])], axis=0)
            m = _dot_nt(a, b)
            mxu.add(1, m if brief else None)
            return m
        return _mm13(lhs, lambda i: rows(i // 4, i // 4) if i in (1, 4) else dst[i], mm)

    def xr(j, k):
        return _upk(xn_u[k, pl.ds(PJ * j, 64, stride=PL), :])

    def qkv_part(t, n):
        js = order[2 * t:2 * t + 2]
        c = nt_product(lambda i: _upk(l_s[i, n * HM // 2:(n + 1) * HM // 2, :]), xs[t], lambda j, k: xr(js[j], k))
        for q in (1, 0, 2, 3):
            put_part(js[q // 2], PARTS[n], (q % 2) * HM, c[q])

    def qkv_quad(n):
        qkv_part(0, n)
        qkv_part(1, n)
        return mxu.take()

    def qkv_pair(t):
        for n in range(3):
            qkv_part(t, n)
        return mxu.take()

    def x_sums(t, pts):
        nt_sums(xs[t], lambda j, k: xr(order[2 * t + j], k), pts)

    def w2_sums(p, pts):
        def strip(r):
            top = w2_v[r * H:(r + 1) * H, _tiles(2 * p, 2)].astype(f32)
            bot = w2_v[F // 2 + r * H:F // 2 + (r + 1) * H, _tiles(2 * p, 2)].astype(f32)
            return top[:, 0:128], top[:, 128:], bot[:, 0:128], bot[:, 128:]
        rhs_sums(w2s[p], strip, F // 2 // H, pts, range(7))

    edge = lax.broadcasted_iota(jnp.int32, (H, 128), 1) < 2
    scale = DH ** -0.5

    def attn_block(j, pts, pace_sm):
        n_sm = (len(pts) * SMF) // 100
        half = (len(pts) - n_sm) // 2

        def kv_rows(w, p, d):
            if j >= w:
                return qkv[j - w][pl.ds(p * D + d * H, H), :]
            return kvr[j - w + (W - 1)][pl.ds((p - 1) * D + d * H, H), :]

        def sm(v, f):
            return tie(v, pts[half + (f * n_sm) // 20]) if pace_sm else v

        acc = [None] * W
        for d in range(DH):
            qd = tie(qkv[j][pl.ds(d * H, H), :], pts[(d * half) // DH])
            for w in range(W):
                t = qd * kv_rows(w, 1, d)
                acc[w] = t if acc[w] is None else acc[w] + t
        lg = [jnp.where(edge, -1e9 / scale, acc[w]) if w > j else acc[w] for w in range(W)]
        m = sm(_tree(jnp.maximum, lg), 2)
        e = [jnp.exp2(sm((l - m) * (scale * LOG2E), 4 + 2 * (w // 2))) for w, l in enumerate(lg)]
        ssum = sm(_tree(jnp.add, e), 14)
        inv = pl.reciprocal(ssum, approx=True)
        inv = sm(inv * (2.0 - ssum * inv), 18)
        a = [ew * inv for ew in e]
        for d in range(DH):
            o = a[0] * kv_rows(0, 2, d)
            for w in range(1, W):
                o = o + a[w] * kv_rows(w, 2, d)
            ob = tie(o, pts[half + n_sm + (d * half) // DH]).astype(bf16)
            oT[j][pl.ds(z0 + d * 8, 8), :] = _pk(ob)

    def last_wait(i, carry):
        _wait(group(12))
        return carry

    x_sums(0, _win(pts_last, XW[0], XW[1]))
    x_sums(1, _win(pts_last, XW[2], XW[3]))
    prep_part(1, qkv_quad(0))
    prep_part(2, qkv_quad(1))
    pts = qkv_quad(2)
    x_sums(2, _win(pts, 0, 20))
    gelu_cols((0,), _win(pts, 20, 100))
    mid = []
    for t in range(2, NB // 2):
        pts = qkv_pair(t)
        mid += pts
        if WOP == -1 and t == 4:
            prep_wo(_win(mid, 0, 92))
        if WOP == -2 and t == NB // 2 - 1:
            prep_wo(mid[n4:])
        if t + 1 < NB // 2:
            x_sums(t + 1, _win(pts, 0, 12 if t <= 4 else 70))
            pts = _win(pts, 12, 100)
        else:
            w2_sums(0, _win(mid[n4:], 0, 95) if W0S else _win(pts, 0, 88))
        if t <= 4:
            gelu_cols((2 * t - 3, 2 * t - 2), _win(pts, 0, 100 if t < 4 else 94))
        if t == 4:
            lax.fori_loop(0, 1 + zi, last_wait, 0)
            cut1[0] = (0, 48, 96, 160, HM)
            n4 = len(mid)

    b2 = b2_v[...].astype(f32)

    def dot_rounds(a, b):
        k, nk, acc = 0, a.shape[1] // 128, None
        while k < nk:
            n = min(4 - mxu.n % 4, nk - k)
            if n > 1:
                p = _dot(a[:, k * 128:(k + n - 1) * 128], b[k * 128:(k + n - 1) * 128, :])
                acc = p if acc is None else acc + p
            p = _dot(a[:, (k + n - 1) * 128:(k + n) * 128], b[(k + n - 1) * 128:(k + n) * 128, :])
            mxu.add(n, None if acc is None else p)
            acc = p if acc is None else acc + p
            k += n
        return acc

    def mix2_pair(p):
        _, c = _strassen(lambda i: _upk(ga[i]), lambda i: w2s[p][i], dot_rounds)
        pts = mxu.take()
        if p + 1 < NB // 2 - W7:
            w2_sums(p + 1, _win(pts, W2A, W2B))
        return pts, c

    def o_rows(n, k):
        return _upk(_cat([o_u[k, pl.ds(PL * (n * 4 + i), NB, stride=PJ), :] for i in range(4)], axis=0))

    def o_sums(p, pts):
        nt_sums(os_[p], lambda j, k: o_rows(2 * p + j, k), pts)

    def send(r0, r1, cols):
        pltpu.make_async_copy(out_v.at[r0:r1, cols], out_hbm.at[0, r0:r1, cols], sems.at[0]).start()

    late = []

    def wo_pair(p):
        c = nt_product(lambda i: _upk(wa[i]), os_[p], lambda j, k: o_rows(2 * p + j, k))
        pts = mxu.take()
        late.extend(pts)
        if p + 2 < NB // 2:
            o_sums(p + 2, pts)
        if W7 and p == NB // 2 - 2:
            w2_sums(NB // 2 - 1, late)
        return c

    def store_pair(p, first, second):
        last = p == NB // 2 - 1
        for q in (1, 0, 2, 3):
            n, r0 = 2 * p + q // 2, (q % 2) * HM
            res = ((x_v[n, r0:r0 + HM, :].astype(f32) + b2[n:n + 1, :] + first(q)) + second(q)).astype(bf16)
            if last and q == 3:
                for a, b in LASTR:
                    out_v[r0 + a:r0 + b, _tiles(n)] = res[a:b, :]
                    send(r0 + a, r0 + b, _tiles(n))
            else:
                out_v[r0:r0 + HM, _tiles(n)] = res
                if last:
                    send(r0, r0 + HM, _tiles(n))
        if not last:
            send(0, D, _tiles(2 * p, 2))

    pts = []
    for p in range(NPRE):
        pp, c = mix2_pair(p)
        for q in range(4):
            y_v[4 * p + q] = c[q]
        pts += _win(pp, W2B, 100) if (SEQ and p < NPRE - 1) else pp
    if WOP >= 0:
        prep_wo(pts[WOP * 171:(WOP + WON) * 171])
    line = mid[n4:] + pts
    pos = 0
    for j in range(NB):
        n = PPA if pos < len(mid) - n4 - PPA // 2 else PPB
        attn_block(j, line[pos:pos + n], True)
        pos += n
    for j in range(NB):
        to_rows(put_o, j, oT[j][...])
    o_sums(0, pts[-5 * HG:-3 * HG])
    o_sums(1, pts[-3 * HG:-HG])
    for p in range(NPRE):
        c = wo_pair(p)
        store_pair(p, lambda q: y_v[4 * p + q], lambda q: c[q])
    for p in range(NPRE, NB // 2):
        c = wo_pair(p)
        _, y = mix2_pair(p)
        store_pair(p, lambda q: c[q], lambda q: y[q])
    _wait([pltpu.make_async_copy(out_v, out_hbm.at[0], sems.at[0])])


@jax.jit
def pallas_parallel_sum__sliding_local_dilated__mixer_token_mlp__prompt_kernel(
        A_x, A_wqkv, A_wo, B_x, B_w1, B_b1, B_w2, B_b2):
    any_spec = pl.BlockSpec(memory_space=pl.ANY)
    out_t = pl.pallas_call(
        _kernel,
        out_shape=jax.ShapeDtypeStruct((1, D, S), bf16),
        in_specs=[any_spec] * 7,
        out_specs=any_spec,
        scratch_shapes=[
            pltpu.VMEM((NB, D, 128), bf16),
            pltpu.VMEM((D, 3 * D), bf16),
            pltpu.VMEM((D, D), bf16),
            pltpu.VMEM((S, F), bf16),
            pltpu.VMEM((F, S), bf16),
            pltpu.VMEM((NF, 128), bf16),
            pltpu.VMEM((NB, 128), bf16),
            pltpu.VMEM((D // 2, 128), u32),
            pltpu.VMEM((7, HM // 2, 128), u32),
            pltpu.VMEM((7 * HM // 2, 128), u32),
            pltpu.VMEM((4, D // 2, 128), u32),
            pltpu.VMEM((KT, PROWS, 128), u32),
            pltpu.VMEM((D, F), f32),
            pltpu.VMEM((D, F), f32),
            pltpu.VMEM((7, HM // 2, F // 2), u32),
            pltpu.VMEM((13, HM // 2, 128), u32),
            pltpu.VMEM((KT, D + 32, 128), f32),
            pltpu.VMEM((KT, D + 32, 128), f32),
            pltpu.VMEM((KT, D + 32, 128), f32),
            pltpu.VMEM((KT, D + 32, 128), f32),
            pltpu.VMEM((13, MS // 2, 128), u32),
            pltpu.VMEM((KT, PROWS, 128), u32),
            pltpu.VMEM((4 * NPRE, HM, 128), f32),
            pltpu.VMEM((D, S), bf16),
            pltpu.SemaphoreType.DMA((NG,)),
        ] + [pltpu.VMEM((3 * D, 128), f32)] * NB + [pltpu.VMEM((2 * D, 128), f32)] * (W - 1)
          + [pltpu.VMEM((D // 2, 128), u32)] * NB + [pltpu.VMEM((7, F // 2, 128), bf16)] * 8
          + [pltpu.VMEM((10, 128, 128), bf16)] * 16,
        compiler_params=pltpu.CompilerParams(vmem_limit_bytes=100 * 2**20, disable_semaphore_checks=True),
    )(jnp.swapaxes(A_x, 1, 2), A_wqkv, A_wo, B_w1, B_b1.reshape(NF, 128), B_w2, B_b2.reshape(NB, 128))
    return jnp.swapaxes(out_t, 1, 2)
```

```python
import jax
import jax.numpy as jnp
from jax import lax
import jax.experimental.pallas as pl
import jax.experimental.pallas.tpu as pltpu

S, D, F = 2048, 448, 1792
H, DH, W = 16, 28, 8
EPS = 1e-5
LOG2E = 1.4426950408889634
NB = S // 128
NF = F // 128
DP = 512
KT = DP // 128
HM = D // 2
HG = HM // H
PJ, PL = 132, 2
PROWS = PJ * NB + 128
NG = 13
N0 = 6
NPRE = 7
PPA, PPB = 134, 67
SKIP = (6, 7, 8)
KEEP = HG - len(SKIP)
LASTR = ((0, 128), (128, 192), (192, 224))
LNW = ((0, 21, 42, 64, 85), (0, 14, 32, 58, 90), (0, 18, 38, 62, 88))
PTILES = ((0, 1, 2, 3), (4, 5, 6), (7, 8, 9, 10))
bf16, f32, u32 = jnp.bfloat16, jnp.float32, jnp.uint32
NT = (((1,), (1,)), ((), ()))


def _wait(cps):
    for cp in cps:
        cp.wait()


def _cat(parts, axis=1):
    return parts[0] if len(parts) == 1 else jnp.concatenate(parts, axis=axis)


def _pk(x):
    return pltpu.bitcast(x, u32)


def _upk(x):
    return pltpu.bitcast(x, bf16)


def _tiles(t, n=1):
    if isinstance(t, int):
        return pl.ds(t * 128, n * 128)
    return pl.ds(pl.multiple_of(t * 128, 128), n * 128)


def _tree(op, xs):
    xs = list(xs)
    while len(xs) > 1:
        xs = [op(xs[i], xs[i + 1]) for i in range(0, len(xs), 2)]
    return xs[0]


def _rows16(v, d):
    return v[d * H:(d + 1) * H, :]


def _groups(v):
    return [_rows16(v, d) for d in range(v.shape[0] // H)]


def _win(pts, a, b):
    return pts[(len(pts) * a) // 100:(len(pts) * b) // 100]


def _gelu(x):
    c = 0.7978845608028654
    h = 0.5 * x
    return h + h * jnp.tanh(x * (c + (c * 0.044715) * (x * x)))


def _dot(a, b):
    return jnp.dot(a, b, preferred_element_type=f32)


def _dot_nt(a, b):
    return lax.dot_general(a, b, NT, preferred_element_type=f32)


def _lhs7(a11, a12, a21, a22):
    return [v.astype(bf16) for v in (a11 + a22, a21 + a22, a11, a22, a11 + a12, a21 - a11, a12 - a22)]


def _rhs7(b11, b12, b21, b22):
    return [v.astype(bf16) for v in (b11 + b22, b11, b12 - b22, b21 - b11, b22, b11 + b12, b21 + b22)]


def _strassen(lhs, rhs, mm, split=None):
    m2 = mm(lhs(1), rhs(1))
    m4 = mm(lhs(3), rhs(3))
    c21 = m2 + m4
    m7 = mm(lhs(6), rhs(6))
    c11 = m4 + m7
    m5 = mm(lhs(4), rhs(4))
    c11 = c11 - m5
    m1 = mm(lhs(0), rhs(0))
    c11 = c11 + m1
    c22 = m1 - m2
    m3 = mm(lhs(2), rhs(2))
    c12 = m5 + m3
    c22 = c22 + m3
    a6, b6 = lhs(5), rhs(5)
    if split is None:
        m6 = mm(a6, b6)
    else:
        m6 = jnp.concatenate([mm(a6[r0:r1, :], b6) for r0, r1 in zip(split[:-1], split[1:])], axis=0)
    return [m2, m4, m7, m5, m1, m3, m6], (c11, c21, c12, c22 + m6)


def _lhs13(top, bot, lo):
    rest = (jnp.where(lo, -top[2], top[2]), jnp.where(lo, bot[2], -bot[2]),
            jnp.where(lo, top[3], top[2]), jnp.where(lo, bot[3], bot[2]),
            jnp.where(lo, top[2], top[3]), jnp.where(lo, bot[2], bot[3]))
    return _lhs7(top[0], top[1], bot[0], bot[1]) + [v.astype(bf16) for v in rest]


def _rhs10(b, c, lo):
    t = b[2] + c[2]
    rest = (jnp.where(lo, b[2], c[2]), jnp.where(lo, b[3], t), jnp.where(lo, t, c[3]))
    return _rhs7(b[0], c[0], b[1], c[1]) + [v.astype(bf16) for v in rest]


def _mm13(lhs, rhs, mm):
    def p(i, j):
        return mm(lhs(i), rhs(j), i in (5, 6, 7, 8, 9, 10, 11, 12))
    p2 = p(1, 1)
    p2 = p2 + p(8, 7)
    c21 = p2 + p(10, 8)
    m4 = p(3, 3)
    c21 = c21 + m4
    c11 = m4 + p(6, 6)
    c11 = c11 + p(9, 8)
    p5 = p(4, 4)
    p5 = p5 + p(7, 7)
    c11 = c11 - p5
    m1 = p(0, 0)
    c11 = c11 + m1
    c22 = m1 - p2
    m3 = p(2, 2)
    c22 = c22 + m3
    c12 = p5 + m3
    c12 = c12 + p(11, 9)
    c22 = c22 + p(5, 5)
    c22 = c22 + p(12, 9)
    return c11, c21, c12, c22


class _Rounds:
    def __init__(self, n):
        self.n = n
        self.res = {}

    def add(self, n, m=None):
        if m is not None:
            self.res.setdefault((self.n + n - 1) // 4, m)
        self.n += n

    def take(self, skip=()):
        pts = [g for r in sorted(self.res) if self.res[r] is not None
               for n, g in enumerate(_groups(self.res[r])) if n not in skip]
        self.res = {max(self.res): None}
        return pts


def _interleave(ms, par):
    return [_rows16(m, d) for i in range(0, len(ms), par) for d in range(ms[0].shape[0] // H)
            for m in ms[i:i + par]]


class _Acc:
    def __init__(self, n):
        self.p = [None] * n
        self.i = 0

    def add(self, v):
        k = self.i % len(self.p)
        self.p[k] = v if self.p[k] is None else self.p[k] + v
        self.i += 1

    def mean(self):
        t = self.p[0]
        for q in self.p[1:]:
            t = t + q
        return jnp.sum(t, axis=0, keepdims=True) * (1.0 / D)


def _kernel(x_hbm, wqkv_hbm, wo_hbm, w1_hbm, b1_hbm, w2_hbm, b2_hbm, out_hbm,
            x_v, wqkv_v, wo_v, w1_v, w2_v, b1_v, b2_v, hT, ha, hb, xnT, xn_u, u_acc, u_fin, ga, wa,
            wt0, wt1, wt2, wtmp2, l_s, o_u, y_v, out_v, sems, *blk):
    wtmp = (wt0, wt1, wt2)
    qkv = blk[0:NB]
    kvr = blk[NB:NB + W - 1]
    oT = blk[NB + W - 1:2 * NB + W - 1]
    w2s = blk[2 * NB + W - 1:2 * NB + W + 7]
    xs = blk[2 * NB + W + 7:2 * NB + W + 15]
    os_ = blk[2 * NB + W + 15:]

    def cp_x(t, n, sem):
        return [pltpu.make_async_copy(x_hbm.at[0, :, _tiles(t + q)], x_v.at[t + q], sem) for q in range(n)]

    def cp_w1(t, n, sem):
        return [pltpu.make_async_copy(w1_hbm.at[_tiles(t, n), :], w1_v.at[_tiles(t, n), :], sem)]

    def group_a(i):
        return cp_x(1 + i, 1, sems.at[2 + i]) + cp_w1(i, 1, sems.at[2 + i])

    def group_b(i):
        return cp_x(6 + 2 * i, 2, sems.at[6 + i]) + cp_w1(4 + 2 * i, 2, sems.at[6 + i])

    def group(g):
        sem = sems.at[g]
        if g == 0:
            return cp_x(0, 1, sem)
        if g == 1:
            return [pltpu.make_async_copy(w1_hbm.at[0:128, 0:N0 * 128], w1_v.at[0:128, 0:N0 * 128], sem)]
        if g == 2:
            return cp_x(1, 1, sem) + [
                pltpu.make_async_copy(w1_hbm.at[0:128, N0 * 128:], w1_v.at[0:128, N0 * 128:], sem)]
        if g < 5:
            return group_a(g - 2)
        if g == 5:
            return cp_x(4, 2, sem) + cp_w1(3, 1, sem)
        if g < 11:
            return group_b(g - 6)
        if g == 11:
            return cp_w1(14, 2, sem) + [pltpu.make_async_copy(wqkv_hbm, wqkv_v, sem),
                                        pltpu.make_async_copy(b1_hbm, b1_v, sem),
                                        pltpu.make_async_copy(wo_hbm, wo_v, sem)]
        return [pltpu.make_async_copy(b2_hbm, b2_v, sem),
                pltpu.make_async_copy(w2_hbm, w2_v, sem)]

    def start(gs):
        for g in gs:
            for cp in group(g):
                cp.start()

    start(range(4))
    _wait(group(0))
    never = x_v[0, 0:H, :].astype(f32) > jnp.inf

    lo = lax.broadcasted_iota(jnp.int32, (H, 128), 1) < 64

    def tie(x, dep):
        return x if dep is None else jnp.where(never, dep, x)

    def rhs_sums(dst, strip, n, pts, which):
        for r in range(n):
            pt = pts[(r * len(pts)) // n]
            b11, b12, b21, b22 = strip(r)
            ops = _rhs7(tie(b11, pt), b12, b21, tie(b22, pt))
            for i in which:
                dst[i, r * H:(r + 1) * H, :] = ops[i]

    def to_rows(dst, j, packed):
        t = _upk(jnp.concatenate([packed, packed[(2 * D - DP) // 2:, :]], axis=0)).T
        for k in range(KT):
            dst(k, j, _pk(t[:, k * 128:(k + 1) * 128]))

    def put_xn(k, t, w):
        for q in range(4):
            xn_u[k, pl.ds(PL * (t * 4 + q), NB, stride=PJ), :] = w[q * NB:(q + 1) * NB, :]

    def put_o(k, j, w):
        o_u[k, pl.ds(PJ * j, 64, stride=PL), :] = w

    def ln_tiles(ts, pts=None, z=0, slot=0, transpose=True, win=0):
        nt = len(ts)
        nch = 2 if pts is not None else 4
        cut = LNW[win]

        def dep(p, d, i):
            if pts is None:
                return None
            f = cut[p] + (cut[p + 1] - 2 - cut[p]) * (d * nt + i) / (DH * nt)
            return pts[int(f * len(pts) / 100)]

        def xrow(p, d, i):
            return tie(x_v[ts[i], d * H:(d + 1) * H, :].astype(f32), dep(p, d, i))

        a = [_Acc(nch) for _ in ts]
        for d in range(DH):
            for i in range(nt):
                a[i].add(xrow(0, d, i))
        m = [q.mean() for q in a]
        a = [_Acc(nch) for _ in ts]
        for d in range(DH):
            for i in range(nt):
                c = xrow(1, d, i) - m[i]
                a[i].add(c * c)
        r = [lax.rsqrt(q.mean() + EPS) for q in a]
        m = [q.astype(bf16).astype(f32) for q in m]
        a = [_Acc(nch) for _ in ts]
        b = [_Acc(nch) for _ in ts]
        rows = [[] for _ in ts]
        for d in range(DH):
            for i in range(nt):
                xu = _pk(((xrow(2, d, i) - m[i]) * r[i]).astype(bf16))
                xnT[slot + i, d * 8:(d + 1) * 8, :] = xu
                rows[i].append(xu)
                xf = _upk(xu).astype(f32)
                a[i].add(xf)
                b[i].add(xf * xf)
        m2 = [q.mean() for q in a]
        r2 = [lax.rsqrt(jnp.maximum(q.mean() - mm * mm, 0.0) + EPS) for q, mm in zip(b, m2)]
        m2 = [q.astype(bf16).astype(f32) for q in m2]

        def hrow(d, i, dp):
            xf = tie(_upk(xnT[slot + i, pl.ds(z + d * 8, 8), :]).astype(f32), dp)
            return (xf - m2[i]) * r2[i]

        if nt == 1:
            for d in range(DH):
                hT[d * 8:(d + 1) * 8, :] = _pk(hrow(d, 0, dep(3, d, 0)).astype(bf16))
        else:
            for d in range(HG):
                dp = dep(3, 2 * d, 0)
                ops = _lhs7(hrow(d, 0, dp), hrow(d, 1, dp), hrow(HG + d, 0, dp), hrow(HG + d, 1, dp))
                for q in range(7):
                    ha[q, d * 8:(d + 1) * 8, :] = _pk(ops[q])
        if transpose:
            for i in range(nt):
                to_rows(put_xn, ts[i], jnp.concatenate(rows[i], axis=0))

    def prep_t(cs, pts):
        cs = list(cs)
        for ci, c in enumerate(cs):
            wd = min(128, 3 * D - c * 128)
            w = wqkv_v[:, c * 128:c * 128 + wd]
            if wd < 128:
                w = jnp.concatenate([w, jnp.zeros((D, 128 - wd), bf16)], axis=1)
            w = pltpu.bitcast(w, f32)
            per = len(pts) / (len(cs) + 1)
            w = [tie(_rows16(w, r), pts[int((ci + r / HG) * per)]) for r in range(HG)]
            w = _cat(w + w[-2:], axis=0)
            wt = _upk(w).T.astype(f32)
            for k in range(KT):
                for h in range(0, wd, H):
                    p, r = divmod(c * 128 + h, D)
                    pt = pts[int((ci + 1 + (k * 128 + h) / DP) * per)]
                    wtmp[p][k, r:r + H, :] = tie(wt[h:h + H, k * 128:(k + 1) * 128], pt)

    def wrows(p, d, k):
        return wtmp[p][k, pl.ds(d, H, stride=DH), :]

    def prep_part(p, pts):
        prep_t(PTILES[p], _win(pts, 0, 50))
        pts = _win(pts, 55, 92)
        for d in range(HG):
            pt = [pts[((d * 2 + c) * len(pts)) // (2 * HG)] for c in range(2)]
            ops = _lhs13([tie(wrows(p, d, k), pt[k // 2]) for k in range(KT)],
                         [tie(wrows(p, HG + d, k), pt[k // 2]) for k in range(KT)], lo)
            r = (p * HM + d * H) // 2
            for q in range(13):
                l_s[q, r:r + 8, :] = _pk(ops[q])

    def prep_wo(pts):
        p1, p2, p3 = _win(pts, 0, 30), _win(pts, 30, 62), _win(pts, 66, 100)
        wo = jnp.concatenate([wo_v[...].astype(f32), jnp.zeros((D, DP - D), f32)], axis=1)
        for k in range(KT):
            for d in range(DH):
                wtmp2[k, d * H:(d + 1) * H, :] = tie(wo[d * H:(d + 1) * H, k * 128:(k + 1) * 128],
                                                     p1[((k * DH + d) * len(p1)) // (KT * DH)])
        parts = []
        for k in range(KT):
            rows = [_pk(tie(wtmp2[k, pl.ds(d, H, stride=DH), :],
                            p2[((k * DH + d) * len(p2)) // (KT * DH)]).astype(bf16)) for d in range(DH)]
            parts.append(jnp.concatenate(rows + rows[-4:], axis=0))
        wt = _upk(jnp.concatenate(parts, axis=1)).T
        for d in range(HG):
            def a(i, k):
                w = wt[(i * HG + d) * H:(i * HG + d + 1) * H, k * 128:(k + 1) * 128]
                return tie(w.astype(f32), p3[((d * 2 + k // 2) * len(p3)) // (2 * HG)])
            ops = _lhs13([a(0, k) for k in range(KT)], [a(1, k) for k in range(KT)], lo)
            for q in range(13):
                wa[q, pl.ds(z0 + d * 8, 8), :] = _pk(ops[q])

    def mix1(t, n0=0, n1=NF):
        lhs = _upk(hT[...])
        if (n1 - n0) % 4 == 0:
            part = _dot(lhs, w1_v[_tiles(t), n0 * 128:n1 * 128])
        else:
            main = _dot(lhs, w1_v[_tiles(t), n0 * 128:(n1 - 2) * 128])
            wl = w1_v[_tiles(t), (n1 - 2) * 128:n1 * 128]
            tail = [_dot(lhs[h * HM:(h + 1) * HM, :], wl) for h in range(2)]
            part = jnp.concatenate([main, jnp.concatenate(tail, axis=0)], axis=1)
        return part, _interleave([part[:, n * 128:(n + 1) * 128] for n in range(n1 - n0)], 4)

    def mix1_pair(p, dst, split, copy):
        ms = []
        hr = HM // 2
        for i in range(7):
            if copy:
                hb[pl.ds(z0 + i * hr, hr), :] = ha[i]
        for q in range(NF // 2):
            wb = [w1_v[_tiles(2 * p + i), (2 * q + j) * 128:(2 * q + j + 1) * 128]
                  for i in range(2) for j in range(2)]
            rhs = _rhs7(*[w.astype(f32) for w in wb])
            rhs[1], rhs[4] = wb[0], wb[3]
            m, c = _strassen(lambda i: _upk(hb[i * hr:(i + 1) * hr, :] if (copy and q > 0) else ha[i]), lambda i: rhs[i],
                             _dot, split if q == NF // 2 - 1 else None)
            ms += m
            for n in (1, 0, 2, 3):
                cb = c[n]
                cols = slice((2 * q + n // 2) * 128, (2 * q + n // 2 + 1) * 128)
                r0 = (n % 2) * HM
                dst[r0:r0 + HM, cols] = u_acc[r0:r0 + HM, cols] + cb
        return _interleave(ms, 4)

    ln_tiles([0], slot=3, transpose=False)
    start(range(4, NG))
    _wait(group(1))
    u_acc[:, 0:N0 * 128] = mix1(0, 0, N0)[0]
    to_rows(put_xn, 0, xnT[3])
    _wait(group(2))
    part, pts = mix1(0, N0, NF)
    u_acc[:, N0 * 128:] = part
    ln_tiles([1], pts)

    def step_a(i, z):
        _wait(group_a(i))
        part, pts = mix1(i)
        u_acc[...] += part
        ln_tiles([i + 1], pts, pl.multiple_of(z * 64, 64))
        return (i - 1) * (i - 2)

    zi = lax.fori_loop(1, 3, step_a, 0)
    z0 = pl.multiple_of(zi * 64, 64)
    _wait(group(5))
    part, pts = mix1(3)
    u_acc[...] += part
    ln_tiles([4, 5], pts, z0, win=1)

    def step_b(i, carry):
        _wait(group_b(i))
        pts = mix1_pair(2 + i, u_acc, (0, 64, 128, 176, HM), True)
        ln_tiles([6 + 2 * i, 7 + 2 * i], pts, z0, win=2)
        return carry

    lax.fori_loop(0, 5, step_b, 0)
    _wait(group(11))
    pts_last = mix1_pair(7, u_fin, None, False)
    prep_part(0, pts_last)
    b1 = b1_v[...].astype(f32)

    def gelu_cols(cs, pts):
        cs = list(cs)
        for ci, c in enumerate(cs):
            for d in range(HG):
                def g(i, j):
                    pt = pts[(((ci * HG + d) * 4 + 2 * i + j) * len(pts)) // (len(cs) * HG * 4)]
                    n = j * (NF // 2) + c
                    u = tie(u_fin[(i * HG + d) * H:(i * HG + d + 1) * H, n * 128:(n + 1) * 128], pt)
                    return _gelu(u + b1[n:n + 1, :])
                ops = _lhs7(g(0, 0), g(0, 1), g(1, 0), g(1, 1))
                for q in range(7):
                    ga[q, d * 8:(d + 1) * 8, c * 128:(c + 1) * 128] = _pk(ops[q])

    order = list(range(NB - (W - 1), NB)) + list(range(NB - (W - 1)))

    def put_part(j, p, r0, v):
        z = z0 if order.index(j) >= 10 else 0
        qkv[j][pl.ds(z + p * D + r0, v.shape[0]), :] = v
        if j >= NB - (W - 1) and p > 0:
            kvr[j - (NB - (W - 1))][pl.ds((p - 1) * D + r0, v.shape[0]), :] = pltpu.roll(v, 2, axis=1)

    def nt_sums(dst, rows, pts):
        for g in range(8):
            pt = [pts[((2 * g + c) * len(pts)) // 16] for c in range(2)]
            b, c = [[_rows16(rows(j, k), g).astype(f32) for k in range(KT)] for j in range(2)]
            b[0], c[1], b[2] = tie(b[0], pt[0]), tie(c[1], pt[0]), tie(b[2], pt[1])
            ops = _rhs10(b, c, lo)
            for i in (0, 2, 3, 5, 6, 7, 8, 9):
                dst[i, g * H:(g + 1) * H, :] = ops[i]

    mxu = _Rounds(49)
    cut1 = [None]

    def nt_product(lhs, dst, rows):
        def mm(a, b, brief):
            if cut1[0] is not None:
                cuts, cut1[0] = cut1[0], None
                mxu.add(4)
                return _cat([_dot_nt(a[r0:r1, :], b) for r0, r1 in zip(cuts[:-1], cuts[1:])], axis=0)
            m = _dot_nt(a, b)
            mxu.add(1, m if brief else None)
            return m
        return _mm13(lhs, lambda i: rows(i // 4, i // 4) if i in (1, 4) else dst[i], mm)

    def xr(j, k):
        return _upk(xn_u[k, pl.ds(PJ * j, 64, stride=PL), :])

    def qkv_part(t, n):
        js = order[2 * t:2 * t + 2]
        c = nt_product(lambda i: _upk(l_s[i, n * HM // 2:(n + 1) * HM // 2, :]), xs[t], lambda j, k: xr(js[j], k))
        for q in (1, 0, 2, 3):
            put_part(js[q // 2], n, (q % 2) * HM, c[q])

    def qkv_quad(n):
        qkv_part(0, n)
        qkv_part(1, n)
        return mxu.take()

    def qkv_pair(t):
        for n in range(3):
            qkv_part(t, n)
        return mxu.take()

    def x_sums(t, pts):
        nt_sums(xs[t], lambda j, k: xr(order[2 * t + j], k), pts)

    def w2_sums(p, pts):
        def strip(r):
            top = w2_v[r * H:(r + 1) * H, _tiles(2 * p, 2)].astype(f32)
            bot = w2_v[F // 2 + r * H:F // 2 + (r + 1) * H, _tiles(2 * p, 2)].astype(f32)
            return top[:, 0:128], top[:, 128:], bot[:, 0:128], bot[:, 128:]
        rhs_sums(w2s[p], strip, F // 2 // H, pts, range(7))

    edge = lax.broadcasted_iota(jnp.int32, (H, 128), 1) < 2
    scale = DH ** -0.5

    def attn_block(j, pts):
        n_sm = (len(pts) * 14) // 100
        half = (len(pts) - n_sm) // 2

        def kv_rows(w, p, d):
            if j >= w:
                return qkv[j - w][pl.ds(p * D + d * H, H), :]
            return kvr[j - w + (W - 1)][pl.ds((p - 1) * D + d * H, H), :]

        def sm(v, f):
            return tie(v, pts[half + (f * n_sm) // 20])

        acc = [None] * W
        for d in range(DH):
            qd = tie(qkv[j][pl.ds(d * H, H), :], pts[(d * half) // DH])
            for w in range(W):
                t = qd * kv_rows(w, 1, d)
                acc[w] = t if acc[w] is None else acc[w] + t
        lg = [jnp.where(edge, -1e9 / scale, acc[w]) if w > j else acc[w] for w in range(W)]
        m = sm(_tree(jnp.maximum, lg), 2)
        e = [jnp.exp2(sm((l - m) * (scale * LOG2E), 4 + 2 * (w // 2))) for w, l in enumerate(lg)]
        ssum = sm(_tree(jnp.add, e), 14)
        inv = pl.reciprocal(ssum, approx=True)
        inv = sm(inv * (2.0 - ssum * inv), 18)
        a = [ew * inv for ew in e]
        for d in range(DH):
            o = a[0] * kv_rows(0, 2, d)
            for w in range(1, W):
                o = o + a[w] * kv_rows(w, 2, d)
            ob = tie(o, pts[half + n_sm + (d * half) // DH]).astype(bf16)
            oT[j][pl.ds(z0 + d * 8, 8), :] = _pk(ob)

    def last_wait(i, carry):
        _wait(group(12))
        return carry

    x_sums(0, _win(pts_last, 0, 15))
    x_sums(1, _win(pts_last, 80, 95))
    prep_part(1, qkv_quad(0))
    prep_part(2, qkv_quad(1))
    pts = qkv_quad(2)
    x_sums(2, _win(pts, 0, 20))
    gelu_cols((0,), _win(pts, 20, 100))
    mid = []
    for t in range(2, NB // 2):
        pts = qkv_pair(t)
        mid += pts
        if t == NB // 2 - 1:
            prep_wo(mid[n4:])
        if t + 1 < NB // 2:
            x_sums(t + 1, _win(pts, 0, 12 if t <= 4 else 70))
            pts = _win(pts, 12, 100)
        else:
            w2_sums(0, _win(mid[n4:], 0, 95))
        if t <= 4:
            gelu_cols((2 * t - 3, 2 * t - 2), _win(pts, 0, 100 if t < 4 else 94))
        if t == 4:
            lax.fori_loop(0, 1 + zi, last_wait, 0)
            cut1[0] = (0, 48, 96, 160, HM)
            n4 = len(mid)

    b2 = b2_v[...].astype(f32)

    def dot_rounds(a, b):
        k, nk, acc = 0, a.shape[1] // 128, None
        while k < nk:
            n = min(4 - mxu.n % 4, nk - k)
            if n > 1:
                p = _dot(a[:, k * 128:(k + n - 1) * 128], b[k * 128:(k + n - 1) * 128, :])
                acc = p if acc is None else acc + p
            p = _dot(a[:, (k + n - 1) * 128:(k + n) * 128], b[(k + n - 1) * 128:(k + n) * 128, :])
            mxu.add(n, None if acc is None else p)
            acc = p if acc is None else acc + p
            k += n
        return acc

    def mix2_pair(p):
        _, c = _strassen(lambda i: _upk(ga[i]), lambda i: w2s[p][i], dot_rounds)
        pts = mxu.take(SKIP)
        if p + 1 < NB // 2 - 1:
            w2_sums(p + 1, _win(pts, 0, 90))
        return pts, c

    def o_rows(n, k):
        return _upk(_cat([o_u[k, pl.ds(PL * (n * 4 + i), NB, stride=PJ), :] for i in range(4)], axis=0))

    def o_sums(p, pts):
        nt_sums(os_[p], lambda j, k: o_rows(2 * p + j, k), pts)

    def send(r0, r1, cols):
        pltpu.make_async_copy(out_v.at[r0:r1, cols], out_hbm.at[0, r0:r1, cols], sems.at[0]).start()

    late = []

    def wo_pair(p):
        c = nt_product(lambda i: _upk(wa[i]), os_[p], lambda j, k: o_rows(2 * p + j, k))
        pts = mxu.take()
        late.extend(pts)
        if p + 2 < NB // 2:
            o_sums(p + 2, pts)
        if p == NB // 2 - 2:
            w2_sums(NB // 2 - 1, late)
        return c

    def store_pair(p, first, second):
        last = p == NB // 2 - 1
        for q in (1, 0, 2, 3):
            n, r0 = 2 * p + q // 2, (q % 2) * HM
            res = ((x_v[n, r0:r0 + HM, :].astype(f32) + b2[n:n + 1, :] + first(q)) + second(q)).astype(bf16)
            if last and q == 3:
                for a, b in LASTR:
                    out_v[r0 + a:r0 + b, _tiles(n)] = res[a:b, :]
                    send(r0 + a, r0 + b, _tiles(n))
            else:
                out_v[r0:r0 + HM, _tiles(n)] = res
                if last:
                    send(r0, r0 + HM, _tiles(n))
        if not last:
            send(0, D, _tiles(2 * p, 2))

    pts = []
    for p in range(NPRE):
        pp, c = mix2_pair(p)
        for q in range(4):
            y_v[4 * p + q] = c[q]
        pts += pp
    line = mid[n4:] + pts
    pos = 0
    for j in range(NB):
        n = PPA if pos < len(mid) - n4 - PPA // 2 else PPB
        attn_block(j, line[pos:pos + n])
        pos += n
    for j in range(NB):
        to_rows(put_o, j, oT[j][...])
    o_sums(0, pts[-5 * KEEP:-3 * KEEP])
    o_sums(1, pts[-3 * KEEP:-KEEP])
    for p in range(NPRE):
        c = wo_pair(p)
        store_pair(p, lambda q: y_v[4 * p + q], lambda q: c[q])
    for p in range(NPRE, NB // 2):
        c = wo_pair(p)
        _, y = mix2_pair(p)
        store_pair(p, lambda q: c[q], lambda q: y[q])
    _wait([pltpu.make_async_copy(out_v, out_hbm.at[0], sems.at[0])])


@jax.jit
def pallas_parallel_sum__sliding_local_dilated__mixer_token_mlp__prompt_kernel(
        A_x, A_wqkv, A_wo, B_x, B_w1, B_b1, B_w2, B_b2):
    any_spec = pl.BlockSpec(memory_space=pl.ANY)
    out_t = pl.pallas_call(
        _kernel,
        out_shape=jax.ShapeDtypeStruct((1, D, S), bf16),
        in_specs=[any_spec] * 7,
        out_specs=any_spec,
        scratch_shapes=[
            pltpu.VMEM((NB, D, 128), bf16),
            pltpu.VMEM((D, 3 * D), bf16),
            pltpu.VMEM((D, D), bf16),
            pltpu.VMEM((S, F), bf16),
            pltpu.VMEM((F, S), bf16),
            pltpu.VMEM((NF, 128), bf16),
            pltpu.VMEM((NB, 128), bf16),
            pltpu.VMEM((D // 2, 128), u32),
            pltpu.VMEM((7, HM // 2, 128), u32),
            pltpu.VMEM((7 * HM // 2, 128), u32),
            pltpu.VMEM((4, D // 2, 128), u32),
            pltpu.VMEM((KT, PROWS, 128), u32),
            pltpu.VMEM((D, F), f32),
            pltpu.VMEM((D, F), f32),
            pltpu.VMEM((7, HM // 2, F // 2), u32),
            pltpu.VMEM((13, HM // 2, 128), u32),
            pltpu.VMEM((KT, D + 32, 128), f32),
            pltpu.VMEM((KT, D + 32, 128), f32),
            pltpu.VMEM((KT, D + 32, 128), f32),
            pltpu.VMEM((KT, D + 32, 128), f32),
            pltpu.VMEM((13, 3 * HM // 2, 128), u32),
            pltpu.VMEM((KT, PROWS, 128), u32),
            pltpu.VMEM((4 * NPRE, HM, 128), f32),
            pltpu.VMEM((D, S), bf16),
            pltpu.SemaphoreType.DMA((NG,)),
        ] + [pltpu.VMEM((3 * D, 128), f32)] * NB + [pltpu.VMEM((2 * D, 128), f32)] * (W - 1)
          + [pltpu.VMEM((D // 2, 128), u32)] * NB + [pltpu.VMEM((7, F // 2, 128), bf16)] * 8
          + [pltpu.VMEM((10, 128, 128), bf16)] * 16,
        compiler_params=pltpu.CompilerParams(vmem_limit_bytes=100 * 2**20, disable_semaphore_checks=True),
    )(jnp.swapaxes(A_x, 1, 2), A_wqkv, A_wo, B_w1, B_b1.reshape(NF, 128), B_w2, B_b2.reshape(NB, 128))
    return jnp.swapaxes(out_t, 1, 2)
```
